```python
import jax
import jax.numpy as jnp

def _softmax(x, axis=-1):
    return jax.nn.softmax(x, axis=axis)
def _gelu(x):
    return jax.nn.gelu(x, approximate=True)
def _silu(x):
    return jax.nn.silu(x)
def _sigmoid(x):
    return jax.nn.sigmoid(x)
def _layernorm(x, axis=-1, eps=1e-5):
    m = jnp.mean(x, axis=axis, keepdims=True)
    v = jnp.var(x, axis=axis, keepdims=True)
    return (x - m) / jnp.sqrt(v + eps)
def _scatter_add(tgt, idx, src, axis=0):
    return tgt.at[idx].add(src)
def _segment_sum(src, seg, n):
    return jax.ops.segment_sum(src, seg, n)
class _Rng:
    def __init__(self, key):
        self._k = key
    def _next(self):
        self._k, sub = jax.random.split(self._k)
        return sub
    def normal(self, shape):
        return jax.random.normal(self._next(), shape, dtype=jnp.bfloat16)
    def randint(self, lo, hi, shape):
        return jax.random.randint(self._next(), shape, lo, hi, dtype=jnp.int32)
    def uniform(self, shape, lo=0.0, hi=1.0):
        return jax.random.uniform(self._next(), shape, jnp.bfloat16, lo, hi)
    def permutation(self, n):
        return jax.random.permutation(self._next(), n)


kernel_name = 'gated_mix__compressed_kv_cla__ssm_conv_h3__prompt'

def setup_inputs():
    _rng = _Rng(jax.random.key(int.from_bytes(__import__("os").urandom(4), "little")))
    _w = (lambda a: (lambda t: t.astype(jnp.bfloat16) if jnp.issubdtype(t.dtype, jnp.floating) else t)(jnp.asarray(a)))
    def _A_setup():
        B, H, Sq, Sk, D, M = 1, 32, 2048, 2048, 128, 1024
        Dc = 4 * D
        return {
            "x": _w((lambda *s: _rng.normal(s) * 0.05)(B, Sq, M)),
            "c_kv": _w((lambda *s: _rng.normal(s) * 0.05)(B, Sk, Dc)),
            "w_q": _w((lambda *s: _rng.normal(s) * 0.05)(M, H, D) * (M ** -0.5)),
            "w_uk": _w((lambda *s: _rng.normal(s) * 0.05)(Dc, H, D) * (Dc ** -0.5)),
            "w_uv": _w((lambda *s: _rng.normal(s) * 0.05)(Dc, H, D) * (Dc ** -0.5)),
            "w_o": _w((lambda *s: _rng.normal(s) * 0.05)(H, D, M) * ((H * D) ** -0.5)),
        }
    _A_in = _A_setup()

    def _B_setup():
        B, S, D = 1, 2048, 1024
        ks = 4
        return {
            "q": _w((lambda *s: _rng.normal(s) * 0.05)(B, S, D)),
            "k": _w((lambda *s: _rng.normal(s) * 0.05)(B, S, D)),
            "v": _w((lambda *s: _rng.normal(s) * 0.05)(B, S, D)),
            "shift_k": _w((lambda *s: _rng.normal(s) * 0.05)(D, ks) * 0.5),
            "ssm_k": _w((lambda *s: _rng.normal(s) * 0.05)(D, S) * (1.0 / S ** 0.5)),
            "ssm_D": _w((lambda *s: _rng.normal(s) * 0.05)(D)),
        }
    _B_in = _B_setup()

    return {
        "A_x": _A_in["x"],
        "A_c_kv": _A_in["c_kv"],
        "A_w_q": _A_in["w_q"],
        "A_w_uk": _A_in["w_uk"],
        "A_w_uv": _A_in["w_uv"],
        "A_w_o": _A_in["w_o"],
        "B_q": _B_in["q"],
        "B_k": _B_in["k"],
        "B_v": _B_in["v"],
        "B_shift_k": _B_in["shift_k"],
        "B_ssm_k": _B_in["ssm_k"],
        "B_ssm_D": _B_in["ssm_D"],
        "gate_w": _w((lambda *s: _rng.normal(s) * 0.05)(1024)),
    }

def reference(A_x, A_c_kv, A_w_q, A_w_uk, A_w_uv, A_w_o, B_q, B_k, B_v, B_shift_k, B_ssm_k, B_ssm_D, gate_w):
    def _A_ref(x, c_kv, w_q, w_uk, w_uv, w_o):
        B, Sq, M = x.shape[0], x.shape[1], x.shape[2]
        Sk = c_kv.shape[1]
        H, D = w_q.shape[1], w_q.shape[2]
        q = jnp.einsum("bqm,mhd->bhqd", x, w_q)
        k = jnp.einsum("bkc,chd->bhkd", c_kv, w_uk)
        v = jnp.einsum("bkc,chd->bhkd", c_kv, w_uv)
        scores = jnp.einsum("bhqd,bhkd->bhqk", q, k) * (D ** -0.5)
        off = Sk - Sq
        qi = jnp.arange(Sq)[:, None]
        kj = jnp.arange(Sk)[None, :]
        cmask = kj <= (qi + off)
        scores = jnp.where(cmask[None, None], scores, -1e9)
        p = _softmax(scores, axis=-1)
        ctx = jnp.einsum("bhqk,bhkd->bhqd", p, v)
        return jnp.einsum("bhqd,hdm->bqm", ctx, w_o)

    def _B_ref(q, k, v, shift_k, ssm_k, ssm_D):
        B, S, D = q.shape
        ks = shift_k.shape[-1]
        k_pad = jnp.pad(k, ((0, 0), (ks - 1, 0), (0, 0)))
        k_shift = jnp.zeros_like(k)
        for t in range(ks):
            k_shift = k_shift + k_pad[:, t:t + S, :] * shift_k[:, ks - 1 - t][None, None, :]
        kv = k_shift * v
        L = 2 * S
        kv_pad = jnp.pad(kv, ((0, 0), (0, S), (0, 0)))
        kf_pad = jnp.pad(ssm_k, ((0, 0), (0, S)))
        kv_f = (lambda x, axes=(-2,-1): jnp.fft.rfft2(x.astype(jnp.float32), axes=axes))(kv_pad[:, None, :, :], axes=(1, 2))
        kf_f = (lambda x, axes=(-2,-1): jnp.fft.rfft2(x.astype(jnp.float32), axes=axes))(kf_pad[:, None, :], axes=(1, 2))
        kf_f = (lambda x, *d: x.transpose(*d))(kf_f, 1, 2, 0)
        y_f = kv_f * kf_f[None, :, :, :]
        y = (lambda x, s, axes=(-2,-1): jnp.fft.irfft2(x, s=s, axes=axes).astype(jnp.bfloat16))(y_f, (1, L), axes=(1, 2))[:, 0, :S, :]
        y = y + kv * ssm_D[None, None, :]
        return q * y

    x = A_x
    g = _sigmoid((x * gate_w).sum(-1, keepdims=True))
    a = _A_ref(x, A_c_kv, A_w_q, A_w_uk, A_w_uv, A_w_o)
    b = _B_ref(x, B_k, B_v, B_shift_k, B_ssm_k, B_ssm_D)
    return g * a + (1 - g) * b
```

```python
import functools
import math

import jax
import jax.numpy as jnp
import numpy as np
import jax.experimental.pallas as pl
import jax.experimental.pallas.tpu as pltpu

BF = jnp.bfloat16
F32 = jnp.float32
U32 = jnp.uint32

S = 2048
M = 1024
C = 512
H = 32
D = 128
T = 128
NB = S // T
NL = M // T
NEG = -1e30
NT_DIMS = (((1,), (1,)), ((), ()))

ATT_G = 2
OUT_R = 256


def _tobf(x):
    return pltpu.bitcast(x, BF)


def _tou(x):
    return pltpu.bitcast(x, U32)


def _lo_hi(w):
    lo = pltpu.bitcast(w << 16, F32)
    hi = pltpu.bitcast(w & jnp.uint32(0xFFFF0000), F32)
    return lo, hi


def _dft_consts():
    n_fft = 2 * T
    f = np.concatenate([np.arange(0, T, 2), np.arange(1, T, 2)]).astype(np.float64)
    theta = 2.0 * np.pi * (f + 0.5) / n_fft
    n = np.arange(T, dtype=np.float64)
    ang = theta[:, None] * n[None, :]
    fwd = np.concatenate([np.cos(ang), -np.sin(ang)], axis=0)
    inv = np.concatenate([np.cos(ang).T, -np.sin(ang).T], axis=1) * (2.0 / n_fft)
    return fwd.astype(np.float32), inv.astype(np.float32)


def _attn_qtile(h, j, k_s, qT_s, vT_s, ctx_s):
    q0 = j * T
    qT = _tobf(qT_s[h, :, q0:q0 + T])
    m = None
    for i in range(j + 1):
        k0 = i * T
        kk = _tobf(k_s[h, k0 // 2:(k0 + T) // 2, :])
        s = jnp.dot(kk, qT, preferred_element_type=F32)
        if i == j:
            ki = jax.lax.broadcasted_iota(jnp.int32, (T, T), 0)
            qi = jax.lax.broadcasted_iota(jnp.int32, (T, T), 1)
            s = jnp.where(ki <= qi, s, NEG)
        mc = jnp.max(s, axis=0, keepdims=True)
        m_new = mc if m is None else jnp.maximum(m, mc)
        p = jnp.exp2(s - m_new)
        lc = jnp.sum(p.reshape(T // 8, 8, T), axis=0)
        pv = jnp.dot(_tobf(vT_s[h, :, k0:k0 + T]), p.astype(BF), preferred_element_type=F32)
        if m is None:
            acc, l = pv, lc
        else:
            alpha = jnp.exp2(m - m_new)
            l = alpha * l + lc
            acc = alpha * acc + pv
        m = m_new
    lsum = jnp.sum(l, axis=0, keepdims=True)
    o = acc * (1.0 / lsum)
    ctx_s[h, q0 // 2:(q0 + T) // 2, :] = _tou(o.T.astype(BF))


def _conv_tile(lt, bk_v, bv_v, sk_v, skT_s, fwd, kpad_s, kv_s, q_s):
    kf = bk_v[lt].astype(F32)
    kpad_s[8:, :] = kf
    sk = skT_s[lt]
    ksh = kf * sk[0:1, :]
    for j in range(1, 4):
        ksh = ksh + kpad_s[8 - j:8 - j + S, :] * sk[j:j + 1, :]
    kv = (ksh * bv_v[lt].astype(F32)).astype(BF)
    kv_s[lt] = _tou(kv)
    us, ks = [], []
    ssm = sk_v[pl.ds(pl.multiple_of(lt * T, T), T), :]
    for i in range(NB):
        us.append(jnp.dot(fwd, kv[i * T:(i + 1) * T], preferred_element_type=F32))
        ks.append(jax.lax.dot_general(fwd, ssm[:, i * T:(i + 1) * T], NT_DIMS,
                                      preferred_element_type=F32))
    q_re = [[None] * (T // 8) for _ in range(NB)]
    q_im = [[None] * (T // 8) for _ in range(NB)]
    for g in range(T // 8):
        r0 = g * 8
        ur = [u[r0:r0 + 8] for u in us]
        ui = [u[T + r0:T + r0 + 8] for u in us]
        kr = [k[r0:r0 + 8] for k in ks]
        ki = [k[T + r0:T + r0 + 8] for k in ks]
        even = g < T // 16
        wr, wi = [kr[0]], [ki[0]]
        for d in range(1, NB):
            if even:
                wr.append(kr[d] - ki[d - 1])
                wi.append(ki[d] + kr[d - 1])
            else:
                wr.append(kr[d] + ki[d - 1])
                wi.append(ki[d] - kr[d - 1])

        def tconv(a, b):
            outs = []
            for mm in range(NB):
                t = a[0] * b[mm]
                for i in range(1, mm + 1):
                    t = t + a[i] * b[mm - i]
                outs.append(t)
            return outs

        ca = tconv([a + b for a, b in zip(ur, ui)], wr)
        cb = tconv(ur, [b - a for a, b in zip(wr, wi)])
        cc = tconv(ui, [a + b for a, b in zip(wr, wi)])
        for mm in range(NB):
            q_re[mm][g] = ca[mm] - cc[mm]
            q_im[mm][g] = ca[mm] + cb[mm]
    for mm in range(NB):
        qm = jnp.concatenate(q_re[mm] + q_im[mm], axis=0).astype(BF)
        q_s[lt, mm] = _tou(qm)


def _kernel(x_hbm, c_hbm, wq_hbm, wuk_hbm, wuv_hbm, wo_hbm, bk_hbm, bv_hbm, sk_hbm,
            shT_ref, dvec_ref, gw_ref, fwd_ref, inv_ref,
            out_hbm,
            x_v, wo_v, qT_s, k_s, vT_s, kv_s, q_s, sems, osems):
    qscale = (D ** -0.5) * math.log2(math.e)

    def phase1(c_v, wq_v, wuk_v, wuv_v, bk_v, bv_v, sk_v, skT_s, kpad_s):
        cp_c = pltpu.make_async_copy(c_hbm, c_v, sems.at[0])
        cp_wuk = pltpu.make_async_copy(wuk_hbm, wuk_v, sems.at[1])
        cp_c.start()
        cp_wuk.start()
        cp_wuv = pltpu.make_async_copy(wuv_hbm, wuv_v, sems.at[2])
        cp_x = pltpu.make_async_copy(x_hbm, x_v, sems.at[3])
        cp_wq = pltpu.make_async_copy(wq_hbm, wq_v, sems.at[4])
        cp_sk = pltpu.make_async_copy(sk_hbm, sk_v, sems.at[5])
        cp_bk = [pltpu.make_async_copy(bk_hbm.at[:, pl.ds(lt * T, T)], bk_v.at[lt], sems.at[6])
                 for lt in range(NL)]
        cp_bv = [pltpu.make_async_copy(bv_hbm.at[:, pl.ds(lt * T, T)], bv_v.at[lt], sems.at[7])
                 for lt in range(NL)]
        cp_wo = pltpu.make_async_copy(wo_hbm, wo_v, sems.at[8])

        shT = shT_ref[...].astype(F32)
        for lt in range(NL):
            skT_s[lt] = jnp.concatenate(
                [shT[:, lt * T:(lt + 1) * T], jnp.zeros((4, T), F32)], axis=0)
        kpad_s[:, 0:8, :] = jnp.zeros((2, 8, T), F32)

        cp_c.wait()
        cp_wuk.wait()
        for cp in [cp_wuv, cp_x, cp_wq, cp_sk] + cp_bk + cp_bv + [cp_wo]:
            cp.start()

        wq32 = wq_v.bitcast(U32)
        wuk32 = wuk_v.bitcast(U32)
        wuv32 = wuv_v.bitcast(U32)

        def load_pairs(w32, rows, it, transpose):
            view = w32.at[pl.ds(pl.multiple_of(it * 4, 4), rows * 16 - 12)]
            outs = []
            for g in range(4):
                w = view[pl.ds(g, rows, stride=16), :]
                if transpose:
                    w = w.T
                lo, hi = _lo_hi(w)
                outs += [lo.astype(BF), hi.astype(BF)]
            return jnp.concatenate(outs, axis=0 if transpose else 1)

        def k_body(it, carry):
            w = load_pairs(wuk32, C, it, False)
            k = jnp.dot(c_v[...], w, preferred_element_type=F32)
            for g in range(8):
                k_s[it * 8 + g] = _tou(k[:, g * D:(g + 1) * D].astype(BF))
            return carry

        jax.lax.fori_loop(0, 4, k_body, 0)
        cp_wuv.wait()

        def v_body(it, carry):
            w = load_pairs(wuv32, C, it, True)
            vT = jax.lax.dot_general(w, c_v[...], NT_DIMS, preferred_element_type=F32)
            for g in range(8):
                vT_s[it * 8 + g] = _tou(vT[g * D:(g + 1) * D].astype(BF))
            return carry

        jax.lax.fori_loop(0, 4, v_body, 0)
        for cp in [cp_x, cp_wq, cp_sk] + cp_bk + cp_bv:
            cp.wait()

        def q_body(it, carry):
            w = load_pairs(wq32, M, it, True)
            qT = jax.lax.dot_general(w, x_v[...], NT_DIMS, preferred_element_type=F32) * qscale
            for g in range(8):
                qT_s[it * 8 + g] = _tou(qT[g * D:(g + 1) * D].astype(BF))
            fwd = fwd_ref[...]
            for u in range(2):
                _conv_tile(it * 2 + u, bk_v, bv_v, sk_v, skT_s, fwd, kpad_s.at[u], kv_s, q_s)
            return carry

        jax.lax.fori_loop(0, 4, q_body, 0)
        cp_wo.wait()

    pl.run_scoped(
        phase1,
        pltpu.VMEM((S, C), BF),
        pltpu.VMEM((M * H, D), BF),
        pltpu.VMEM((C * H, D), BF),
        pltpu.VMEM((C * H, D), BF),
        pltpu.VMEM((NL, S, T), BF),
        pltpu.VMEM((NL, S, T), BF),
        pltpu.VMEM((M, S), BF),
        pltpu.VMEM((NL, 8, T), F32),
        pltpu.VMEM((2, S + 8, T), F32),
    )

    def phase23(ctx_s, out_v):
        def att_body(it, carry):
            for j in range(NB):
                for g in range(ATT_G):
                    _attn_qtile(it * ATT_G + g, j, k_s, qT_s, vT_s, ctx_s)
            return carry

        jax.lax.fori_loop(0, H // ATT_G, att_body, 0)

        R = OUT_R
        gw = gw_ref[...].astype(F32).reshape(1, M)
        dv = dvec_ref[...].astype(F32).reshape(1, M)

        def out_copy(it):
            rows = pl.ds(pl.multiple_of(it * R, R), R)
            return pltpu.make_async_copy(out_v.at[rows], out_hbm.at[rows], osems.at[it])

        def out_body(it, carry):
            rows = pl.ds(pl.multiple_of(it * R, R), R)
            prow = pl.ds(pl.multiple_of(it * (R // 2), R // 2), R // 2)
            ctx = jnp.concatenate([_tobf(ctx_s[h, prow, :]) for h in range(H)], axis=1)
            a = jnp.dot(ctx, wo_v[...], preferred_element_type=F32)
            inv = inv_ref[...]
            ys = []
            for mm in range(R // T):
                m = it * (R // T) + mm
                qm = jnp.concatenate([_tobf(q_s[lt, m]) for lt in range(NL)], axis=1)
                ys.append(jnp.dot(inv, qm, preferred_element_type=F32))
            y = jnp.concatenate(ys, axis=0)
            kv = jnp.concatenate([_tobf(kv_s[lt, prow, :]) for lt in range(NL)], axis=1).astype(F32)
            xr = x_v[rows, :].astype(F32)
            g = jax.nn.sigmoid(jnp.sum(xr * gw, axis=-1, keepdims=True))
            b = xr * (y + kv * dv)
            out_v[rows, :] = (g * a + (1.0 - g) * b).astype(BF)
            out_copy(it).start()
            return carry

        jax.lax.fori_loop(0, S // R, out_body, 0)
        for it in range(S // R):
            out_copy(it).wait()

    pl.run_scoped(
        phase23,
        pltpu.VMEM((H, S // 2, D), U32),
        pltpu.VMEM((S, M), BF),
    )


@jax.jit
def pallas_gated_mix__compressed_kv_cla__ssm_conv_h3__prompt_kernel(
    A_x, A_c_kv, A_w_q, A_w_uk, A_w_uv, A_w_o, B_q, B_k, B_v, B_shift_k, B_ssm_k, B_ssm_D, gate_w,
):
    fwd_np, inv_np = _dft_consts()
    fwd = jnp.asarray(fwd_np, dtype=BF)
    inv = jnp.asarray(inv_np, dtype=BF)
    any_spec = pl.BlockSpec(memory_space=pl.ANY)
    vmem_spec = pl.BlockSpec(memory_space=pltpu.VMEM)
    out = pl.pallas_call(
        _kernel,
        out_shape=jax.ShapeDtypeStruct((S, M), BF),
        in_specs=[any_spec] * 9 + [vmem_spec] * 5,
        out_specs=any_spec,
        scratch_shapes=[
            pltpu.VMEM((S, M), BF),
            pltpu.VMEM((H * D, M), BF),
            pltpu.VMEM((H, D // 2, S), U32),
            pltpu.VMEM((H, S // 2, D), U32),
            pltpu.VMEM((H, D // 2, S), U32),
            pltpu.VMEM((NL, S // 2, T), U32),
            pltpu.VMEM((NL, NB, T, T), U32),
            pltpu.SemaphoreType.DMA((9,)),
            pltpu.SemaphoreType.DMA((S // OUT_R,)),
        ],
        compiler_params=pltpu.CompilerParams(vmem_limit_bytes=120 * 1024 * 1024),
    )(
        A_x.reshape(S, M), A_c_kv.reshape(S, C),
        A_w_q.reshape(M * H, D), A_w_uk.reshape(C * H, D), A_w_uv.reshape(C * H, D),
        A_w_o.reshape(H * D, M),
        B_k.reshape(S, M), B_v.reshape(S, M), B_ssm_k,
        B_shift_k.T, B_ssm_D, gate_w, fwd, inv,
    )
    return out.reshape(1, S, M)
```

```python
import functools
import math

import jax
import jax.numpy as jnp
import numpy as np
import jax.experimental.pallas as pl
import jax.experimental.pallas.tpu as pltpu

BF = jnp.bfloat16
F32 = jnp.float32
U32 = jnp.uint32

S = 2048
M = 1024
C = 512
H = 32
D = 128
T = 128
NB = S // T
NL = M // T
NEG = -1e30
NT_DIMS = (((1,), (1,)), ((), ()))

ATT_G = 2
OUT_R = 256


def _tobf(x):
    return pltpu.bitcast(x, BF)


def _tou(x):
    return pltpu.bitcast(x, U32)


def _lo_hi(w):
    lo = pltpu.bitcast(w << 16, F32)
    hi = pltpu.bitcast(w & jnp.uint32(0xFFFF0000), F32)
    return lo, hi


def _dft_consts():
    n_fft = 2 * T
    f = np.concatenate([np.arange(0, T, 2), np.arange(1, T, 2)]).astype(np.float64)
    theta = 2.0 * np.pi * (f + 0.5) / n_fft
    n = np.arange(T, dtype=np.float64)
    ang = theta[:, None] * n[None, :]
    fwd = np.concatenate([np.cos(ang), -np.sin(ang)], axis=0)
    inv = np.concatenate([np.cos(ang).T, -np.sin(ang).T], axis=1) * (2.0 / n_fft)
    return fwd.astype(np.float32), inv.astype(np.float32)


def _attn_qtile(h, j, k_s, qT_s, vT_s, ctx_s):
    q0 = j * T
    qT = _tobf(qT_s[h, :, q0:q0 + T])
    m = None
    for i in range(j + 1):
        k0 = i * T
        kk = _tobf(k_s[h, k0 // 2:(k0 + T) // 2, :])
        s = jnp.dot(kk, qT, preferred_element_type=F32)
        if i == j:
            ki = jax.lax.broadcasted_iota(jnp.int32, (T, T), 0)
            qi = jax.lax.broadcasted_iota(jnp.int32, (T, T), 1)
            s = jnp.where(ki <= qi, s, NEG)
        mc = jnp.max(s, axis=0, keepdims=True)
        m_new = mc if m is None else jnp.maximum(m, mc)
        p = jnp.exp2(s - m_new)
        lc = jnp.sum(p.reshape(T // 8, 8, T), axis=0)
        pv = jnp.dot(_tobf(vT_s[h, :, k0:k0 + T]), p.astype(BF), preferred_element_type=F32)
        if m is None:
            acc, l = pv, lc
        else:
            alpha = jnp.exp2(m - m_new)
            l = alpha * l + lc
            acc = alpha * acc + pv
        m = m_new
    lsum = jnp.sum(l, axis=0, keepdims=True)
    o = acc * (1.0 / lsum)
    ctx_s[h, q0 // 2:(q0 + T) // 2, :] = _tou(o.T.astype(BF))


def _conv_tile(lt, bk_v, bv_v, sk_v, skT_s, fwd, kpad_s, kv_s, q_s):
    kf = bk_v[lt].astype(F32)
    kpad_s[8:, :] = kf
    sk = skT_s[lt]
    ksh = kf * sk[0:1, :]
    for j in range(1, 4):
        ksh = ksh + kpad_s[8 - j:8 - j + S, :] * sk[j:j + 1, :]
    kv = (ksh * bv_v[lt].astype(F32)).astype(BF)
    kv_s[lt] = _tou(kv)
    us, ks = [], []
    ssm = sk_v[pl.ds(pl.multiple_of(lt * T, T), T), :]
    for i in range(NB):
        us.append(jnp.dot(fwd, kv[i * T:(i + 1) * T], preferred_element_type=F32))
        ks.append(jax.lax.dot_general(fwd, ssm[:, i * T:(i + 1) * T], NT_DIMS,
                                      preferred_element_type=F32))
    q_re = [[None] * (T // 8) for _ in range(NB)]
    q_im = [[None] * (T // 8) for _ in range(NB)]
    for g in range(T // 8):
        r0 = g * 8
        ur = [u[r0:r0 + 8] for u in us]
        ui = [u[T + r0:T + r0 + 8] for u in us]
        kr = [k[r0:r0 + 8] for k in ks]
        ki = [k[T + r0:T + r0 + 8] for k in ks]
        even = g < T // 16
        wr, wi = [kr[0]], [ki[0]]
        for d in range(1, NB):
            if even:
                wr.append(kr[d] - ki[d - 1])
                wi.append(ki[d] + kr[d - 1])
            else:
                wr.append(kr[d] + ki[d - 1])
                wi.append(ki[d] - kr[d - 1])

        def tconv(a, b):
            outs = []
            for mm in range(NB):
                t = a[0] * b[mm]
                for i in range(1, mm + 1):
                    t = t + a[i] * b[mm - i]
                outs.append(t)
            return outs

        ca = tconv([a + b for a, b in zip(ur, ui)], wr)
        cb = tconv(ur, [b - a for a, b in zip(wr, wi)])
        cc = tconv(ui, [a + b for a, b in zip(wr, wi)])
        for mm in range(NB):
            q_re[mm][g] = ca[mm] - cc[mm]
            q_im[mm][g] = ca[mm] + cb[mm]
    for mm in range(NB):
        qm = jnp.concatenate(q_re[mm] + q_im[mm], axis=0).astype(BF)
        q_s[lt, mm] = _tou(qm)


def _kernel(x_hbm, c_hbm, wq_hbm, wuk_hbm, wuv_hbm, wo_hbm, bk_hbm, bv_hbm, sk_hbm,
            shT_ref, dvec_ref, gw_ref, fwd_ref, inv_ref,
            out_hbm,
            x_v, wo_v, qT_s, k_s, vT_s, kv_s, q_s, sems, osems):
    qscale = (D ** -0.5) * math.log2(math.e)

    def phase1(c_v, wq_v, wuk_v, wuv_v, bk_v, bv_v, sk_v, skT_s, kpad_s):
        cp_c = pltpu.make_async_copy(c_hbm, c_v, sems.at[0])
        cp_wuk = pltpu.make_async_copy(wuk_hbm, wuk_v, sems.at[1])
        cp_c.start()
        cp_wuk.start()
        cp_wuv = pltpu.make_async_copy(wuv_hbm, wuv_v, sems.at[2])
        cp_x = pltpu.make_async_copy(x_hbm, x_v, sems.at[3])
        cp_wq = pltpu.make_async_copy(wq_hbm, wq_v, sems.at[4])
        cp_sk = pltpu.make_async_copy(sk_hbm, sk_v, sems.at[5])
        cp_bk = [pltpu.make_async_copy(bk_hbm.at[:, pl.ds(lt * T, T)], bk_v.at[lt], sems.at[6])
                 for lt in range(NL)]
        cp_bv = [pltpu.make_async_copy(bv_hbm.at[:, pl.ds(lt * T, T)], bv_v.at[lt], sems.at[7])
                 for lt in range(NL)]
        cp_wo = pltpu.make_async_copy(wo_hbm, wo_v, sems.at[8])

        shT = shT_ref[...].astype(F32)
        for lt in range(NL):
            skT_s[lt] = jnp.concatenate(
                [shT[:, lt * T:(lt + 1) * T], jnp.zeros((4, T), F32)], axis=0)
        kpad_s[:, 0:8, :] = jnp.zeros((2, 8, T), F32)

        with jax.named_scope("wait0"):
            cp_c.wait()
            cp_wuk.wait()
        for cp in [cp_wuv, cp_x, cp_wq, cp_sk] + cp_bk + cp_bv + [cp_wo]:
            cp.start()

        wq32 = wq_v.bitcast(U32)
        wuk32 = wuk_v.bitcast(U32)
        wuv32 = wuv_v.bitcast(U32)

        def load_pairs(w32, rows, it, transpose):
            view = w32.at[pl.ds(pl.multiple_of(it * 4, 4), rows * 16 - 12)]
            outs = []
            for g in range(4):
                w = view[pl.ds(g, rows, stride=16), :]
                if transpose:
                    w = w.T
                lo, hi = _lo_hi(w)
                outs += [lo.astype(BF), hi.astype(BF)]
            return jnp.concatenate(outs, axis=0 if transpose else 1)

        def k_body(it, carry):
            w = load_pairs(wuk32, C, it, False)
            k = jnp.dot(c_v[...], w, preferred_element_type=F32)
            for g in range(8):
                k_s[it * 8 + g] = _tou(k[:, g * D:(g + 1) * D].astype(BF))
            return carry

        with jax.named_scope("kproj"):
            jax.lax.fori_loop(0, 4, k_body, 0)
        with jax.named_scope("wait1"):
            cp_wuv.wait()

        def v_body(it, carry):
            w = load_pairs(wuv32, C, it, True)
            vT = jax.lax.dot_general(w, c_v[...], NT_DIMS, preferred_element_type=F32)
            for g in range(8):
                vT_s[it * 8 + g] = _tou(vT[g * D:(g + 1) * D].astype(BF))
            return carry

        with jax.named_scope("vproj"):
            jax.lax.fori_loop(0, 4, v_body, 0)
        with jax.named_scope("wait2"):
            for cp in [cp_x, cp_wq, cp_sk] + cp_bk + cp_bv:
                cp.wait()

        def q_body(it, carry):
            w = load_pairs(wq32, M, it, True)
            qT = jax.lax.dot_general(w, x_v[...], NT_DIMS, preferred_element_type=F32) * qscale
            for g in range(8):
                qT_s[it * 8 + g] = _tou(qT[g * D:(g + 1) * D].astype(BF))
            fwd = fwd_ref[...]
            for u in range(2):
                _conv_tile(it * 2 + u, bk_v, bv_v, sk_v, skT_s, fwd, kpad_s.at[u], kv_s, q_s)
            return carry

        with jax.named_scope("qproj"):
            jax.lax.fori_loop(0, 4, q_body, 0)
        with jax.named_scope("wait3"):
            cp_wo.wait()

    pl.run_scoped(
        phase1,
        pltpu.VMEM((S, C), BF),
        pltpu.VMEM((M * H, D), BF),
        pltpu.VMEM((C * H, D), BF),
        pltpu.VMEM((C * H, D), BF),
        pltpu.VMEM((NL, S, T), BF),
        pltpu.VMEM((NL, S, T), BF),
        pltpu.VMEM((M, S), BF),
        pltpu.VMEM((NL, 8, T), F32),
        pltpu.VMEM((2, S + 8, T), F32),
    )

    def phase23(ctx_s, out_v):
        def att_body(it, carry):
            for j in range(NB):
                for g in range(ATT_G):
                    _attn_qtile(it * ATT_G + g, j, k_s, qT_s, vT_s, ctx_s)
            return carry

        with jax.named_scope("attn"):
            jax.lax.fori_loop(0, H // ATT_G, att_body, 0)

        R = OUT_R
        gw = gw_ref[...].astype(F32).reshape(1, M)
        dv = dvec_ref[...].astype(F32).reshape(1, M)

        def out_copy(it):
            rows = pl.ds(pl.multiple_of(it * R, R), R)
            return pltpu.make_async_copy(out_v.at[rows], out_hbm.at[rows], osems.at[it])

        def out_body(it, carry):
            rows = pl.ds(pl.multiple_of(it * R, R), R)
            prow = pl.ds(pl.multiple_of(it * (R // 2), R // 2), R // 2)
            ctx = jnp.concatenate([_tobf(ctx_s[h, prow, :]) for h in range(H)], axis=1)
            a = jnp.dot(ctx, wo_v[...], preferred_element_type=F32)
            inv = inv_ref[...]
            ys = []
            for mm in range(R // T):
                m = it * (R // T) + mm
                qm = jnp.concatenate([_tobf(q_s[lt, m]) for lt in range(NL)], axis=1)
                ys.append(jnp.dot(inv, qm, preferred_element_type=F32))
            y = jnp.concatenate(ys, axis=0)
            kv = jnp.concatenate([_tobf(kv_s[lt, prow, :]) for lt in range(NL)], axis=1).astype(F32)
            xr = x_v[rows, :].astype(F32)
            g = jax.nn.sigmoid(jnp.sum(xr * gw, axis=-1, keepdims=True))
            b = xr * (y + kv * dv)
            out_v[rows, :] = (g * a + (1.0 - g) * b).astype(BF)
            out_copy(it).start()
            return carry

        with jax.named_scope("oproj"):
            jax.lax.fori_loop(0, S // R, out_body, 0)
        with jax.named_scope("wait4"):
            for it in range(S // R):
                out_copy(it).wait()

    pl.run_scoped(
        phase23,
        pltpu.VMEM((H, S // 2, D), U32),
        pltpu.VMEM((S, M), BF),
    )


@jax.jit
def pallas_gated_mix__compressed_kv_cla__ssm_conv_h3__prompt_kernel(
    A_x, A_c_kv, A_w_q, A_w_uk, A_w_uv, A_w_o, B_q, B_k, B_v, B_shift_k, B_ssm_k, B_ssm_D, gate_w,
):
    fwd_np, inv_np = _dft_consts()
    fwd = jnp.asarray(fwd_np, dtype=BF)
    inv = jnp.asarray(inv_np, dtype=BF)
    any_spec = pl.BlockSpec(memory_space=pl.ANY)
    vmem_spec = pl.BlockSpec(memory_space=pltpu.VMEM)
    out = pl.pallas_call(
        _kernel,
        out_shape=jax.ShapeDtypeStruct((S, M), BF),
        in_specs=[any_spec] * 9 + [vmem_spec] * 5,
        out_specs=any_spec,
        scratch_shapes=[
            pltpu.VMEM((S, M), BF),
            pltpu.VMEM((H * D, M), BF),
            pltpu.VMEM((H, D // 2, S), U32),
            pltpu.VMEM((H, S // 2, D), U32),
            pltpu.VMEM((H, D // 2, S), U32),
            pltpu.VMEM((NL, S // 2, T), U32),
            pltpu.VMEM((NL, NB, T, T), U32),
            pltpu.SemaphoreType.DMA((9,)),
            pltpu.SemaphoreType.DMA((S // OUT_R,)),
        ],
        compiler_params=pltpu.CompilerParams(vmem_limit_bytes=120 * 1024 * 1024),
    )(
        A_x.reshape(S, M), A_c_kv.reshape(S, C),
        A_w_q.reshape(M * H, D), A_w_uk.reshape(C * H, D), A_w_uv.reshape(C * H, D),
        A_w_o.reshape(H * D, M),
        B_k.reshape(S, M), B_v.reshape(S, M), B_ssm_k,
        B_shift_k.T, B_ssm_D, gate_w, fwd, inv,
    )
    return out.reshape(1, S, M)
```

```python
import functools
import math

import jax
import jax.numpy as jnp
import numpy as np
import jax.experimental.pallas as pl
import jax.experimental.pallas.tpu as pltpu

BF = jnp.bfloat16
F32 = jnp.float32
U32 = jnp.uint32

S = 2048
M = 1024
C = 512
H = 32
D = 128
T = 128
NB = S // T
NL = M // T
NEG = -1e30
NT_DIMS = (((1,), (1,)), ((), ()))

ATT_G = 4
OUT_R = 256


def _tobf(x):
    return pltpu.bitcast(x, BF)


def _tou(x):
    return pltpu.bitcast(x, U32)


def _lo_hi(w):
    lo = pltpu.bitcast(w << 16, F32)
    hi = pltpu.bitcast(w & jnp.uint32(0xFFFF0000), F32)
    return lo, hi


def _dft_consts():
    n_fft = 2 * T
    f = np.concatenate([np.arange(0, T, 2), np.arange(1, T, 2)]).astype(np.float64)
    theta = 2.0 * np.pi * (f + 0.5) / n_fft
    n = np.arange(T, dtype=np.float64)
    ang = theta[:, None] * n[None, :]
    re = np.cos(ang)
    im = -np.sin(ang)
    fwd = np.concatenate([re.reshape(T // 8, 8, T), im.reshape(T // 8, 8, T)], axis=1)
    fwd = fwd.reshape(2 * T, T)
    inv = np.stack([re, im], axis=1).reshape(2 * T, T).T * (2.0 / n_fft)
    return fwd.astype(np.float32), inv.astype(np.float32)


def _attn_qtile(h, j, k_s, qT_s, vT_s, ctx_s):
    q0 = j * T
    qT = _tobf(qT_s[h, :, q0:q0 + T])
    m = None
    for i in range(j + 1):
        k0 = i * T
        kk = _tobf(k_s[h, k0 // 2:(k0 + T) // 2, :])
        s = jnp.dot(kk, qT, preferred_element_type=F32)
        if i == j:
            ki = jax.lax.broadcasted_iota(jnp.int32, (T, T), 0)
            qi = jax.lax.broadcasted_iota(jnp.int32, (T, T), 1)
            s = jnp.where(ki <= qi, s, NEG)
        mc = jnp.max(s, axis=0, keepdims=True)
        m_new = mc if m is None else jnp.maximum(m, mc)
        p = jnp.exp2(s - m_new)
        lc = jnp.sum(p.reshape(T // 8, 8, T), axis=0)
        pv = jnp.dot(_tobf(vT_s[h, :, k0:k0 + T]), p.astype(BF), preferred_element_type=F32)
        if m is None:
            acc, l = pv, lc
        else:
            alpha = jnp.exp2(m - m_new)
            l = alpha * l + lc
            acc = alpha * acc + pv
        m = m_new
    lsum = jnp.sum(l, axis=0, keepdims=True)
    o = acc * (1.0 / lsum)
    ctx_s[h, :, q0:q0 + T] = _tou(o.astype(BF))


MG = 8
IG = 4
KVCH = 2
FIRST = 3
LAST = 15
NG = T // 8
U_OFF = 0
W_OFF = U_OFF + NB * NG * 24
A_OFF = W_OFF + NB * NG * 24
R_OFF = A_OFF + NB * 8
DUMMY = R_OFF + NB * 8
UK_ROWS = DUMMY + 8


def _conv_pieces(lt, bk_v, bv_v, sk_v, skT_s, fwd_ref, kpad_s, kv_s, q_s, uk_s, dyn, dyn2):
    st = {}

    def p_kv(i, val):
        if val is not None:
            kpad_s[pl.ds(dyn2, 8), :] = val
        r0 = i * T
        kf = bk_v[lt, r0:r0 + T, :].astype(F32)
        kpad_s[8 + r0:8 + r0 + T, :] = kf
        sk = skT_s[lt]
        ksh = kf * sk[0:1, :]
        for j in range(1, 4):
            ksh = ksh + kpad_s[8 + r0 - j:8 + r0 - j + T, :] * sk[j:j + 1, :]
        kv = (ksh * bv_v[lt, r0:r0 + T, :].astype(F32)).astype(BF)
        kv_s[lt, r0 // 2:(r0 + T) // 2, :] = _tou(kv)
        st["kv", i] = kv

    def p_dft_k(_):
        fwd = fwd_ref[...]
        ssm = sk_v[pl.ds(pl.multiple_of(lt * T, T), T), :]
        prev = None
        for d in range(NB):
            k = jax.lax.dot_general(fwd, ssm[:, d * T:(d + 1) * T], NT_DIMS,
                                    preferred_element_type=F32)
            for g in range(NG):
                kr, ki = k[16 * g:16 * g + 8], k[16 * g + 8:16 * g + 16]
                if prev is None:
                    wr, wi = kr, ki
                else:
                    pr, pi = prev[16 * g:16 * g + 8], prev[16 * g + 8:16 * g + 16]
                    if g < NG // 2:
                        wr, wi = kr - pi, ki + pr
                    else:
                        wr, wi = kr + pi, ki - pr
                r = W_OFF + (d * NG + g) * 24
                uk_s[r:r + 8, :] = wr
                uk_s[r + 8:r + 16, :] = wi - wr
                uk_s[r + 16:r + 24, :] = -(wr + wi)
            prev = k

    def p_dft_u(i):
        fwd = fwd_ref[...]
        u = jnp.dot(fwd, st["kv", i], preferred_element_type=F32)
        for g in range(NG):
            ur, ui = u[16 * g:16 * g + 8], u[16 * g + 8:16 * g + 16]
            r = U_OFF + (i * NG + g) * 24
            uk_s[r:r + 8, :] = ur
            uk_s[r + 8:r + 16, :] = ui
            uk_s[r + 16:r + 24, :] = ur + ui

    def gate(val):
        if val is not None:
            uk_s[pl.ds(dyn, 8), :] = val

    def ld1(off, g, k, i):
        r = off + (i * NG + g) * 24 + 8 * k
        return uk_s[r:r + 8, :]

    def sub(kind, g, m0, i0, val):
        gate(val)
        ka, kb = {"a": (2, 0), "c": (1, 2), "b": (0, 1)}[kind]
        ms = range(m0, m0 + MG)
        if i0 == 0:
            if kind == "a":
                st["acc"] = {m: None for m in ms}
            else:
                st["acc"] = {m: uk_s[A_OFF + 8 * m:A_OFF + 8 * m + 8, :] for m in ms}
        acc = st["acc"]
        av = {i: ld1(U_OFF, g, ka, i) for i in range(i0, min(i0 + IG, m0 + MG))}
        bv = {}
        for i in av:
            for m in ms:
                j = m - i
                if j < 0:
                    continue
                if j not in bv:
                    bv[j] = ld1(W_OFF, g, kb, j)
                t = av[i] * bv[j]
                acc[m] = t if acc[m] is None else acc[m] + t
        if i0 + IG >= m0 + MG:
            for m in ms:
                if kind == "a":
                    uk_s[A_OFF + 8 * m:A_OFF + 8 * m + 8, :] = acc[m]
                elif kind == "c":
                    uk_s[R_OFF + 8 * m:R_OFF + 8 * m + 8, :] = acc[m]
                else:
                    re = uk_s[R_OFF + 8 * m:R_OFF + 8 * m + 8, :]
                    q_s[lt, m, g * 8:(g + 1) * 8, :] = pltpu.pack_elementwise(
                        [re, acc[m]], packed_dtype=BF)

    subs = []
    for g in range(NG):
        for kind in ("a", "c", "b"):
            for m0 in range(0, NB, MG):
                for i0 in range(0, m0 + MG, IG):
                    subs.append(functools.partial(sub, kind, g, m0, i0))
    return p_dft_k, p_kv, p_dft_u, subs


def _spread(subs, n, first, last, slabs=128):
    sched = [[] for _ in range(n)]
    npts = (last - first) * slabs
    for i, pc in enumerate(subs):
        pt = (i * npts) // len(subs)
        sched[first + pt // slabs].append((pt % slabs, pc))
    return sched


def _kernel(x_hbm, c_hbm, wq_hbm, wuk_hbm, wuv_hbm, wo_hbm, bk_hbm, bv_hbm, sk_hbm,
            shT_ref, dvec_ref, gw_ref, fwd_ref, inv_ref,
            out_hbm,
            x_v, wo_v, qT_s, k_s, vT_s, kv_s, q_s, sems, osems):
    qscale = (D ** -0.5) * math.log2(math.e)

    def phase1(c_v, wq_v, wuk_v, wuv_v, bk_v, bv_v, sk_v, skT_s, kpad_s, uk_s, dyn_s):
        dyn_s[0] = DUMMY
        dyn_s[1] = S + 8
        cp_c = pltpu.make_async_copy(c_hbm, c_v, sems.at[0])
        cp_wuk = pltpu.make_async_copy(wuk_hbm, wuk_v, sems.at[1])
        cp_c.start()
        cp_wuk.start()
        cp_wuv = pltpu.make_async_copy(wuv_hbm, wuv_v, sems.at[2])
        cp_x = pltpu.make_async_copy(x_hbm, x_v, sems.at[3])
        cp_wq = pltpu.make_async_copy(wq_hbm, wq_v, sems.at[4])
        cp_sk = pltpu.make_async_copy(sk_hbm, sk_v, sems.at[5])
        cp_bk = [pltpu.make_async_copy(bk_hbm.at[:, pl.ds(lt * T, T)], bk_v.at[lt], sems.at[6])
                 for lt in range(NL)]
        cp_bv = [pltpu.make_async_copy(bv_hbm.at[:, pl.ds(lt * T, T)], bv_v.at[lt], sems.at[7])
                 for lt in range(NL)]
        cp_wo = pltpu.make_async_copy(wo_hbm, wo_v, sems.at[8])

        shT = shT_ref[...].astype(F32)
        for lt in range(NL):
            skT_s[lt] = jnp.concatenate(
                [shT[:, lt * T:(lt + 1) * T], jnp.zeros((4, T), F32)], axis=0)
        kpad_s[0:8, :] = jnp.zeros((8, T), F32)

        with jax.named_scope("wait0"):
            cp_c.wait()
            cp_wuk.wait()
        for cp in [cp_wuv, cp_sk] + cp_bk + cp_bv:
            cp.start()

        wq32 = wq_v.bitcast(U32)
        wuk32 = wuk_v.bitcast(U32)
        wuv32 = wuv_v.bitcast(U32)

        def load_pairs(w32, rows, it, transpose):
            view = w32.at[pl.ds(pl.multiple_of(it * 4, 4), rows * 16 - 12)]
            outs = []
            for g in range(4):
                w = view[pl.ds(g, rows, stride=16), :]
                if transpose:
                    w = w.T
                outs += list(_lo_hi(w))
            return jnp.concatenate(outs, axis=0 if transpose else 1).astype(BF)

        def k_body(it, carry):
            view = wuk32.at[pl.ds(pl.multiple_of(it * 4, 4), C * 16 - 12)]
            for g in range(4):
                lo, hi = _lo_hi(view[pl.ds(g, C, stride=16), :])
                w = jnp.concatenate([lo, hi], axis=1).astype(BF)
                k = jnp.dot(c_v[...], w, preferred_element_type=F32)
                for u in range(2):
                    k_s[it * 8 + 2 * g + u] = _tou(k[:, u * D:(u + 1) * D].astype(BF))
            return carry

        with jax.named_scope("kproj"):
            jax.lax.fori_loop(0, 4, k_body, 0)
        for cp in [cp_x, cp_wq, cp_wo]:
            cp.start()
        with jax.named_scope("wait1"):
            for cp in [cp_wuv, cp_sk] + cp_bk + cp_bv:
                cp.wait()

        def proj_conv_body(it, lt, w32, rows, src_v, dst_s, scale):
            p_dft_k, p_kv, p_dft_u, subs = _conv_pieces(
                lt, bk_v, bv_v, sk_v, skT_s, fwd_ref, kpad_s, kv_s, q_s, uk_s,
                pl.multiple_of(dyn_s[0], 8), pl.multiple_of(dyn_s[1], 8))
            p_dft_k(None)
            w = load_pairs(w32, rows, it, True)
            sched = _spread(subs, NB, FIRST, LAST)
            nkv = NB // KVCH
            for n in range(NB):
                o = jax.lax.dot_general(w, src_v[n * T:(n + 1) * T, :], NT_DIMS,
                                        preferred_element_type=F32)
                if scale is not None:
                    o = o * scale
                for g in range(8):
                    dst_s[it * 8 + g, :, n * T:(n + 1) * T] = _tou(o[g * D:(g + 1) * D].astype(BF))
                if 1 <= n <= KVCH:
                    for i in range((n - 1) * nkv, n * nkv):
                        p_dft_u(i)
                if n < KVCH:
                    for k_ in range(nkv):
                        sl = (128 * k_) // nkv
                        p_kv(n * nkv + k_, o[8 * sl:8 * sl + 8])
                for sl, pc in sched[n]:
                    pc(o[8 * sl:8 * sl + 8])

        def v_body(it, carry):
            proj_conv_body(it, it, wuv32, C, c_v, vT_s, None)
            return carry

        with jax.named_scope("vproj"):
            jax.lax.fori_loop(0, 4, v_body, 0)
        with jax.named_scope("wait2"):
            for cp in [cp_x, cp_wq]:
                cp.wait()

        def q_body(it, carry):
            proj_conv_body(it, 4 + it, wq32, M, x_v, qT_s, qscale)
            return carry

        with jax.named_scope("qproj"):
            jax.lax.fori_loop(0, 4, q_body, 0)
        with jax.named_scope("wait3"):
            cp_wo.wait()

    pl.run_scoped(
        phase1,
        pltpu.VMEM((S, C), BF),
        pltpu.VMEM((M * H, D), BF),
        pltpu.VMEM((C * H, D), BF),
        pltpu.VMEM((C * H, D), BF),
        pltpu.VMEM((NL, S, T), BF),
        pltpu.VMEM((NL, S, T), BF),
        pltpu.VMEM((M, S), BF),
        pltpu.VMEM((NL, 8, T), F32),
        pltpu.VMEM((S + 16, T), F32),
        pltpu.VMEM((UK_ROWS, T), F32),
        pltpu.SMEM((2,), jnp.int32),
    )

    def phase23(ctx_s, out_v):
        def att_body(it, carry):
            for j in range(NB):
                for g in range(ATT_G):
                    _attn_qtile(it * ATT_G + g, j, k_s, qT_s, vT_s, ctx_s)
            return carry

        with jax.named_scope("attn"):
            jax.lax.fori_loop(0, H // ATT_G, att_body, 0)

        R = OUT_R
        gw = gw_ref[...].astype(F32).reshape(1, M)
        dv = dvec_ref[...].astype(F32).reshape(1, M)

        def out_copy(it):
            rows = pl.ds(pl.multiple_of(it * R, R), R)
            return pltpu.make_async_copy(out_v.at[rows], out_hbm.at[rows], osems.at[it])

        def out_body(it, carry):
            rows = pl.ds(pl.multiple_of(it * R, R), R)
            prow = pl.ds(pl.multiple_of(it * (R // 2), R // 2), R // 2)
            inv = inv_ref[...]
            ys = []
            for mm in range(R // T):
                m = it * (R // T) + mm
                qm = jnp.concatenate([_tobf(q_s[lt, m]) for lt in range(NL)], axis=1)
                ys.append(jnp.dot(inv, qm, preferred_element_type=F32))
            y = jnp.concatenate(ys, axis=0)
            ctx = jnp.concatenate([_tobf(ctx_s[h, :, rows]).T for h in range(H)], axis=1)
            a = jnp.dot(ctx, wo_v[...], preferred_element_type=F32)
            kv = jnp.concatenate([_tobf(kv_s[lt, prow, :]) for lt in range(NL)], axis=1).astype(F32)
            xr = x_v[rows, :].astype(F32)
            g = jax.nn.sigmoid(jnp.sum(xr * gw, axis=-1, keepdims=True))
            b = xr * (y + kv * dv)
            out_v[rows, :] = (g * a + (1.0 - g) * b).astype(BF)
            out_copy(it).start()
            return carry

        with jax.named_scope("oproj"):
            jax.lax.fori_loop(0, S // R, out_body, 0)
        with jax.named_scope("wait4"):
            for it in range(S // R):
                out_copy(it).wait()

    pl.run_scoped(
        phase23,
        pltpu.VMEM((H, D // 2, S), U32),
        pltpu.VMEM((S, M), BF),
    )


@jax.jit
def pallas_gated_mix__compressed_kv_cla__ssm_conv_h3__prompt_kernel(
    A_x, A_c_kv, A_w_q, A_w_uk, A_w_uv, A_w_o, B_q, B_k, B_v, B_shift_k, B_ssm_k, B_ssm_D, gate_w,
):
    fwd_np, inv_np = _dft_consts()
    fwd = jnp.asarray(fwd_np, dtype=BF)
    inv = jnp.asarray(inv_np, dtype=BF)
    any_spec = pl.BlockSpec(memory_space=pl.ANY)
    vmem_spec = pl.BlockSpec(memory_space=pltpu.VMEM)
    out = pl.pallas_call(
        _kernel,
        out_shape=jax.ShapeDtypeStruct((S, M), BF),
        in_specs=[any_spec] * 9 + [vmem_spec] * 5,
        out_specs=any_spec,
        scratch_shapes=[
            pltpu.VMEM((S, M), BF),
            pltpu.VMEM((H * D, M), BF),
            pltpu.VMEM((H, D // 2, S), U32),
            pltpu.VMEM((H, S // 2, D), U32),
            pltpu.VMEM((H, D // 2, S), U32),
            pltpu.VMEM((NL, S // 2, T), U32),
            pltpu.VMEM((NL, NB, T, T), U32),
            pltpu.SemaphoreType.DMA((9,)),
            pltpu.SemaphoreType.DMA((S // OUT_R,)),
        ],
        compiler_params=pltpu.CompilerParams(vmem_limit_bytes=120 * 1024 * 1024),
    )(
        A_x.reshape(S, M), A_c_kv.reshape(S, C),
        A_w_q.reshape(M * H, D), A_w_uk.reshape(C * H, D), A_w_uv.reshape(C * H, D),
        A_w_o.reshape(H * D, M),
        B_k.reshape(S, M), B_v.reshape(S, M), B_ssm_k,
        B_shift_k.T, B_ssm_D, gate_w, fwd, inv,
    )
    return out.reshape(1, S, M)
```

```python
import functools
import math

import jax
import jax.numpy as jnp
import numpy as np
import jax.experimental.pallas as pl
import jax.experimental.pallas.tpu as pltpu

BF = jnp.bfloat16
F32 = jnp.float32
U32 = jnp.uint32

S = 2048
M = 1024
C = 512
H = 32
D = 128
T = 128
NB = S // T
NL = M // T
NEG = -1e30
NT_DIMS = (((1,), (1,)), ((), ()))

ATT_G = 4
C0 = 512
OUT_R = 256


def _tobf(x):
    return pltpu.bitcast(x, BF)


def _tou(x):
    return pltpu.bitcast(x, U32)


def _lo_hi(w):
    lo = pltpu.bitcast(w << 16, F32)
    hi = pltpu.bitcast(w & jnp.uint32(0xFFFF0000), F32)
    return lo, hi


def _dft_consts():
    n_fft = 2 * T
    f = np.concatenate([np.arange(0, T, 2), np.arange(1, T, 2)]).astype(np.float64)
    theta = 2.0 * np.pi * (f + 0.5) / n_fft
    n = np.arange(T, dtype=np.float64)
    ang = theta[:, None] * n[None, :]
    re = np.cos(ang)
    im = -np.sin(ang)
    fwd = np.concatenate([re.reshape(T // 8, 8, T), im.reshape(T // 8, 8, T)], axis=1)
    fwd = fwd.reshape(2 * T, T)
    inv = np.stack([re, im], axis=1).reshape(2 * T, T).T * (2.0 / n_fft)
    return fwd.astype(np.float32), inv.astype(np.float32)


def _attn_qtile(h, j, k_s, qT_s, vT_s, ctx_s):
    q0 = j * T
    qT = _tobf(qT_s[h, :, q0:q0 + T])
    m = None
    for i in range(j + 1):
        k0 = i * T
        kk = _tobf(k_s[h, k0 // 2:(k0 + T) // 2, :])
        s = jnp.dot(kk, qT, preferred_element_type=F32)
        if i == j:
            ki = jax.lax.broadcasted_iota(jnp.int32, (T, T), 0)
            qi = jax.lax.broadcasted_iota(jnp.int32, (T, T), 1)
            s = jnp.where(ki <= qi, s, NEG)
        mc = jnp.max(s, axis=0, keepdims=True)
        m_new = mc if m is None else jnp.maximum(m, mc)
        p = jnp.exp2(s - m_new)
        lc = jnp.sum(p.reshape(T // 8, 8, T), axis=0)
        pv = jnp.dot(_tobf(vT_s[h, :, k0:k0 + T]), p.astype(BF), preferred_element_type=F32)
        if m is None:
            acc, l = pv, lc
        else:
            alpha = jnp.exp2(m - m_new)
            l = alpha * l + lc
            acc = alpha * acc + pv
        m = m_new
    lsum = jnp.sum(l, axis=0, keepdims=True)
    o = acc * (1.0 / lsum)
    ctx_s[h, :, q0:q0 + T] = _tou(o.astype(BF))


MG = 8
IG = 4
SPLIT0 = 1
KV0 = 1
KVCH = 2
FIRST = 4
LAST = 15
NG = T // 8
U_OFF = 0
W_OFF = U_OFF + NB * NG * 24
A_OFF = W_OFF + NB * NG * 24
R_OFF = A_OFF + NB * 8
DUMMY = R_OFF + NB * 8
UK_ROWS = DUMMY + 8


def _conv_pieces(lt, bk_v, bv_v, sk_v, skT_s, fwd_ref, kpad_s, kv_s, q_s, uk_s, dyn, dyn2):
    st = {}

    def p_kv(i, val):
        if val is not None:
            kpad_s[pl.ds(dyn2, 8), :] = val
        r0 = i * T
        kf = bk_v[lt, r0:r0 + T, :].astype(F32)
        kpad_s[8 + r0:8 + r0 + T, :] = kf
        sk = skT_s[lt]
        ksh = kf * sk[0:1, :]
        for j in range(1, 4):
            ksh = ksh + kpad_s[8 + r0 - j:8 + r0 - j + T, :] * sk[j:j + 1, :]
        kv = (ksh * bv_v[lt, r0:r0 + T, :].astype(F32)).astype(BF)
        kv_s[lt, r0 // 2:(r0 + T) // 2, :] = _tou(kv)
        st["kv", i] = kv

    def p_dft_k(_):
        fwd = fwd_ref[...]
        ssm = sk_v[pl.ds(pl.multiple_of(lt * T, T), T), :]
        prev = None
        for d in range(NB):
            k = jax.lax.dot_general(fwd, ssm[:, d * T:(d + 1) * T], NT_DIMS,
                                    preferred_element_type=F32)
            for g in range(NG):
                kr, ki = k[16 * g:16 * g + 8], k[16 * g + 8:16 * g + 16]
                if prev is None:
                    wr, wi = kr, ki
                else:
                    pr, pi = prev[16 * g:16 * g + 8], prev[16 * g + 8:16 * g + 16]
                    if g < NG // 2:
                        wr, wi = kr - pi, ki + pr
                    else:
                        wr, wi = kr + pi, ki - pr
                r = W_OFF + (d * NG + g) * 24
                uk_s[r:r + 8, :] = wr
                uk_s[r + 8:r + 16, :] = wi - wr
                uk_s[r + 16:r + 24, :] = -(wr + wi)
            prev = k

    def p_dft_u(i):
        fwd = fwd_ref[...]
        u = jnp.dot(fwd, st["kv", i], preferred_element_type=F32)
        for g in range(NG):
            ur, ui = u[16 * g:16 * g + 8], u[16 * g + 8:16 * g + 16]
            r = U_OFF + (i * NG + g) * 24
            uk_s[r:r + 8, :] = ur
            uk_s[r + 8:r + 16, :] = ui
            uk_s[r + 16:r + 24, :] = ur + ui

    def gate(val):
        if val is not None:
            uk_s[pl.ds(dyn, 8), :] = val

    def ld1(off, g, k, i):
        r = off + (i * NG + g) * 24 + 8 * k
        return uk_s[r:r + 8, :]

    def sub(kind, g, m0, i0, val):
        gate(val)
        ka, kb = {"a": (2, 0), "c": (1, 2), "b": (0, 1)}[kind]
        ms = range(m0, m0 + MG)
        if i0 == 0:
            if kind == "a":
                st["acc"] = {m: None for m in ms}
            else:
                st["acc"] = {m: uk_s[A_OFF + 8 * m:A_OFF + 8 * m + 8, :] for m in ms}
        acc = st["acc"]
        av = {i: ld1(U_OFF, g, ka, i) for i in range(i0, min(i0 + IG, m0 + MG))}
        bv = {}
        for i in av:
            for m in ms:
                j = m - i
                if j < 0:
                    continue
                if j not in bv:
                    bv[j] = ld1(W_OFF, g, kb, j)
                t = av[i] * bv[j]
                acc[m] = t if acc[m] is None else acc[m] + t
        if i0 + IG >= m0 + MG:
            for m in ms:
                if kind == "a":
                    uk_s[A_OFF + 8 * m:A_OFF + 8 * m + 8, :] = acc[m]
                elif kind == "c":
                    uk_s[R_OFF + 8 * m:R_OFF + 8 * m + 8, :] = acc[m]
                else:
                    re = uk_s[R_OFF + 8 * m:R_OFF + 8 * m + 8, :]
                    q_s[lt, m, g * 8:(g + 1) * 8, :] = pltpu.pack_elementwise(
                        [re, acc[m]], packed_dtype=BF)

    subs = []
    for g in range(NG):
        for kind in ("a", "c", "b"):
            for m0 in range(0, NB, MG):
                for i0 in range(0, m0 + MG, IG):
                    subs.append(functools.partial(sub, kind, g, m0, i0))
    return p_dft_k, p_kv, p_dft_u, subs


def _spread(subs, n, first, last, slabs=128):
    sched = [[] for _ in range(n)]
    npts = (last - first) * slabs
    for i, pc in enumerate(subs):
        pt = (i * npts) // len(subs)
        sched[first + pt // slabs].append((pt % slabs, pc))
    return sched


def _kernel(x_hbm, c_hbm, wq_hbm, wuk_hbm, wuv_hbm, wo_hbm, bk_hbm, bv_hbm, sk_hbm,
            shT_ref, dvec_ref, gw_ref, fwd_ref, inv_ref,
            out_hbm,
            x_v, wo_v, qT_s, k_s, vT_s, kv_s, q_s, sems, osems):
    qscale = (D ** -0.5) * math.log2(math.e)

    def phase1(c_v, wq_v, wuk_v, wuv_v, bk_v, bv_v, sk_v, skT_s, kpad_s, uk_s, dyn_s):
        dyn_s[0] = DUMMY
        dyn_s[1] = S + 8
        wuk_hbm32 = wuk_hbm.bitcast(U32)
        cp_wuk = [pltpu.make_async_copy(
            wuk_hbm32.at[:, pl.ds(4 * a, 4), :], wuk_v.at[a, :, pl.ds(0, 4), :], sems.at[9 + a])
            for a in range(4)]
        cp_c = [pltpu.make_async_copy(c_hbm.at[pl.ds(0, C0)], c_v.at[pl.ds(0, C0)], sems.at[0]),
                pltpu.make_async_copy(c_hbm.at[pl.ds(C0, S - C0)], c_v.at[pl.ds(C0, S - C0)],
                                      sems.at[1])]
        cp_wuv = pltpu.make_async_copy(wuv_hbm, wuv_v, sems.at[2])
        cp_x = pltpu.make_async_copy(x_hbm, x_v, sems.at[3])
        cp_wq = pltpu.make_async_copy(wq_hbm, wq_v, sems.at[4])
        cp_sk = pltpu.make_async_copy(sk_hbm, sk_v, sems.at[5])
        cp_bk = [pltpu.make_async_copy(bk_hbm.at[:, pl.ds(lt * T, T)], bk_v.at[lt], sems.at[6])
                 for lt in range(NL)]
        cp_bv = [pltpu.make_async_copy(bv_hbm.at[:, pl.ds(lt * T, T)], bv_v.at[lt], sems.at[7])
                 for lt in range(NL)]
        cp_wo = pltpu.make_async_copy(wo_hbm, wo_v, sems.at[8])
        for cp in ([cp_wuk[0], cp_c[0], cp_c[1]] + cp_wuk[1:] + [cp_wuv, cp_sk] + cp_bk + cp_bv
                   + [cp_x, cp_wq, cp_wo]):
            cp.start()

        shT = shT_ref[...].astype(F32)
        for lt in range(NL):
            skT_s[lt] = jnp.concatenate(
                [shT[:, lt * T:(lt + 1) * T], jnp.zeros((4, T), F32)], axis=0)
        kpad_s[0:8, :] = jnp.zeros((8, T), F32)

        wq32 = wq_v.bitcast(U32)
        wuv32 = wuv_v.bitcast(U32)

        def load_pairs(w32, rows, it, transpose):
            view = w32.at[pl.ds(pl.multiple_of(it * 4, 4), rows * 16 - 12)]
            outs = []
            for g in range(4):
                w = view[pl.ds(g, rows, stride=16), :]
                if transpose:
                    w = w.T
                outs += list(_lo_hi(w))
            return jnp.concatenate(outs, axis=0 if transpose else 1).astype(BF)

        wuk2 = wuk_v.reshape(4 * C * 8, D)

        def k_body(it, carry):
            pltpu.make_async_copy(wuk_hbm32.at[:, pl.ds(0, 4), :], wuk_v.at[it, :, pl.ds(0, 4), :],
                                  sems.at[9 + it]).wait()
            view = wuk2.at[pl.ds(pl.multiple_of(it * C * 8, 8), C * 8)]
            ws = []
            for g in range(4):
                lo, hi = _lo_hi(view[pl.ds(g, C, stride=8), :])
                ws.append(jnp.concatenate([lo, hi], axis=1).astype(BF))

            def k_proj(r0, r1):
                for g in range(4):
                    k = jnp.dot(c_v[r0:r1, :], ws[g], preferred_element_type=F32)
                    for u in range(2):
                        k_s[it * 8 + 2 * g + u, r0 // 2:r1 // 2, :] = _tou(
                            k[:, u * D:(u + 1) * D].astype(BF))

            k_proj(0, C0)

            @pl.when(it == 0)
            def _():
                cp_c[1].wait()

            k_proj(C0, S)
            return carry

        with jax.named_scope("wait0"):
            cp_c[0].wait()
        with jax.named_scope("kproj"):
            jax.lax.fori_loop(0, 4, k_body, 0)
        with jax.named_scope("wait1"):
            for cp in [cp_wuv, cp_sk] + cp_bk + cp_bv:
                cp.wait()

        def proj_conv_body(it, lt, w32, rows, src_v, dst_s, scale):
            p_dft_k, p_kv, p_dft_u, subs = _conv_pieces(
                lt, bk_v, bv_v, sk_v, skT_s, fwd_ref, kpad_s, kv_s, q_s, uk_s,
                pl.multiple_of(dyn_s[0], 8), pl.multiple_of(dyn_s[1], 8))
            p_dft_k(None)
            w = load_pairs(w32, rows, it, True)
            sched = _spread(subs, NB, FIRST, LAST)
            nkv = NB // KVCH
            for n in range(NB):
                src = src_v[n * T:(n + 1) * T, :]
                if n < SPLIT0:
                    o = jnp.concatenate(
                        [jax.lax.dot_general(w[p * 2 * D:(p + 1) * 2 * D], src, NT_DIMS,
                                             preferred_element_type=F32) for p in range(4)], axis=0)
                else:
                    o = jax.lax.dot_general(w, src, NT_DIMS, preferred_element_type=F32)
                if scale is not None:
                    o = o * scale
                for g in range(8):
                    dst_s[it * 8 + g, :, n * T:(n + 1) * T] = _tou(o[g * D:(g + 1) * D].astype(BF))
                if KV0 + 1 <= n <= KV0 + KVCH:
                    for i in range((n - KV0 - 1) * nkv, (n - KV0) * nkv):
                        p_dft_u(i)
                if KV0 <= n < KV0 + KVCH:
                    for k_ in range(nkv):
                        sl = (128 * k_) // nkv
                        p_kv((n - KV0) * nkv + k_, o[8 * sl:8 * sl + 8])
                for sl, pc in sched[n]:
                    pc(o[8 * sl:8 * sl + 8])

        def v_body(it, carry):
            proj_conv_body(it, it, wuv32, C, c_v, vT_s, None)
            return carry

        with jax.named_scope("vproj"):
            jax.lax.fori_loop(0, 4, v_body, 0)
        with jax.named_scope("wait2"):
            for cp in [cp_x, cp_wq]:
                cp.wait()

        def q_body(it, carry):
            proj_conv_body(it, 4 + it, wq32, M, x_v, qT_s, qscale)
            return carry

        with jax.named_scope("qproj"):
            jax.lax.fori_loop(0, 4, q_body, 0)
        with jax.named_scope("wait3"):
            cp_wo.wait()

    pl.run_scoped(
        phase1,
        pltpu.VMEM((S, C), BF),
        pltpu.VMEM((M * H, D), BF),
        pltpu.VMEM((4, C, 8, D), U32),
        pltpu.VMEM((C * H, D), BF),
        pltpu.VMEM((NL, S, T), BF),
        pltpu.VMEM((NL, S, T), BF),
        pltpu.VMEM((M, S), BF),
        pltpu.VMEM((NL, 8, T), F32),
        pltpu.VMEM((S + 16, T), F32),
        pltpu.VMEM((UK_ROWS, T), F32),
        pltpu.SMEM((2,), jnp.int32),
    )

    def phase23(ctx_s, out_v):
        def att_body(it, carry):
            for j in range(NB):
                for g in range(ATT_G):
                    _attn_qtile(it * ATT_G + g, j, k_s, qT_s, vT_s, ctx_s)
            return carry

        with jax.named_scope("attn"):
            jax.lax.fori_loop(0, H // ATT_G, att_body, 0)

        R = OUT_R
        gw = gw_ref[...].astype(F32).reshape(1, M)
        dv = dvec_ref[...].astype(F32).reshape(1, M)

        def out_copy(it):
            rows = pl.ds(pl.multiple_of(it * R, R), R)
            return pltpu.make_async_copy(out_v.at[rows], out_hbm.at[rows], osems.at[it])

        def out_body(it, carry):
            rows = pl.ds(pl.multiple_of(it * R, R), R)
            prow = pl.ds(pl.multiple_of(it * (R // 2), R // 2), R // 2)
            inv = inv_ref[...]
            ys = []
            for mm in range(R // T):
                m = it * (R // T) + mm
                qm = jnp.concatenate([_tobf(q_s[lt, m]) for lt in range(NL)], axis=1)
                ys.append(jnp.dot(inv, qm, preferred_element_type=F32))
            y = jnp.concatenate(ys, axis=0)
            ctx = jnp.concatenate([_tobf(ctx_s[h, :, rows]).T for h in range(H)], axis=1)
            a = jnp.dot(ctx, wo_v[...], preferred_element_type=F32)
            kv = jnp.concatenate([_tobf(kv_s[lt, prow, :]) for lt in range(NL)], axis=1).astype(F32)
            xr = x_v[rows, :].astype(F32)
            g = jax.nn.sigmoid(jnp.sum(xr * gw, axis=-1, keepdims=True))
            b = xr * (y + kv * dv)
            out_v[rows, :] = (g * a + (1.0 - g) * b).astype(BF)
            out_copy(it).start()
            return carry

        with jax.named_scope("oproj"):
            jax.lax.fori_loop(0, S // R, out_body, 0)
        with jax.named_scope("wait4"):
            for it in range(S // R):
                out_copy(it).wait()

    pl.run_scoped(
        phase23,
        pltpu.VMEM((H, D // 2, S), U32),
        pltpu.VMEM((S, M), BF),
    )


@jax.jit
def pallas_gated_mix__compressed_kv_cla__ssm_conv_h3__prompt_kernel(
    A_x, A_c_kv, A_w_q, A_w_uk, A_w_uv, A_w_o, B_q, B_k, B_v, B_shift_k, B_ssm_k, B_ssm_D, gate_w,
):
    fwd_np, inv_np = _dft_consts()
    fwd = jnp.asarray(fwd_np, dtype=BF)
    inv = jnp.asarray(inv_np, dtype=BF)
    any_spec = pl.BlockSpec(memory_space=pl.ANY)
    vmem_spec = pl.BlockSpec(memory_space=pltpu.VMEM)
    out = pl.pallas_call(
        _kernel,
        out_shape=jax.ShapeDtypeStruct((S, M), BF),
        in_specs=[any_spec] * 9 + [vmem_spec] * 5,
        out_specs=any_spec,
        scratch_shapes=[
            pltpu.VMEM((S, M), BF),
            pltpu.VMEM((H * D, M), BF),
            pltpu.VMEM((H, D // 2, S), U32),
            pltpu.VMEM((H, S // 2, D), U32),
            pltpu.VMEM((H, D // 2, S), U32),
            pltpu.VMEM((NL, S // 2, T), U32),
            pltpu.VMEM((NL, NB, T, T), U32),
            pltpu.SemaphoreType.DMA((13,)),
            pltpu.SemaphoreType.DMA((S // OUT_R,)),
        ],
        compiler_params=pltpu.CompilerParams(vmem_limit_bytes=120 * 1024 * 1024),
    )(
        A_x.reshape(S, M), A_c_kv.reshape(S, C),
        A_w_q.reshape(M * H, D), A_w_uk, A_w_uv.reshape(C * H, D),
        A_w_o.reshape(H * D, M),
        B_k.reshape(S, M), B_v.reshape(S, M), B_ssm_k,
        B_shift_k.T, B_ssm_D, gate_w, fwd, inv,
    )
    return out.reshape(1, S, M)
```

```python
import functools
import math

import jax
import jax.numpy as jnp
import numpy as np
import jax.experimental.pallas as pl
import jax.experimental.pallas.tpu as pltpu

BF = jnp.bfloat16
F32 = jnp.float32
U32 = jnp.uint32

S = 2048
M = 1024
C = 512
H = 32
D = 128
T = 128
NB = S // T
NL = M // T
NEG = -1e30
NT_DIMS = (((1,), (1,)), ((), ()))

ATT_G = 4
C0 = 512
SKEW = 8
OUT_R = 256


def _tobf(x):
    return pltpu.bitcast(x, BF)


def _tou(x):
    return pltpu.bitcast(x, U32)


def _lo_hi(w):
    lo = pltpu.bitcast(w << 16, F32)
    hi = pltpu.bitcast(w & jnp.uint32(0xFFFF0000), F32)
    return lo, hi


def _dft_consts():
    n_fft = 2 * T
    f = np.concatenate([np.arange(0, T, 2), np.arange(1, T, 2)]).astype(np.float64)
    theta = 2.0 * np.pi * (f + 0.5) / n_fft
    n = np.arange(T, dtype=np.float64)
    ang = theta[:, None] * n[None, :]
    re = np.cos(ang)
    im = -np.sin(ang)
    fwd = np.concatenate([re.reshape(T // 8, 8, T), im.reshape(T // 8, 8, T)], axis=1)
    fwd = fwd.reshape(2 * T, T)
    inv = np.stack([re, im], axis=1).reshape(2 * T, T).T * (2.0 / n_fft)
    return fwd.astype(np.float32), inv.astype(np.float32)


def _qk_tile(h, j, i, k_s, qT_s):
    qT = _tobf(qT_s[h, :, j * T:(j + 1) * T])
    kk = _tobf(k_s[h, i * T // 2:(i + 1) * T // 2, :])
    return jnp.dot(kk, qT, preferred_element_type=F32)


def _softmax_pv(h, j, i, s, st, vT_s, ctx_s):
    if i == j:
        ki = jax.lax.broadcasted_iota(jnp.int32, (T, T), 0)
        qi = jax.lax.broadcasted_iota(jnp.int32, (T, T), 1)
        s = jnp.where(ki <= qi, s, NEG)
    mc = jnp.max(s, axis=0, keepdims=True)
    m_new = mc if i == 0 else jnp.maximum(st["m"], mc)
    p = jnp.exp2(s - m_new)
    lc = jnp.sum(p.reshape(T // 8, 8, T), axis=0)
    pv = jnp.dot(_tobf(vT_s[h, :, i * T:(i + 1) * T]), p.astype(BF), preferred_element_type=F32)
    if i == 0:
        acc, l = pv, lc
    else:
        alpha = jnp.exp2(st["m"] - m_new)
        l = alpha * st["l"] + lc
        acc = alpha * st["acc"] + pv
    st.update(m=m_new, l=l, acc=acc)
    if i == j:
        lsum = jnp.sum(l, axis=0, keepdims=True)
        o = acc * (1.0 / lsum)
        ctx_s[h, :, j * T:(j + 1) * T] = _tou(o.astype(BF))


MG = 8
IG = 4
SPLIT0 = 1
KV0 = 1
KVCH = 2
FIRST = 4
LAST = 15
NG = T // 8
U_OFF = 0
W_OFF = U_OFF + NB * NG * 24
A_OFF = W_OFF + NB * NG * 24
R_OFF = A_OFF + NB * 8
DUMMY = R_OFF + NB * 8
UK_ROWS = DUMMY + 8


def _conv_pieces(lt, bk_v, bv_v, sk_v, skT_s, fwd_ref, kpad_s, kv_s, q_s, uk_s, dyn, dyn2):
    st = {}

    def p_kv(i, val):
        if val is not None:
            kpad_s[pl.ds(dyn2, 8), :] = val
        r0 = i * T
        kf = bk_v[lt, r0:r0 + T, :].astype(F32)
        kpad_s[8 + r0:8 + r0 + T, :] = kf
        sk = skT_s[lt]
        ksh = kf * sk[0:1, :]
        for j in range(1, 4):
            ksh = ksh + kpad_s[8 + r0 - j:8 + r0 - j + T, :] * sk[j:j + 1, :]
        kv = (ksh * bv_v[lt, r0:r0 + T, :].astype(F32)).astype(BF)
        kv_s[lt, r0 // 2:(r0 + T) // 2, :] = _tou(kv)
        st["kv", i] = kv

    def p_dft_k(_):
        fwd = fwd_ref[...]
        ssm = sk_v[pl.ds(pl.multiple_of(lt * T, T), T), :]
        prev = None
        for d in range(NB):
            k = jax.lax.dot_general(fwd, ssm[:, d * T:(d + 1) * T], NT_DIMS,
                                    preferred_element_type=F32)
            for g in range(NG):
                kr, ki = k[16 * g:16 * g + 8], k[16 * g + 8:16 * g + 16]
                if prev is None:
                    wr, wi = kr, ki
                else:
                    pr, pi = prev[16 * g:16 * g + 8], prev[16 * g + 8:16 * g + 16]
                    if g < NG // 2:
                        wr, wi = kr - pi, ki + pr
                    else:
                        wr, wi = kr + pi, ki - pr
                r = W_OFF + (d * NG + g) * 24
                uk_s[r:r + 8, :] = wr
                uk_s[r + 8:r + 16, :] = wi - wr
                uk_s[r + 16:r + 24, :] = -(wr + wi)
            prev = k

    def p_dft_u(i):
        fwd = fwd_ref[...]
        u = jnp.dot(fwd, st["kv", i], preferred_element_type=F32)
        for g in range(NG):
            ur, ui = u[16 * g:16 * g + 8], u[16 * g + 8:16 * g + 16]
            r = U_OFF + (i * NG + g) * 24
            uk_s[r:r + 8, :] = ur
            uk_s[r + 8:r + 16, :] = ui
            uk_s[r + 16:r + 24, :] = ur + ui

    def gate(val):
        if val is not None:
            uk_s[pl.ds(dyn, 8), :] = val

    def ld1(off, g, k, i):
        r = off + (i * NG + g) * 24 + 8 * k
        return uk_s[r:r + 8, :]

    def sub(kind, g, m0, i0, val):
        gate(val)
        ka, kb = {"a": (2, 0), "c": (1, 2), "b": (0, 1)}[kind]
        ms = range(m0, m0 + MG)
        if i0 == 0:
            if kind == "a":
                st["acc"] = {m: None for m in ms}
            else:
                st["acc"] = {m: uk_s[A_OFF + 8 * m:A_OFF + 8 * m + 8, :] for m in ms}
        acc = st["acc"]
        av = {i: ld1(U_OFF, g, ka, i) for i in range(i0, min(i0 + IG, m0 + MG))}
        bv = {}
        for i in av:
            for m in ms:
                j = m - i
                if j < 0:
                    continue
                if j not in bv:
                    bv[j] = ld1(W_OFF, g, kb, j)
                t = av[i] * bv[j]
                acc[m] = t if acc[m] is None else acc[m] + t
        if i0 + IG >= m0 + MG:
            for m in ms:
                if kind == "a":
                    uk_s[A_OFF + 8 * m:A_OFF + 8 * m + 8, :] = acc[m]
                elif kind == "c":
                    uk_s[R_OFF + 8 * m:R_OFF + 8 * m + 8, :] = acc[m]
                else:
                    re = uk_s[R_OFF + 8 * m:R_OFF + 8 * m + 8, :]
                    q_s[lt, m, g * 8:(g + 1) * 8, :] = pltpu.pack_elementwise(
                        [re, acc[m]], packed_dtype=BF)

    subs = []
    for g in range(NG):
        for kind in ("a", "c", "b"):
            for m0 in range(0, NB, MG):
                for i0 in range(0, m0 + MG, IG):
                    subs.append(functools.partial(sub, kind, g, m0, i0))
    return p_dft_k, p_kv, p_dft_u, subs


def _spread(subs, n, first, last, slabs=128):
    sched = [[] for _ in range(n)]
    npts = (last - first) * slabs
    for i, pc in enumerate(subs):
        pt = (i * npts) // len(subs)
        sched[first + pt // slabs].append((pt % slabs, pc))
    return sched


def _kernel(x_hbm, c_hbm, wq_hbm, wuk_hbm, wuv_hbm, wo_hbm, bk_hbm, bv_hbm, sk_hbm,
            shT_ref, dvec_ref, gw_ref, fwd_ref, inv_ref,
            out_hbm,
            x_v, wo_v, qT_s, k_s, vT_s, kv_s, q_s, sems, osems):
    qscale = (D ** -0.5) * math.log2(math.e)

    def phase1(c_v, wq_v, wuk_v, wuv_v, bk_v, bv_v, sk_v, skT_s, kpad_s, uk_s, dyn_s):
        dyn_s[0] = DUMMY
        dyn_s[1] = S + 8
        wuk_hbm32 = wuk_hbm.bitcast(U32)
        cp_wuk = [pltpu.make_async_copy(
            wuk_hbm32.at[:, pl.ds(4 * a, 4), :], wuk_v.at[a, :, pl.ds(0, 4), :], sems.at[9 + a])
            for a in range(4)]
        cp_c = [pltpu.make_async_copy(c_hbm.at[pl.ds(0, C0)], c_v.at[pl.ds(0, C0)], sems.at[0]),
                pltpu.make_async_copy(c_hbm.at[pl.ds(C0, S - C0)], c_v.at[pl.ds(C0, S - C0)],
                                      sems.at[1])]
        cp_wuv = pltpu.make_async_copy(wuv_hbm, wuv_v, sems.at[2])
        cp_x = pltpu.make_async_copy(x_hbm, x_v, sems.at[3])
        cp_wq = pltpu.make_async_copy(wq_hbm, wq_v, sems.at[4])
        cp_sk = pltpu.make_async_copy(sk_hbm, sk_v, sems.at[5])
        cp_bk = [pltpu.make_async_copy(bk_hbm.at[:, pl.ds(lt * T, T)], bk_v.at[lt], sems.at[6])
                 for lt in range(NL)]
        cp_bv = [pltpu.make_async_copy(bv_hbm.at[:, pl.ds(lt * T, T)], bv_v.at[lt], sems.at[7])
                 for lt in range(NL)]
        cp_wo = pltpu.make_async_copy(wo_hbm, wo_v, sems.at[8])
        for cp in ([cp_wuk[0], cp_c[0], cp_c[1]] + cp_wuk[1:] + [cp_x, cp_wq, cp_sk] + cp_bk + cp_bv
                   + [cp_wuv, cp_wo]):
            cp.start()

        shT = shT_ref[...].astype(F32)
        for lt in range(NL):
            skT_s[lt] = jnp.concatenate(
                [shT[:, lt * T:(lt + 1) * T], jnp.zeros((4, T), F32)], axis=0)
        kpad_s[0:8, :] = jnp.zeros((8, T), F32)

        wq32 = wq_v.bitcast(U32)
        wuv32 = wuv_v.bitcast(U32)

        def load_pairs(w32, rows, it, transpose):
            view = w32.at[pl.ds(pl.multiple_of(it * 4, 4), rows * 16 - 12)]
            outs = []
            for g in range(4):
                w = view[pl.ds(g, rows, stride=16), :]
                if transpose:
                    w = w.T
                outs += list(_lo_hi(w))
            return jnp.concatenate(outs, axis=0 if transpose else 1).astype(BF)

        wuk2 = wuk_v.reshape(4 * C * 8, D)

        def k_body(it, carry):
            pltpu.make_async_copy(wuk_hbm32.at[:, pl.ds(0, 4), :], wuk_v.at[it, :, pl.ds(0, 4), :],
                                  sems.at[9 + it]).wait()
            view = wuk2.at[pl.ds(pl.multiple_of(it * C * 8, 8), C * 8)]
            ws = []
            for g in range(4):
                lo, hi = _lo_hi(view[pl.ds(g, C, stride=8), :])
                ws.append(jnp.concatenate([lo, hi], axis=1).astype(BF))

            def k_proj(r0, r1):
                for g in range(4):
                    k = jnp.dot(c_v[r0:r1, :], ws[g], preferred_element_type=F32)
                    for u in range(2):
                        k_s[it * 8 + 2 * g + u, r0 // 2:r1 // 2, :] = _tou(
                            k[:, u * D:(u + 1) * D].astype(BF))

            k_proj(0, C0)

            @pl.when(it == 0)
            def _():
                cp_c[1].wait()

            k_proj(C0, S)
            return carry

        with jax.named_scope("wait0"):
            cp_c[0].wait()
        with jax.named_scope("kproj"):
            jax.lax.fori_loop(0, 4, k_body, 0)
        def proj_conv_body(it, lt, w32, rows, src_v, dst_s, scale):
            p_dft_k, p_kv, p_dft_u, subs = _conv_pieces(
                lt, bk_v, bv_v, sk_v, skT_s, fwd_ref, kpad_s, kv_s, q_s, uk_s,
                pl.multiple_of(dyn_s[0], 8), pl.multiple_of(dyn_s[1], 8))
            p_dft_k(None)
            w = load_pairs(w32, rows, it, True)
            sched = _spread(subs, NB, FIRST, LAST)
            nkv = NB // KVCH
            for n in range(NB):
                src = src_v[n * T:(n + 1) * T, :]
                if n < SPLIT0:
                    o = jnp.concatenate(
                        [jax.lax.dot_general(w[p * 2 * D:(p + 1) * 2 * D], src, NT_DIMS,
                                             preferred_element_type=F32) for p in range(4)], axis=0)
                else:
                    o = jax.lax.dot_general(w, src, NT_DIMS, preferred_element_type=F32)
                if scale is not None:
                    o = o * scale
                for g in range(8):
                    dst_s[it * 8 + g, :, n * T:(n + 1) * T] = _tou(o[g * D:(g + 1) * D].astype(BF))
                if KV0 + 1 <= n <= KV0 + KVCH:
                    for i in range((n - KV0 - 1) * nkv, (n - KV0) * nkv):
                        p_dft_u(i)
                if KV0 <= n < KV0 + KVCH:
                    for k_ in range(nkv):
                        sl = (128 * k_) // nkv
                        p_kv((n - KV0) * nkv + k_, o[8 * sl:8 * sl + 8])
                for sl, pc in sched[n]:
                    pc(o[8 * sl:8 * sl + 8])

        def q_body(it, carry):
            proj_conv_body(it, it, wq32, M, x_v, qT_s, qscale)
            return carry

        def v_body(it, carry):
            proj_conv_body(it, 4 + it, wuv32, C, c_v, vT_s, None)
            return carry

        with jax.named_scope("wait1"):
            for cp in [cp_x, cp_wq, cp_sk] + cp_bk + cp_bv:
                cp.wait()
        with jax.named_scope("qproj"):
            jax.lax.fori_loop(0, 4, q_body, 0)
        with jax.named_scope("wait2"):
            cp_wuv.wait()
        with jax.named_scope("vproj"):
            jax.lax.fori_loop(0, 4, v_body, 0)
        with jax.named_scope("wait3"):
            cp_wo.wait()

    pl.run_scoped(
        phase1,
        pltpu.VMEM((S, C), BF),
        pltpu.VMEM((M * H, D), BF),
        pltpu.VMEM((4, C, 8, D), U32),
        pltpu.VMEM((C * H, D), BF),
        pltpu.VMEM((NL, S, T), BF),
        pltpu.VMEM((NL, S, T), BF),
        pltpu.VMEM((M, S), BF),
        pltpu.VMEM((NL, 8, T), F32),
        pltpu.VMEM((S + 16, T), F32),
        pltpu.VMEM((UK_ROWS, T), F32),
        pltpu.SMEM((2,), jnp.int32),
    )

    def phase23(ctx_s, out_v, spre_s):
        tiles = [(g, j, i) for j in range(NB) for g in range(ATT_G) for i in range(j + 1)]

        def qk_next(base, k):
            g, j, i = tiles[k]
            spre_s[k] = _qk_tile(base + g, j, i, k_s, qT_s)

        def att_body(it, carry):
            with jax.named_scope("att_it"):
                return att_body2(it, carry)

        def att_body2(it, carry):
            base = it * ATT_G
            nxt = jnp.minimum(base + ATT_G, H - ATT_G)
            sv = {k: spre_s[k] for k in range(SKEW)}
            states = {}
            for k, (g, j, i) in enumerate(tiles):
                if k + SKEW < len(tiles):
                    g2, j2, i2 = tiles[k + SKEW]
                    sv[k + SKEW] = _qk_tile(base + g2, j2, i2, k_s, qT_s)
                else:
                    qk_next(nxt, k + SKEW - len(tiles))
                _softmax_pv(base + g, j, i, sv.pop(k), states.setdefault((g, j), {}), vT_s, ctx_s)
            return carry

        with jax.named_scope("attn"):
            for k in range(SKEW):
                qk_next(0, k)
            jax.lax.fori_loop(0, H // ATT_G, att_body, 0)

        R = OUT_R
        gw = gw_ref[...].astype(F32).reshape(1, M)
        dv = dvec_ref[...].astype(F32).reshape(1, M)

        def out_copy(it):
            rows = pl.ds(pl.multiple_of(it * R, R), R)
            return pltpu.make_async_copy(out_v.at[rows], out_hbm.at[rows], osems.at[it])

        def out_body(it, carry):
            rows = pl.ds(pl.multiple_of(it * R, R), R)
            prow = pl.ds(pl.multiple_of(it * (R // 2), R // 2), R // 2)
            inv = inv_ref[...]
            ys = []
            for mm in range(R // T):
                m = it * (R // T) + mm
                qm = jnp.concatenate([_tobf(q_s[lt, m]) for lt in range(NL)], axis=1)
                ys.append(jnp.dot(inv, qm, preferred_element_type=F32))
            y = jnp.concatenate(ys, axis=0)
            ctx = jnp.concatenate([_tobf(ctx_s[h, :, rows]).T for h in range(H)], axis=1)
            a = jnp.dot(ctx, wo_v[...], preferred_element_type=F32)
            kv = jnp.concatenate([_tobf(kv_s[lt, prow, :]) for lt in range(NL)], axis=1).astype(F32)
            xr = x_v[rows, :].astype(F32)
            g = jax.nn.sigmoid(jnp.sum(xr * gw, axis=-1, keepdims=True))
            b = xr * (y + kv * dv)
            out_v[rows, :] = (g * a + (1.0 - g) * b).astype(BF)
            out_copy(it).start()
            return carry

        with jax.named_scope("oproj"):
            jax.lax.fori_loop(0, S // R, out_body, 0)
        with jax.named_scope("wait4"):
            for it in range(S // R):
                out_copy(it).wait()

    pl.run_scoped(
        phase23,
        pltpu.VMEM((H, D // 2, S), U32),
        pltpu.VMEM((S, M), BF),
        pltpu.VMEM((SKEW, T, T), F32),
    )


@jax.jit
def pallas_gated_mix__compressed_kv_cla__ssm_conv_h3__prompt_kernel(
    A_x, A_c_kv, A_w_q, A_w_uk, A_w_uv, A_w_o, B_q, B_k, B_v, B_shift_k, B_ssm_k, B_ssm_D, gate_w,
):
    fwd_np, inv_np = _dft_consts()
    fwd = jnp.asarray(fwd_np, dtype=BF)
    inv = jnp.asarray(inv_np, dtype=BF)
    any_spec = pl.BlockSpec(memory_space=pl.ANY)
    vmem_spec = pl.BlockSpec(memory_space=pltpu.VMEM)
    out = pl.pallas_call(
        _kernel,
        out_shape=jax.ShapeDtypeStruct((S, M), BF),
        in_specs=[any_spec] * 9 + [vmem_spec] * 5,
        out_specs=any_spec,
        scratch_shapes=[
            pltpu.VMEM((S, M), BF),
            pltpu.VMEM((H * D, M), BF),
            pltpu.VMEM((H, D // 2, S), U32),
            pltpu.VMEM((H, S // 2, D), U32),
            pltpu.VMEM((H, D // 2, S), U32),
            pltpu.VMEM((NL, S // 2, T), U32),
            pltpu.VMEM((NL, NB, T, T), U32),
            pltpu.SemaphoreType.DMA((13,)),
            pltpu.SemaphoreType.DMA((S // OUT_R,)),
        ],
        compiler_params=pltpu.CompilerParams(vmem_limit_bytes=120 * 1024 * 1024),
    )(
        A_x.reshape(S, M), A_c_kv.reshape(S, C),
        A_w_q.reshape(M * H, D), A_w_uk, A_w_uv.reshape(C * H, D),
        A_w_o.reshape(H * D, M),
        B_k.reshape(S, M), B_v.reshape(S, M), B_ssm_k,
        B_shift_k.T, B_ssm_D, gate_w, fwd, inv,
    )
    return out.reshape(1, S, M)
```

```python
import functools
import math

import jax
import jax.numpy as jnp
import numpy as np
import jax.experimental.pallas as pl
import jax.experimental.pallas.tpu as pltpu

BF = jnp.bfloat16
F32 = jnp.float32
U32 = jnp.uint32

S = 2048
M = 1024
C = 512
H = 32
D = 128
T = 128
NB = S // T
NL = M // T
NEG = -1e30
NT_DIMS = (((1,), (1,)), ((), ()))

ATT_G = 4
C0 = 512
SKEW = 8
OUT_R = 256


def _tobf(x):
    return pltpu.bitcast(x, BF)


def _tou(x):
    return pltpu.bitcast(x, U32)


def _lo_hi(w):
    lo = pltpu.bitcast(w << 16, F32)
    hi = pltpu.bitcast(w & jnp.uint32(0xFFFF0000), F32)
    return lo, hi


def _dft_consts():
    n_fft = 2 * T
    f = np.concatenate([np.arange(0, T, 2), np.arange(1, T, 2)]).astype(np.float64)
    theta = 2.0 * np.pi * (f + 0.5) / n_fft
    n = np.arange(T, dtype=np.float64)
    ang = theta[:, None] * n[None, :]
    re = np.cos(ang)
    im = -np.sin(ang)
    fwd = np.concatenate([re.reshape(T // 8, 8, T), im.reshape(T // 8, 8, T)], axis=1)
    fwd = fwd.reshape(2 * T, T)
    inv = np.stack([re, im], axis=1).reshape(2 * T, T).T * (2.0 / n_fft)
    return fwd.astype(np.float32), inv.astype(np.float32)


def _qk_tile(h, j, i, k_s, qT_s):
    qT = _tobf(qT_s[h, :, j * T:(j + 1) * T])
    kk = _tobf(k_s[h, i * T // 2:(i + 1) * T // 2, :])
    return jnp.dot(kk, qT, preferred_element_type=F32)


def _softmax_pv(h, j, i, s, st, vT_s, ctx_s):
    if i == j:
        ki = jax.lax.broadcasted_iota(jnp.int32, (T, T), 0)
        qi = jax.lax.broadcasted_iota(jnp.int32, (T, T), 1)
        s = jnp.where(ki <= qi, s, NEG)
    mc = jnp.max(s, axis=0, keepdims=True)
    m_new = mc if i == 0 else jnp.maximum(st["m"], mc)
    p = jnp.exp2(s - m_new)
    lc = jnp.sum(p.reshape(T // 8, 8, T), axis=0)
    pv = jnp.dot(_tobf(vT_s[h, :, i * T:(i + 1) * T]), p.astype(BF), preferred_element_type=F32)
    if i == 0:
        acc, l = pv, lc
    else:
        alpha = jnp.exp2(st["m"] - m_new)
        l = alpha * st["l"] + lc
        acc = alpha * st["acc"] + pv
    st.update(m=m_new, l=l, acc=acc)
    if i == j:
        lsum = jnp.sum(l, axis=0, keepdims=True)
        o = acc * (1.0 / lsum)
        ctx_s[h, :, j * T:(j + 1) * T] = _tou(o.astype(BF))


MG = 8
IG = 4
SPLIT0 = 1
KV0 = 1
KVCH = 2
FIRST = 4
LAST = 15
NG = T // 8
U_OFF = 0
W_OFF = U_OFF + NB * NG * 24
A_OFF = W_OFF + NB * NG * 24
R_OFF = A_OFF + NB * 8
DUMMY = R_OFF + NB * 8
UK_ROWS = DUMMY + 8


def _conv_pieces(lt, bk_v, bv_v, sk_v, skT_s, fwd_ref, kpad_s, kv_s, q_s, uk_s, dyn, dyn2):
    st = {}

    def p_kv(i, val):
        if val is not None:
            kpad_s[pl.ds(dyn2, 8), :] = val
        r0 = i * T
        kf = bk_v[lt, r0:r0 + T, :].astype(F32)
        kpad_s[8 + r0:8 + r0 + T, :] = kf
        sk = skT_s[lt]
        ksh = kf * sk[0:1, :]
        for j in range(1, 4):
            ksh = ksh + kpad_s[8 + r0 - j:8 + r0 - j + T, :] * sk[j:j + 1, :]
        kv = (ksh * bv_v[lt, r0:r0 + T, :].astype(F32)).astype(BF)
        kv_s[lt, r0 // 2:(r0 + T) // 2, :] = _tou(kv)
        st["kv", i] = kv

    def p_dft_k(_):
        fwd = fwd_ref[...]
        ssm = sk_v[pl.ds(pl.multiple_of(lt * T, T), T), :]
        prev = None
        for d in range(NB):
            k = jax.lax.dot_general(fwd, ssm[:, d * T:(d + 1) * T], NT_DIMS,
                                    preferred_element_type=F32)
            for g in range(NG):
                kr, ki = k[16 * g:16 * g + 8], k[16 * g + 8:16 * g + 16]
                if prev is None:
                    wr, wi = kr, ki
                else:
                    pr, pi = prev[16 * g:16 * g + 8], prev[16 * g + 8:16 * g + 16]
                    if g < NG // 2:
                        wr, wi = kr - pi, ki + pr
                    else:
                        wr, wi = kr + pi, ki - pr
                r = W_OFF + (g * NB + d) * 24
                uk_s[r:r + 8, :] = wr
                uk_s[r + 8:r + 16, :] = wi - wr
                uk_s[r + 16:r + 24, :] = -(wr + wi)
            prev = k

    def p_dft_u(i):
        fwd = fwd_ref[...]
        u = jnp.dot(fwd, st["kv", i], preferred_element_type=F32)
        for g in range(NG):
            ur, ui = u[16 * g:16 * g + 8], u[16 * g + 8:16 * g + 16]
            r = U_OFF + (g * NB + i) * 24
            uk_s[r:r + 8, :] = ur
            uk_s[r + 8:r + 16, :] = ui
            uk_s[r + 16:r + 24, :] = ur + ui

    def gate(val):
        if val is not None:
            uk_s[pl.ds(dyn, 8), :] = val

    def ld1(off, g, k, i):
        r = off + (g * NB + i) * 24 + 8 * k
        return uk_s[r:r + 8, :]

    def sub(kind, g, m0, i0, val):
        gate(val)
        ka, kb = {"a": (2, 0), "c": (1, 2), "b": (0, 1)}[kind]
        ms = range(m0, m0 + MG)
        if i0 == 0:
            if kind == "a":
                st["acc"] = {m: None for m in ms}
            else:
                st["acc"] = {m: uk_s[A_OFF + 8 * m:A_OFF + 8 * m + 8, :] for m in ms}
        acc = st["acc"]
        av = {i: ld1(U_OFF, g, ka, i) for i in range(i0, min(i0 + IG, m0 + MG))}
        bv = {}
        for i in av:
            for m in ms:
                j = m - i
                if j < 0:
                    continue
                if j not in bv:
                    bv[j] = ld1(W_OFF, g, kb, j)
                t = av[i] * bv[j]
                acc[m] = t if acc[m] is None else acc[m] + t
        if i0 + IG >= m0 + MG:
            for m in ms:
                if kind == "a":
                    uk_s[A_OFF + 8 * m:A_OFF + 8 * m + 8, :] = acc[m]
                elif kind == "c":
                    uk_s[R_OFF + 8 * m:R_OFF + 8 * m + 8, :] = acc[m]
                else:
                    re = uk_s[R_OFF + 8 * m:R_OFF + 8 * m + 8, :]
                    q_s[lt, m, g * 8:(g + 1) * 8, :] = pltpu.pack_elementwise(
                        [re, acc[m]], packed_dtype=BF)

    subs = []
    for g in range(NG):
        for kind in ("a", "c", "b"):
            for m0 in range(0, NB, MG):
                for i0 in range(0, m0 + MG, IG):
                    subs.append(functools.partial(sub, kind, g, m0, i0))
    return p_dft_k, p_kv, p_dft_u, subs


def _spread(subs, n, first, last, slabs=128):
    sched = [[] for _ in range(n)]
    npts = (last - first) * slabs
    for i, pc in enumerate(subs):
        pt = (i * npts) // len(subs)
        sched[first + pt // slabs].append((pt % slabs, pc))
    return sched


def _kernel(x_hbm, c_hbm, wq_hbm, wuk_hbm, wuv_hbm, wo_hbm, bk_hbm, bv_hbm, sk_hbm,
            shT_hbm, dvec_hbm, gw_hbm, fwd_hbm, inv_hbm,
            out_hbm,
            x_v, wo_v, qT_s, k_s, vT_s, kv_s, q_s,
            shT_ref, dvec_ref, gw_ref, fwd_ref, inv_ref, sems, osems):
    qscale = (D ** -0.5) * math.log2(math.e)

    def phase1(c_v, wq_v, wuk_v, wuv_v, bk_v, bv_v, sk_v, skT_s, kpad_s, uk_s, dyn_s):
        dyn_s[0] = DUMMY
        dyn_s[1] = S + 8
        wuk_hbm32 = wuk_hbm.bitcast(U32)
        cp_wuk = [pltpu.make_async_copy(
            wuk_hbm32.at[:, pl.ds(4 * a, 4), :], wuk_v.at[a, :, pl.ds(0, 4), :], sems.at[9 + a])
            for a in range(4)]
        cp_c = [pltpu.make_async_copy(c_hbm.at[pl.ds(0, C0)], c_v.at[pl.ds(0, C0)], sems.at[0]),
                pltpu.make_async_copy(c_hbm.at[pl.ds(C0, S - C0)], c_v.at[pl.ds(C0, S - C0)],
                                      sems.at[1])]
        cp_wuv = pltpu.make_async_copy(wuv_hbm, wuv_v, sems.at[2])
        cp_x = pltpu.make_async_copy(x_hbm, x_v, sems.at[3])
        cp_wq = pltpu.make_async_copy(wq_hbm, wq_v, sems.at[4])
        cp_sk = pltpu.make_async_copy(sk_hbm, sk_v, sems.at[5])
        cp_bk = [pltpu.make_async_copy(bk_hbm.at[:, pl.ds(lt * T, T)], bk_v.at[lt], sems.at[6])
                 for lt in range(NL)]
        cp_bv = [pltpu.make_async_copy(bv_hbm.at[:, pl.ds(lt * T, T)], bv_v.at[lt], sems.at[7])
                 for lt in range(NL)]
        cp_wo = pltpu.make_async_copy(wo_hbm, wo_v, sems.at[8])
        cp_small = [pltpu.make_async_copy(a, b, sems.at[13]) for a, b in
                    [(shT_hbm, shT_ref), (dvec_hbm, dvec_ref), (gw_hbm, gw_ref),
                     (fwd_hbm, fwd_ref), (inv_hbm, inv_ref)]]
        for cp in ([cp_wuk[0], cp_c[0], cp_c[1]] + cp_wuk[1:] + cp_small + [cp_x, cp_wq, cp_sk]
                   + cp_bk + cp_bv + [cp_wuv, cp_wo]):
            cp.start()

        wq32 = wq_v.bitcast(U32)
        wuv32 = wuv_v.bitcast(U32)

        def load_pairs(w32, rows, it, transpose):
            view = w32.at[pl.ds(pl.multiple_of(it * 4, 4), rows * 16 - 12)]
            outs = []
            for g in range(4):
                w = view[pl.ds(g, rows, stride=16), :]
                if transpose:
                    w = w.T
                outs += list(_lo_hi(w))
            return jnp.concatenate(outs, axis=0 if transpose else 1).astype(BF)

        wuk2 = wuk_v.reshape(4 * C * 8, D)

        def k_body(it, carry):
            with jax.named_scope("k_it"):
                return k_body2(it, carry)

        def k_body2(it, carry):
            pltpu.make_async_copy(wuk_hbm32.at[:, pl.ds(pl.multiple_of(4 * it, 4), 4), :],
                                  wuk_v.at[it, :, pl.ds(0, 4), :], sems.at[9 + it]).wait()
            view = wuk2.at[pl.ds(pl.multiple_of(it * C * 8, 8), C * 8)]
            ws = []
            for g in range(4):
                lo, hi = _lo_hi(view[pl.ds(g, C, stride=8), :])
                ws.append(jnp.concatenate([lo, hi], axis=1).astype(BF))

            def k_proj(r0, r1):
                for g in range(4):
                    k = jnp.dot(c_v[r0:r1, :], ws[g], preferred_element_type=F32)
                    for u in range(2):
                        k_s[it * 8 + 2 * g + u, r0 // 2:r1 // 2, :] = _tou(
                            k[:, u * D:(u + 1) * D].astype(BF))

            k_proj(0, C0)

            @pl.when(it == 0)
            def _():
                cp_c[1].wait()

            k_proj(C0, S)
            return carry

        with jax.named_scope("wait0"):
            cp_c[0].wait()
        with jax.named_scope("kproj"):
            jax.lax.fori_loop(0, 4, k_body, 0)
        def proj_conv_body(it, lt, w32, rows, src_v, dst_s, scale):
            p_dft_k, p_kv, p_dft_u, subs = _conv_pieces(
                lt, bk_v, bv_v, sk_v, skT_s, fwd_ref, kpad_s, kv_s, q_s, uk_s,
                pl.multiple_of(dyn_s[0], 8), pl.multiple_of(dyn_s[1], 8))
            p_dft_k(None)
            w = load_pairs(w32, rows, it, True)
            sched = _spread(subs, NB, FIRST, LAST)
            nkv = NB // KVCH
            for n in range(NB):
                src = src_v[n * T:(n + 1) * T, :]
                if n < SPLIT0:
                    o = jnp.concatenate(
                        [jax.lax.dot_general(w[p * 2 * D:(p + 1) * 2 * D], src, NT_DIMS,
                                             preferred_element_type=F32) for p in range(4)], axis=0)
                else:
                    o = jax.lax.dot_general(w, src, NT_DIMS, preferred_element_type=F32)
                if scale is not None:
                    o = o * scale
                for g in range(8):
                    dst_s[it * 8 + g, :, n * T:(n + 1) * T] = _tou(o[g * D:(g + 1) * D].astype(BF))
                if KV0 + 1 <= n <= KV0 + KVCH:
                    for i in range((n - KV0 - 1) * nkv, (n - KV0) * nkv):
                        p_dft_u(i)
                if KV0 <= n < KV0 + KVCH:
                    for k_ in range(nkv):
                        sl = (128 * k_) // nkv
                        p_kv((n - KV0) * nkv + k_, o[8 * sl:8 * sl + 8])
                for sl, pc in sched[n]:
                    pc(o[8 * sl:8 * sl + 8])

        def q_body(it, carry):
            with jax.named_scope("q_it"):
                proj_conv_body(it, it, wq32, M, x_v, qT_s, qscale)
            return carry

        def v_body(it, carry):
            with jax.named_scope("v_it"):
                proj_conv_body(it, 4 + it, wuv32, C, c_v, vT_s, None)
            return carry

        with jax.named_scope("wait1"):
            for cp in cp_small + [cp_x, cp_wq, cp_sk] + cp_bk + cp_bv:
                cp.wait()
        shT = shT_ref[...].astype(F32)
        for lt in range(NL):
            skT_s[lt] = jnp.concatenate(
                [shT[:, lt * T:(lt + 1) * T], jnp.zeros((4, T), F32)], axis=0)
        kpad_s[0:8, :] = jnp.zeros((8, T), F32)

        with jax.named_scope("qproj"):
            jax.lax.fori_loop(0, 4, q_body, 0)
        with jax.named_scope("wait2"):
            cp_wuv.wait()
        with jax.named_scope("vproj"):
            jax.lax.fori_loop(0, 4, v_body, 0)
        with jax.named_scope("wait3"):
            cp_wo.wait()

    pl.run_scoped(
        phase1,
        pltpu.VMEM((S, C), BF),
        pltpu.VMEM((M * H, D), BF),
        pltpu.VMEM((4, C, 8, D), U32),
        pltpu.VMEM((C * H, D), BF),
        pltpu.VMEM((NL, S, T), BF),
        pltpu.VMEM((NL, S, T), BF),
        pltpu.VMEM((M, S), BF),
        pltpu.VMEM((NL, 8, T), F32),
        pltpu.VMEM((S + 16, T), F32),
        pltpu.VMEM((UK_ROWS, T), F32),
        pltpu.SMEM((2,), jnp.int32),
    )

    def phase23(ctx_s, out_v, spre_s):
        tiles = [(g, j, i) for j in range(NB) for g in range(ATT_G) for i in range(j + 1)]

        def qk_next(base, k):
            g, j, i = tiles[k]
            spre_s[k] = _qk_tile(base + g, j, i, k_s, qT_s)

        def att_body(it, carry):
            with jax.named_scope("att_it"):
                return att_body2(it, carry)

        def att_body2(it, carry):
            base = it * ATT_G
            nxt = jnp.minimum(base + ATT_G, H - ATT_G)
            sv = {k: spre_s[k] for k in range(SKEW)}
            states = {}
            for k, (g, j, i) in enumerate(tiles):
                if k + SKEW < len(tiles):
                    g2, j2, i2 = tiles[k + SKEW]
                    sv[k + SKEW] = _qk_tile(base + g2, j2, i2, k_s, qT_s)
                else:
                    qk_next(nxt, k + SKEW - len(tiles))
                _softmax_pv(base + g, j, i, sv.pop(k), states.setdefault((g, j), {}), vT_s, ctx_s)
            return carry

        with jax.named_scope("attn"):
            for k in range(SKEW):
                qk_next(0, k)
            jax.lax.fori_loop(0, H // ATT_G, att_body, 0)

        R = OUT_R
        gw = gw_ref[...].astype(F32).reshape(1, M)
        dv = dvec_ref[...].astype(F32).reshape(1, M)

        def out_copy(it):
            rows = pl.ds(pl.multiple_of(it * R, R), R)
            return pltpu.make_async_copy(out_v.at[rows], out_hbm.at[rows], osems.at[it])

        def out_body(it, carry):
            with jax.named_scope("o_it"):
                return out_body2(it, carry)

        def out_body2(it, carry):
            rows = pl.ds(pl.multiple_of(it * R, R), R)
            prow = pl.ds(pl.multiple_of(it * (R // 2), R // 2), R // 2)
            inv = inv_ref[...]
            ys = []
            for mm in range(R // T):
                m = it * (R // T) + mm
                qm = jnp.concatenate([_tobf(q_s[lt, m]) for lt in range(NL)], axis=1)
                ys.append(jnp.dot(inv, qm, preferred_element_type=F32))
            y = jnp.concatenate(ys, axis=0)
            ctx = jnp.concatenate([_tobf(ctx_s[h, :, rows]).T for h in range(H)], axis=1)
            a = jnp.dot(ctx, wo_v[...], preferred_element_type=F32)
            kv = jnp.concatenate([_tobf(kv_s[lt, prow, :]) for lt in range(NL)], axis=1).astype(F32)
            xr = x_v[rows, :].astype(F32)
            g = jax.nn.sigmoid(jnp.sum(xr * gw, axis=-1, keepdims=True))
            b = xr * (y + kv * dv)
            out_v[rows, :] = (g * a + (1.0 - g) * b).astype(BF)
            out_copy(it).start()
            return carry

        with jax.named_scope("oproj"):
            jax.lax.fori_loop(0, S // R, out_body, 0)
        with jax.named_scope("wait4"):
            for it in range(S // R):
                out_copy(it).wait()

    pl.run_scoped(
        phase23,
        pltpu.VMEM((H, D // 2, S), U32),
        pltpu.VMEM((S, M), BF),
        pltpu.VMEM((SKEW, T, T), F32),
    )


@jax.jit
def pallas_gated_mix__compressed_kv_cla__ssm_conv_h3__prompt_kernel(
    A_x, A_c_kv, A_w_q, A_w_uk, A_w_uv, A_w_o, B_q, B_k, B_v, B_shift_k, B_ssm_k, B_ssm_D, gate_w,
):
    fwd_np, inv_np = _dft_consts()
    fwd = jnp.asarray(fwd_np.astype(BF))
    inv = jnp.asarray(inv_np.astype(BF))
    any_spec = pl.BlockSpec(memory_space=pl.ANY)
    out = pl.pallas_call(
        _kernel,
        out_shape=jax.ShapeDtypeStruct((S, M), BF),
        in_specs=[any_spec] * 14,
        out_specs=any_spec,
        scratch_shapes=[
            pltpu.VMEM((S, M), BF),
            pltpu.VMEM((H * D, M), BF),
            pltpu.VMEM((H, D // 2, S), U32),
            pltpu.VMEM((H, S // 2, D), U32),
            pltpu.VMEM((H, D // 2, S), U32),
            pltpu.VMEM((NL, S // 2, T), U32),
            pltpu.VMEM((NL, NB, T, T), U32),
            pltpu.VMEM((4, M), BF),
            pltpu.VMEM((M,), BF),
            pltpu.VMEM((M,), BF),
            pltpu.VMEM((2 * T, T), BF),
            pltpu.VMEM((T, 2 * T), BF),
            pltpu.SemaphoreType.DMA((14,)),
            pltpu.SemaphoreType.DMA((S // OUT_R,)),
        ],
        compiler_params=pltpu.CompilerParams(vmem_limit_bytes=120 * 1024 * 1024),
    )(
        A_x.reshape(S, M), A_c_kv.reshape(S, C),
        A_w_q.reshape(M * H, D), A_w_uk, A_w_uv.reshape(C * H, D),
        A_w_o.reshape(H * D, M),
        B_k.reshape(S, M), B_v.reshape(S, M), B_ssm_k,
        B_shift_k.T, B_ssm_D, gate_w, fwd, inv,
    )
    return out.reshape(1, S, M)
```

```python
import functools
import math

import jax
import jax.numpy as jnp
import numpy as np
import jax.experimental.pallas as pl
import jax.experimental.pallas.tpu as pltpu

BF = jnp.bfloat16
F32 = jnp.float32
U32 = jnp.uint32

S = 2048
M = 1024
C = 512
H = 32
D = 128
T = 128
NB = S // T
NL = M // T
NEG = -1e30
NT_DIMS = (((1,), (1,)), ((), ()))

ATT_G = 4
C_CHUNKS = [(0, 128), (128, 512), (512, 2048)]
SKEW = 8
OUNROLL = 1
OCOL = 128
OUT_R = 256


def _tobf(x):
    return pltpu.bitcast(x, BF)


def _tou(x):
    return pltpu.bitcast(x, U32)


def _lo_hi(w):
    lo = pltpu.bitcast(w << 16, F32)
    hi = pltpu.bitcast(w & jnp.uint32(0xFFFF0000), F32)
    return lo, hi


def _dft_consts():
    n_fft = 2 * T
    f = np.concatenate([np.arange(0, T, 2), np.arange(1, T, 2)]).astype(np.float64)
    theta = 2.0 * np.pi * (f + 0.5) / n_fft
    n = np.arange(T, dtype=np.float64)
    ang = theta[:, None] * n[None, :]
    re = np.cos(ang)
    im = -np.sin(ang)
    fwd = np.concatenate([re.reshape(T // 8, 8, T), im.reshape(T // 8, 8, T)], axis=1)
    fwd = fwd.reshape(2 * T, T)
    inv = np.stack([re, im], axis=1).reshape(2 * T, T).T * (2.0 / n_fft)
    return fwd.astype(np.float32), inv.astype(np.float32)


def _qk_tile(h, j, i, k_s, qT_s):
    qT = _tobf(qT_s[h, :, j * T:(j + 1) * T])
    kk = _tobf(k_s[h, i * T // 2:(i + 1) * T // 2, :])
    return jnp.dot(kk, qT, preferred_element_type=F32)


def _softmax_pv(h, j, i, s, st, vT_s, ctx_s):
    if i == j:
        ki = jax.lax.broadcasted_iota(jnp.int32, (T, T), 0)
        qi = jax.lax.broadcasted_iota(jnp.int32, (T, T), 1)
        s = jnp.where(ki <= qi, s, NEG)
    mc = jnp.max(s, axis=0, keepdims=True)
    m_new = mc if i == 0 else jnp.maximum(st["m"], mc)
    p = jnp.exp2(s - m_new)
    lc = jnp.sum(p.reshape(T // 8, 8, T), axis=0)
    pv = jnp.dot(_tobf(vT_s[h, :, i * T:(i + 1) * T]), p.astype(BF), preferred_element_type=F32)
    if i == 0:
        acc, l = pv, lc
    else:
        alpha = jnp.exp2(st["m"] - m_new)
        l = alpha * st["l"] + lc
        acc = alpha * st["acc"] + pv
    st.update(m=m_new, l=l, acc=acc)
    if i == j:
        lsum = jnp.sum(l, axis=0, keepdims=True)
        o = acc * (1.0 / lsum)
        ctx_s[h, :, j * T:(j + 1) * T] = _tou(o.astype(BF))


MG = 8
IG = 4
SPLIT0 = 1
KV0 = 1
KVCH = 2
FIRST = 4
LAST = 15
NG = T // 8
U_OFF = 0
W_OFF = U_OFF + NB * NG * 24
A_OFF = W_OFF + NB * NG * 24
R_OFF = A_OFF + NB * 8
DUMMY = R_OFF + NB * 8
UK_ROWS = DUMMY + 8


def _conv_pieces(lt, bk_v, bv_v, sk_v, skT_s, fwd_ref, kpad_s, kv_s, q_s, uk_s, dyn, dyn2):
    st = {}

    def p_kv(i, val):
        if val is not None:
            kpad_s[pl.ds(dyn2, 8), :] = val
        r0 = i * T
        kf = bk_v[lt, r0:r0 + T, :].astype(F32)
        kpad_s[8 + r0:8 + r0 + T, :] = kf
        sk = skT_s[lt]
        ksh = kf * sk[0:1, :]
        for j in range(1, 4):
            ksh = ksh + kpad_s[8 + r0 - j:8 + r0 - j + T, :] * sk[j:j + 1, :]
        kv = (ksh * bv_v[lt, r0:r0 + T, :].astype(F32)).astype(BF)
        kv_s[lt, r0 // 2:(r0 + T) // 2, :] = _tou(kv)
        st["kv", i] = kv

    def p_dft_k(_):
        fwd = fwd_ref[...]
        ssm = sk_v[pl.ds(pl.multiple_of(lt * T, T), T), :]
        prev = None
        for d in range(NB):
            k = jax.lax.dot_general(fwd, ssm[:, d * T:(d + 1) * T], NT_DIMS,
                                    preferred_element_type=F32)
            for g in range(NG):
                kr, ki = k[16 * g:16 * g + 8], k[16 * g + 8:16 * g + 16]
                if prev is None:
                    wr, wi = kr, ki
                else:
                    pr, pi = prev[16 * g:16 * g + 8], prev[16 * g + 8:16 * g + 16]
                    if g < NG // 2:
                        wr, wi = kr - pi, ki + pr
                    else:
                        wr, wi = kr + pi, ki - pr
                r = W_OFF + (g * NB + d) * 24
                uk_s[r:r + 8, :] = wr
                uk_s[r + 8:r + 16, :] = wi - wr
                uk_s[r + 16:r + 24, :] = -(wr + wi)
            prev = k

    def p_dft_u(i):
        fwd = fwd_ref[...]
        u = jnp.dot(fwd, st["kv", i], preferred_element_type=F32)
        for g in range(NG):
            ur, ui = u[16 * g:16 * g + 8], u[16 * g + 8:16 * g + 16]
            r = U_OFF + (g * NB + i) * 24
            uk_s[r:r + 8, :] = ur
            uk_s[r + 8:r + 16, :] = ui
            uk_s[r + 16:r + 24, :] = ur + ui

    def gate(val):
        if val is not None:
            uk_s[pl.ds(dyn, 8), :] = val

    def ld1(off, g, k, i):
        r = off + (g * NB + i) * 24 + 8 * k
        return uk_s[r:r + 8, :]

    def sub(kind, g, m0, i0, val):
        gate(val)
        ka, kb = {"a": (2, 0), "c": (1, 2), "b": (0, 1)}[kind]
        ms = range(m0, m0 + MG)
        if i0 == 0:
            if kind == "a":
                st["acc"] = {m: None for m in ms}
            else:
                st["acc"] = {m: uk_s[A_OFF + 8 * m:A_OFF + 8 * m + 8, :] for m in ms}
        acc = st["acc"]
        av = {i: ld1(U_OFF, g, ka, i) for i in range(i0, min(i0 + IG, m0 + MG))}
        bv = {}
        for i in av:
            for m in ms:
                j = m - i
                if j < 0:
                    continue
                if j not in bv:
                    bv[j] = ld1(W_OFF, g, kb, j)
                t = av[i] * bv[j]
                acc[m] = t if acc[m] is None else acc[m] + t
        if i0 + IG >= m0 + MG:
            for m in ms:
                if kind == "a":
                    uk_s[A_OFF + 8 * m:A_OFF + 8 * m + 8, :] = acc[m]
                elif kind == "c":
                    uk_s[R_OFF + 8 * m:R_OFF + 8 * m + 8, :] = acc[m]
                else:
                    re = uk_s[R_OFF + 8 * m:R_OFF + 8 * m + 8, :]
                    q_s[lt, m, g * 8:(g + 1) * 8, :] = pltpu.pack_elementwise(
                        [re, acc[m]], packed_dtype=BF)

    subs = []
    for g in range(NG):
        for kind in ("a", "c", "b"):
            for m0 in range(0, NB, MG):
                for i0 in range(0, m0 + MG, IG):
                    subs.append(functools.partial(sub, kind, g, m0, i0))
    return p_dft_k, p_kv, p_dft_u, subs


def _spread(subs, n, first, last, slabs=128):
    sched = [[] for _ in range(n)]
    npts = (last - first) * slabs
    for i, pc in enumerate(subs):
        pt = (i * npts) // len(subs)
        sched[first + pt // slabs].append((pt % slabs, pc))
    return sched


def _kernel(x_hbm, c_hbm, wq_hbm, wuk_hbm, wuv_hbm, wo_hbm, bk_hbm, bv_hbm, sk_hbm,
            shT_hbm, dvec_hbm, gw_hbm, fwd_hbm, inv_hbm,
            out_hbm,
            x_v, wo_v, qT_s, k_s, vT_s, kv_s, q_s,
            shT_ref, dvec_ref, gw_ref, fwd_ref, inv_ref, sems, osems):
    qscale = (D ** -0.5) * math.log2(math.e)

    def phase1(c_v, wq_v, wuk_v, wuv_v, bk_v, bv_v, sk_v, skT_s, kpad_s, uk_s, dyn_s):
        dyn_s[0] = DUMMY
        dyn_s[1] = S + 8
        wuk_hbm32 = wuk_hbm.bitcast(U32)
        cp_wuk = [pltpu.make_async_copy(
            wuk_hbm32.at[:, pl.ds(4 * a, 4), :], wuk_v.at[a, :, pl.ds(0, 4), :], sems.at[9 + a])
            for a in range(4)]
        cp_c = [pltpu.make_async_copy(c_hbm.at[pl.ds(r0, r1 - r0)], c_v.at[pl.ds(r0, r1 - r0)],
                                      sems.at[14 + i]) for i, (r0, r1) in enumerate(C_CHUNKS)]
        cp_wuv = pltpu.make_async_copy(wuv_hbm, wuv_v, sems.at[2])
        cp_x = pltpu.make_async_copy(x_hbm, x_v, sems.at[3])
        cp_wq = pltpu.make_async_copy(wq_hbm, wq_v, sems.at[4])
        cp_sk = pltpu.make_async_copy(sk_hbm, sk_v, sems.at[5])
        cp_bk = [pltpu.make_async_copy(bk_hbm.at[:, pl.ds(lt * T, T)], bk_v.at[lt], sems.at[6])
                 for lt in range(NL)]
        cp_bv = [pltpu.make_async_copy(bv_hbm.at[:, pl.ds(lt * T, T)], bv_v.at[lt], sems.at[7])
                 for lt in range(NL)]
        cp_wo = pltpu.make_async_copy(wo_hbm, wo_v, sems.at[8])
        cp_small = [pltpu.make_async_copy(a, b, sems.at[13]) for a, b in
                    [(shT_hbm, shT_ref), (dvec_hbm, dvec_ref), (gw_hbm, gw_ref),
                     (fwd_hbm, fwd_ref), (inv_hbm, inv_ref)]]
        for cp in ([cp_wuk[0]] + cp_c + cp_wuk[1:] + cp_small + [cp_x, cp_wq, cp_sk]
                   + cp_bk + cp_bv + [cp_wuv, cp_wo]):
            cp.start()

        wq32 = wq_v.bitcast(U32)
        wuv32 = wuv_v.bitcast(U32)

        def load_pairs(w32, rows, it, transpose):
            view = w32.at[pl.ds(pl.multiple_of(it * 4, 4), rows * 16 - 12)]
            outs = []
            for g in range(4):
                w = view[pl.ds(g, rows, stride=16), :]
                if transpose:
                    w = w.T
                outs += list(_lo_hi(w))
            return jnp.concatenate(outs, axis=0 if transpose else 1).astype(BF)

        wuk2 = wuk_v.reshape(4 * C * 8, D)

        def k_group(it, first):
            pltpu.make_async_copy(wuk_hbm32.at[:, pl.ds(pl.multiple_of(4 * it, 4), 4), :],
                                  wuk_v.at[it, :, pl.ds(0, 4), :], sems.at[9 + it]).wait()
            view = wuk2.at[pl.ds(pl.multiple_of(it * C * 8, 8), C * 8)]
            ws = []
            for g in range(4):
                lo, hi = _lo_hi(view[pl.ds(g, C, stride=8), :])
                ws.append(jnp.concatenate([lo, hi], axis=1).astype(BF))
            for i, (r0, r1) in enumerate(C_CHUNKS if first else [(0, S)]):
                if first:
                    cp_c[i].wait()
                for g in range(4):
                    k = jnp.dot(c_v[r0:r1, :], ws[g], preferred_element_type=F32)
                    for u in range(2):
                        k_s[it * 8 + 2 * g + u, r0 // 2:r1 // 2, :] = _tou(
                            k[:, u * D:(u + 1) * D].astype(BF))

        def k_body(it, carry):
            with jax.named_scope("k_it"):
                k_group(it, False)
            return carry

        with jax.named_scope("kproj0"):
            k_group(0, True)
        with jax.named_scope("kproj"):
            jax.lax.fori_loop(1, 4, k_body, 0)

        def proj_conv_body(it, lt, w32, rows, src_v, dst_s, scale):
            p_dft_k, p_kv, p_dft_u, subs = _conv_pieces(
                lt, bk_v, bv_v, sk_v, skT_s, fwd_ref, kpad_s, kv_s, q_s, uk_s,
                pl.multiple_of(dyn_s[0], 8), pl.multiple_of(dyn_s[1], 8))
            p_dft_k(None)
            w = load_pairs(w32, rows, it, True)
            sched = _spread(subs, NB, FIRST, LAST)
            nkv = NB // KVCH
            for n in range(NB):
                src = src_v[n * T:(n + 1) * T, :]
                if n < SPLIT0:
                    o = jnp.concatenate(
                        [jax.lax.dot_general(w[p * 2 * D:(p + 1) * 2 * D], src, NT_DIMS,
                                             preferred_element_type=F32) for p in range(4)], axis=0)
                else:
                    o = jax.lax.dot_general(w, src, NT_DIMS, preferred_element_type=F32)
                if scale is not None:
                    o = o * scale
                for g in range(8):
                    dst_s[it * 8 + g, :, n * T:(n + 1) * T] = _tou(o[g * D:(g + 1) * D].astype(BF))
                if KV0 + 1 <= n <= KV0 + KVCH:
                    for i in range((n - KV0 - 1) * nkv, (n - KV0) * nkv):
                        p_dft_u(i)
                if KV0 <= n < KV0 + KVCH:
                    for k_ in range(nkv):
                        sl = (128 * k_) // nkv
                        p_kv((n - KV0) * nkv + k_, o[8 * sl:8 * sl + 8])
                for sl, pc in sched[n]:
                    pc(o[8 * sl:8 * sl + 8])

        def q_body(it, carry):
            with jax.named_scope("q_it"):
                proj_conv_body(it, it, wq32, M, x_v, qT_s, qscale)
            return carry

        def v_body(it, carry):
            with jax.named_scope("v_it"):
                proj_conv_body(it, 4 + it, wuv32, C, c_v, vT_s, None)
            return carry

        with jax.named_scope("wait1"):
            for cp in cp_small + [cp_x, cp_wq, cp_sk] + cp_bk + cp_bv:
                cp.wait()
        shT = shT_ref[...].astype(F32)
        for lt in range(NL):
            skT_s[lt] = jnp.concatenate(
                [shT[:, lt * T:(lt + 1) * T], jnp.zeros((4, T), F32)], axis=0)
        kpad_s[0:8, :] = jnp.zeros((8, T), F32)

        with jax.named_scope("qproj"):
            jax.lax.fori_loop(0, 4, q_body, 0)
        with jax.named_scope("wait2"):
            cp_wuv.wait()
        with jax.named_scope("vproj"):
            jax.lax.fori_loop(0, 4, v_body, 0)
        with jax.named_scope("wait3"):
            cp_wo.wait()

    pl.run_scoped(
        phase1,
        pltpu.VMEM((S, C), BF),
        pltpu.VMEM((M * H, D), BF),
        pltpu.VMEM((4, C, 8, D), U32),
        pltpu.VMEM((C * H, D), BF),
        pltpu.VMEM((NL, S, T), BF),
        pltpu.VMEM((NL, S, T), BF),
        pltpu.VMEM((M, S), BF),
        pltpu.VMEM((NL, 8, T), F32),
        pltpu.VMEM((S + 16, T), F32),
        pltpu.VMEM((UK_ROWS, T), F32),
        pltpu.SMEM((2,), jnp.int32),
    )

    def phase23(ctx_s, out_v, spre_s):
        tiles = [(g, j, i) for j in range(NB) for g in range(ATT_G) for i in range(j + 1)]

        def qk_next(base, k):
            g, j, i = tiles[k]
            spre_s[k] = _qk_tile(base + g, j, i, k_s, qT_s)

        def att_body(it, carry):
            with jax.named_scope("att_it"):
                return att_body2(it, carry)

        def att_body2(it, carry):
            base = it * ATT_G
            nxt = jnp.minimum(base + ATT_G, H - ATT_G)
            sv = {k: spre_s[k] for k in range(SKEW)}
            states = {}
            for k, (g, j, i) in enumerate(tiles):
                if k + SKEW < len(tiles):
                    g2, j2, i2 = tiles[k + SKEW]
                    sv[k + SKEW] = _qk_tile(base + g2, j2, i2, k_s, qT_s)
                else:
                    qk_next(nxt, k + SKEW - len(tiles))
                _softmax_pv(base + g, j, i, sv.pop(k), states.setdefault((g, j), {}), vT_s, ctx_s)
            return carry

        with jax.named_scope("attn"):
            for k in range(SKEW):
                qk_next(0, k)
            jax.lax.fori_loop(0, H // ATT_G, att_body, 0)

        R = OUT_R
        gw = gw_ref[...].astype(F32).reshape(1, M)
        dv = dvec_ref[...].astype(F32).reshape(1, M)

        NC = M // OCOL

        def out_copy(it, n):
            rows = pl.ds(pl.multiple_of(it * R, R), R)
            cols = pl.ds(n * OCOL, OCOL)
            return pltpu.make_async_copy(out_v.at[rows, cols], out_hbm.at[rows, cols], osems.at[it])

        def out_body(it, carry):
            rows = pl.ds(pl.multiple_of(it * R, R), R)
            prow = pl.ds(pl.multiple_of(it * (R // 2), R // 2), R // 2)
            inv = inv_ref[...]
            ys = []
            for mm in range(R // T):
                m = it * (R // T) + mm
                qm = jnp.concatenate([_tobf(q_s[lt, m]) for lt in range(NL)], axis=1)
                ys.append(jnp.dot(inv, qm, preferred_element_type=F32))
            y = jnp.concatenate(ys, axis=0)
            ctx = jnp.concatenate([_tobf(ctx_s[h, :, rows]).T for h in range(H)], axis=1)
            kv = jnp.concatenate([_tobf(kv_s[lt, prow, :]) for lt in range(NL)], axis=1).astype(F32)
            xr = x_v[rows, :].astype(F32)
            g = jax.nn.sigmoid(jnp.sum(xr * gw, axis=-1, keepdims=True))
            b = (1.0 - g) * (xr * (y + kv * dv))
            for n in range(NC):
                c0, c1 = n * OCOL, (n + 1) * OCOL
                a = jnp.dot(ctx, wo_v[:, c0:c1], preferred_element_type=F32)
                out_v[rows, c0:c1] = (g * a + b[:, c0:c1]).astype(BF)
                out_copy(it, n).start()
            return carry

        with jax.named_scope("oproj"):
            jax.lax.fori_loop(0, S // R, out_body, 0, unroll=OUNROLL)
        with jax.named_scope("wait4"):
            for it in range(S // R):
                for n in range(NC):
                    out_copy(it, n).wait()

    pl.run_scoped(
        phase23,
        pltpu.VMEM((H, D // 2, S), U32),
        pltpu.VMEM((S, M), BF),
        pltpu.VMEM((SKEW, T, T), F32),
    )


@jax.jit
def pallas_gated_mix__compressed_kv_cla__ssm_conv_h3__prompt_kernel(
    A_x, A_c_kv, A_w_q, A_w_uk, A_w_uv, A_w_o, B_q, B_k, B_v, B_shift_k, B_ssm_k, B_ssm_D, gate_w,
):
    fwd_np, inv_np = _dft_consts()
    fwd = jnp.asarray(fwd_np.astype(BF))
    inv = jnp.asarray(inv_np.astype(BF))
    any_spec = pl.BlockSpec(memory_space=pl.ANY)
    out = pl.pallas_call(
        _kernel,
        out_shape=jax.ShapeDtypeStruct((S, M), BF),
        in_specs=[any_spec] * 14,
        out_specs=any_spec,
        scratch_shapes=[
            pltpu.VMEM((S, M), BF),
            pltpu.VMEM((H * D, M), BF),
            pltpu.VMEM((H, D // 2, S), U32),
            pltpu.VMEM((H, S // 2, D), U32),
            pltpu.VMEM((H, D // 2, S), U32),
            pltpu.VMEM((NL, S // 2, T), U32),
            pltpu.VMEM((NL, NB, T, T), U32),
            pltpu.VMEM((4, M), BF),
            pltpu.VMEM((M,), BF),
            pltpu.VMEM((M,), BF),
            pltpu.VMEM((2 * T, T), BF),
            pltpu.VMEM((T, 2 * T), BF),
            pltpu.SemaphoreType.DMA((14 + len(C_CHUNKS),)),
            pltpu.SemaphoreType.DMA((S // OUT_R,)),
        ],
        compiler_params=pltpu.CompilerParams(vmem_limit_bytes=120 * 1024 * 1024),
    )(
        A_x.reshape(S, M), A_c_kv.reshape(S, C),
        A_w_q.reshape(M * H, D), A_w_uk, A_w_uv.reshape(C * H, D),
        A_w_o.reshape(H * D, M),
        B_k.reshape(S, M), B_v.reshape(S, M), B_ssm_k,
        B_shift_k.T, B_ssm_D, gate_w, fwd, inv,
    )
    return out.reshape(1, S, M)
```

```python
import functools
import math

import jax
import jax.numpy as jnp
import numpy as np
import jax.experimental.pallas as pl
import jax.experimental.pallas.tpu as pltpu

BF = jnp.bfloat16
F32 = jnp.float32
U32 = jnp.uint32

S = 2048
M = 1024
C = 512
H = 32
D = 128
T = 128
NB = S // T
NL = M // T
NEG = -1e30
NT_DIMS = (((1,), (1,)), ((), ()))

ATT_G = 4
SKEW = 6
C_CHUNKS = [(0, 128), (128, 512), (512, 2048)]
OUT_R = 256
OCOL = 128


def _tobf(x):
    return pltpu.bitcast(x, BF)


def _tou(x):
    return pltpu.bitcast(x, U32)


def _lo_hi(w):
    lo = pltpu.bitcast(w << 16, F32)
    hi = pltpu.bitcast(w & jnp.uint32(0xFFFF0000), F32)
    return lo, hi


def _dft_consts():
    n_fft = 2 * T
    f = np.concatenate([np.arange(0, T, 2), np.arange(1, T, 2)]).astype(np.float64)
    theta = 2.0 * np.pi * (f + 0.5) / n_fft
    n = np.arange(T, dtype=np.float64)
    ang = theta[:, None] * n[None, :]
    re = np.cos(ang)
    im = -np.sin(ang)
    fwd = np.concatenate([re.reshape(T // 8, 8, T), im.reshape(T // 8, 8, T)], axis=1)
    fwd = fwd.reshape(2 * T, T)
    inv = np.stack([re, im], axis=1).reshape(2 * T, T).T * (2.0 / n_fft)
    return fwd.astype(np.float32), inv.astype(np.float32)


def _qk_tile(h, j, i, k_s, qT_s):
    qT = _tobf(qT_s[h, :, j * T:(j + 1) * T])
    kk = _tobf(k_s[h, i * T // 2:(i + 1) * T // 2, :])
    return jnp.dot(kk, qT, preferred_element_type=F32)


def _softmax_pv(h, j, i, s, st, vT_s, ctx_s):
    if i == j:
        ki = jax.lax.broadcasted_iota(jnp.int32, (T, T), 0)
        qi = jax.lax.broadcasted_iota(jnp.int32, (T, T), 1)
        s = jnp.where(ki <= qi, s, NEG)
    mc = jnp.max(s, axis=0, keepdims=True)
    m_new = mc if i == 0 else jnp.maximum(st["m"], mc)
    p = jnp.exp2(s - m_new)
    lc = jnp.sum(p.reshape(T // 8, 8, T), axis=0)
    pv = jnp.dot(_tobf(vT_s[h, :, i * T:(i + 1) * T]), p.astype(BF), preferred_element_type=F32)
    if i == 0:
        acc, l = pv, lc
    else:
        alpha = jnp.exp2(st["m"] - m_new)
        l = alpha * st["l"] + lc
        acc = alpha * st["acc"] + pv
    st.update(m=m_new, l=l, acc=acc)
    if i == j:
        lsum = jnp.sum(l, axis=0, keepdims=True)
        o = acc * (1.0 / lsum)
        ctx_s[h, :, j * T:(j + 1) * T] = _tou(o.astype(BF))


MG = 8
IG = 4
SPLIT0 = 1
KV0 = 1
KVCH = 2
FIRST = 4
LAST = 15
NG = T // 8
U_OFF = 0
W_OFF = U_OFF + NB * NG * 24
A_OFF = W_OFF + NB * NG * 24
R_OFF = A_OFF + NB * 8
DUMMY = R_OFF + NB * 8
UK_ROWS = DUMMY + 8


def _conv_pieces(lt, bk_v, bv_v, sk_v, skT_s, fwd_ref, kpad_s, kv_s, q_s, uk_s, dyn, dyn2):
    st = {}

    def p_kv(i, val):
        if val is not None:
            kpad_s[pl.ds(dyn2, 8), :] = val
        r0 = i * T
        kf = bk_v[lt, r0:r0 + T, :].astype(F32)
        kpad_s[8 + r0:8 + r0 + T, :] = kf
        sk = skT_s[lt]
        ksh = kf * sk[0:1, :]
        for j in range(1, 4):
            ksh = ksh + kpad_s[8 + r0 - j:8 + r0 - j + T, :] * sk[j:j + 1, :]
        kv = (ksh * bv_v[lt, r0:r0 + T, :].astype(F32)).astype(BF)
        kv_s[lt, r0 // 2:(r0 + T) // 2, :] = _tou(kv)
        st["kv", i] = kv

    def p_dft_k(_):
        fwd = fwd_ref[...]
        ssm = sk_v[pl.ds(pl.multiple_of(lt * T, T), T), :]
        prev = None
        for d in range(NB):
            k = jax.lax.dot_general(fwd, ssm[:, d * T:(d + 1) * T], NT_DIMS,
                                    preferred_element_type=F32)
            for g in range(NG):
                kr, ki = k[16 * g:16 * g + 8], k[16 * g + 8:16 * g + 16]
                if prev is None:
                    wr, wi = kr, ki
                else:
                    pr, pi = prev[16 * g:16 * g + 8], prev[16 * g + 8:16 * g + 16]
                    if g < NG // 2:
                        wr, wi = kr - pi, ki + pr
                    else:
                        wr, wi = kr + pi, ki - pr
                r = W_OFF + (g * NB + d) * 24
                uk_s[r:r + 8, :] = wr
                uk_s[r + 8:r + 16, :] = wi - wr
                uk_s[r + 16:r + 24, :] = -(wr + wi)
            prev = k

    def p_dft_u(i):
        fwd = fwd_ref[...]
        u = jnp.dot(fwd, st["kv", i], preferred_element_type=F32)
        for g in range(NG):
            ur, ui = u[16 * g:16 * g + 8], u[16 * g + 8:16 * g + 16]
            r = U_OFF + (g * NB + i) * 24
            uk_s[r:r + 8, :] = ur
            uk_s[r + 8:r + 16, :] = ui
            uk_s[r + 16:r + 24, :] = ur + ui

    def gate(val):
        if val is not None:
            uk_s[pl.ds(dyn, 8), :] = val

    def ld1(off, g, k, i):
        r = off + (g * NB + i) * 24 + 8 * k
        return uk_s[r:r + 8, :]

    def sub(kind, g, m0, i0, val):
        gate(val)
        ka, kb = {"a": (2, 0), "c": (1, 2), "b": (0, 1)}[kind]
        ms = range(m0, m0 + MG)
        if i0 == 0:
            if kind == "a":
                st["acc"] = {m: None for m in ms}
            else:
                st["acc"] = {m: uk_s[A_OFF + 8 * m:A_OFF + 8 * m + 8, :] for m in ms}
        acc = st["acc"]
        av = {i: ld1(U_OFF, g, ka, i) for i in range(i0, min(i0 + IG, m0 + MG))}
        bv = {}
        for i in av:
            for m in ms:
                j = m - i
                if j < 0:
                    continue
                if j not in bv:
                    bv[j] = ld1(W_OFF, g, kb, j)
                t = av[i] * bv[j]
                acc[m] = t if acc[m] is None else acc[m] + t
        if i0 + IG >= m0 + MG:
            for m in ms:
                if kind == "a":
                    uk_s[A_OFF + 8 * m:A_OFF + 8 * m + 8, :] = acc[m]
                elif kind == "c":
                    uk_s[R_OFF + 8 * m:R_OFF + 8 * m + 8, :] = acc[m]
                else:
                    re = uk_s[R_OFF + 8 * m:R_OFF + 8 * m + 8, :]
                    q_s[lt, m, g * 8:(g + 1) * 8, :] = pltpu.pack_elementwise(
                        [re, acc[m]], packed_dtype=BF)

    subs = []
    for g in range(NG):
        for kind in ("a", "c", "b"):
            for m0 in range(0, NB, MG):
                for i0 in range(0, m0 + MG, IG):
                    subs.append(functools.partial(sub, kind, g, m0, i0))
    return p_dft_k, p_kv, p_dft_u, subs


def _spread(subs, n, first, last, slabs=128):
    sched = [[] for _ in range(n)]
    npts = (last - first) * slabs
    for i, pc in enumerate(subs):
        pt = (i * npts) // len(subs)
        sched[first + pt // slabs].append((pt % slabs, pc))
    return sched


def _kernel(x_hbm, c_hbm, wq_hbm, wuk_hbm, wuv_hbm, wo_hbm, bk_hbm, bv_hbm, sk_hbm,
            shT_hbm, dvec_hbm, gw_hbm, fwd_hbm, inv_hbm,
            out_hbm,
            x_v, wo_v, qT_s, k_s, vT_s, kv_s, q_s,
            shT_ref, dvec_ref, gw_ref, fwd_ref, inv_ref, sems, osem):
    qscale = (D ** -0.5) * math.log2(math.e)

    def phase1(c_v, wq_v, wuk_v, wuv_v, bk_v, bv_v, sk_v, skT_s, kpad_s, uk_s, dyn_s):
        dyn_s[0] = DUMMY
        dyn_s[1] = S + 8
        wuk_hbm32 = wuk_hbm.bitcast(U32)
        cp_wuk = [pltpu.make_async_copy(
            wuk_hbm32.at[:, pl.ds(4 * a, 4), :], wuk_v.at[a, :, pl.ds(0, 4), :], sems.at[9 + a])
            for a in range(4)]
        cp_c = [pltpu.make_async_copy(c_hbm.at[pl.ds(r0, r1 - r0)], c_v.at[pl.ds(r0, r1 - r0)],
                                      sems.at[14 + i]) for i, (r0, r1) in enumerate(C_CHUNKS)]
        cp_wuv = pltpu.make_async_copy(wuv_hbm, wuv_v, sems.at[2])
        cp_x = pltpu.make_async_copy(x_hbm, x_v, sems.at[3])
        cp_wq = pltpu.make_async_copy(wq_hbm, wq_v, sems.at[4])
        cp_sk = pltpu.make_async_copy(sk_hbm, sk_v, sems.at[5])
        cp_bk = [pltpu.make_async_copy(bk_hbm.at[:, pl.ds(lt * T, T)], bk_v.at[lt], sems.at[6])
                 for lt in range(NL)]
        cp_bv = [pltpu.make_async_copy(bv_hbm.at[:, pl.ds(lt * T, T)], bv_v.at[lt], sems.at[7])
                 for lt in range(NL)]
        cp_wo = pltpu.make_async_copy(wo_hbm, wo_v, sems.at[8])
        cp_small = [pltpu.make_async_copy(a, b, sems.at[13]) for a, b in
                    [(shT_hbm, shT_ref), (dvec_hbm, dvec_ref), (gw_hbm, gw_ref),
                     (fwd_hbm, fwd_ref), (inv_hbm, inv_ref)]]
        for cp in ([cp_wuk[0]] + cp_c + cp_wuk[1:] + cp_small + [cp_x, cp_wq, cp_sk]
                   + cp_bk + cp_bv + [cp_wuv, cp_wo]):
            cp.start()

        wq32 = wq_v.bitcast(U32)
        wuv32 = wuv_v.bitcast(U32)

        def load_weights_t(w32, rows, it):
            view = w32.at[pl.ds(pl.multiple_of(it * 4, 4), rows * 16 - 12)]
            outs = []
            for g in range(4):
                outs += list(_lo_hi(view[pl.ds(g, rows, stride=16), :].T))
            return jnp.concatenate(outs, axis=0).astype(BF)

        wuk2 = wuk_v.reshape(4 * C * 8, D)

        def k_group(it, first):
            pltpu.make_async_copy(wuk_hbm32.at[:, pl.ds(pl.multiple_of(4 * it, 4), 4), :],
                                  wuk_v.at[it, :, pl.ds(0, 4), :], sems.at[9 + it]).wait()
            view = wuk2.at[pl.ds(pl.multiple_of(it * C * 8, 8), C * 8)]
            ws = []
            for g in range(4):
                lo, hi = _lo_hi(view[pl.ds(g, C, stride=8), :])
                ws.append(jnp.concatenate([lo, hi], axis=1).astype(BF))
            for i, (r0, r1) in enumerate(C_CHUNKS if first else [(0, S)]):
                if first:
                    cp_c[i].wait()
                for g in range(4):
                    k = jnp.dot(c_v[r0:r1, :], ws[g], preferred_element_type=F32)
                    for u in range(2):
                        k_s[it * 8 + 2 * g + u, r0 // 2:r1 // 2, :] = _tou(
                            k[:, u * D:(u + 1) * D].astype(BF))

        def k_body(it, carry):
            with jax.named_scope("k_it"):
                k_group(it, False)
            return carry

        with jax.named_scope("kproj0"):
            k_group(0, True)
        with jax.named_scope("kproj"):
            jax.lax.fori_loop(1, 4, k_body, 0)

        def proj_conv_body(it, lt, w32, rows, src_v, dst_s, scale):
            p_dft_k, p_kv, p_dft_u, subs = _conv_pieces(
                lt, bk_v, bv_v, sk_v, skT_s, fwd_ref, kpad_s, kv_s, q_s, uk_s,
                pl.multiple_of(dyn_s[0], 8), pl.multiple_of(dyn_s[1], 8))
            p_dft_k(None)
            w = load_weights_t(w32, rows, it)
            sched = _spread(subs, NB, FIRST, LAST)
            nkv = NB // KVCH
            for n in range(NB):
                src = src_v[n * T:(n + 1) * T, :]
                if n < SPLIT0:
                    o = jnp.concatenate(
                        [jax.lax.dot_general(w[p * 2 * D:(p + 1) * 2 * D], src, NT_DIMS,
                                             preferred_element_type=F32) for p in range(4)], axis=0)
                else:
                    o = jax.lax.dot_general(w, src, NT_DIMS, preferred_element_type=F32)
                if scale is not None:
                    o = o * scale
                for g in range(8):
                    dst_s[it * 8 + g, :, n * T:(n + 1) * T] = _tou(o[g * D:(g + 1) * D].astype(BF))
                if KV0 + 1 <= n <= KV0 + KVCH:
                    for i in range((n - KV0 - 1) * nkv, (n - KV0) * nkv):
                        p_dft_u(i)
                if KV0 <= n < KV0 + KVCH:
                    for k_ in range(nkv):
                        sl = (128 * k_) // nkv
                        p_kv((n - KV0) * nkv + k_, o[8 * sl:8 * sl + 8])
                for sl, pc in sched[n]:
                    pc(o[8 * sl:8 * sl + 8])

        def q_body(it, carry):
            with jax.named_scope("q_it"):
                proj_conv_body(it, it, wq32, M, x_v, qT_s, qscale)
            return carry

        def v_body(it, carry):
            with jax.named_scope("v_it"):
                proj_conv_body(it, 4 + it, wuv32, C, c_v, vT_s, None)
            return carry

        with jax.named_scope("wait1"):
            for cp in cp_small + [cp_x, cp_wq, cp_sk]:
                cp.wait()
            pltpu.make_async_copy(bk_v, bk_v, sems.at[6]).wait()
            pltpu.make_async_copy(bv_v, bv_v, sems.at[7]).wait()
        shT = shT_ref[...].astype(F32)
        for lt in range(NL):
            skT_s[lt] = jnp.concatenate(
                [shT[:, lt * T:(lt + 1) * T], jnp.zeros((4, T), F32)], axis=0)
        kpad_s[0:8, :] = jnp.zeros((8, T), F32)

        with jax.named_scope("qproj"):
            jax.lax.fori_loop(0, 4, q_body, 0)
        with jax.named_scope("wait2"):
            cp_wuv.wait()
        with jax.named_scope("vproj"):
            jax.lax.fori_loop(0, 4, v_body, 0)
        with jax.named_scope("wait3"):
            cp_wo.wait()

    pl.run_scoped(
        phase1,
        pltpu.VMEM((S, C), BF),
        pltpu.VMEM((M * H, D), BF),
        pltpu.VMEM((4, C, 8, D), U32),
        pltpu.VMEM((C * H, D), BF),
        pltpu.VMEM((NL, S, T), BF),
        pltpu.VMEM((NL, S, T), BF),
        pltpu.VMEM((M, S), BF),
        pltpu.VMEM((NL, 8, T), F32),
        pltpu.VMEM((S + 16, T), F32),
        pltpu.VMEM((UK_ROWS, T), F32),
        pltpu.SMEM((2,), jnp.int32),
    )

    def phase23(ctx_s, out_v, spre_s):
        ORDER = 0
        if ORDER == 0:
            tiles = [(g, j, i) for j in range(NB) for g in range(ATT_G) for i in range(j + 1)]
        elif ORDER == 1:
            tiles = [(g, j, i) for j in range(NB) for i in range(j + 1) for g in range(ATT_G)]
        elif ORDER == 2:
            tiles = [(g, j, i) for g in range(ATT_G) for j in range(NB) for i in range(j + 1)]
        elif ORDER == 3:
            tiles = [(g, j, i) for j in reversed(range(NB)) for g in range(ATT_G) for i in range(j + 1)]
        elif ORDER == 4:
            tiles = [(g, j, i) for j in range(NB) for gp in range(0, ATT_G, 2) for i in range(j + 1)
                     for g in (gp, gp + 1)]

        def qk_next(base, k):
            g, j, i = tiles[k]
            spre_s[k] = _qk_tile(base + g, j, i, k_s, qT_s)

        def att_body(it, carry):
            with jax.named_scope("att_it"):
                return att_body2(it, carry)

        def att_body2(it, carry):
            base = it * ATT_G
            nxt = jnp.minimum(base + ATT_G, H - ATT_G)
            sv = {k: spre_s[k] for k in range(SKEW)}
            states = {}
            for k, (g, j, i) in enumerate(tiles):
                if k + SKEW < len(tiles):
                    g2, j2, i2 = tiles[k + SKEW]
                    sv[k + SKEW] = _qk_tile(base + g2, j2, i2, k_s, qT_s)
                else:
                    qk_next(nxt, k + SKEW - len(tiles))
                _softmax_pv(base + g, j, i, sv.pop(k), states.setdefault((g, j), {}), vT_s, ctx_s)
            return carry

        with jax.named_scope("attn"):
            for k in range(SKEW):
                qk_next(0, k)
            jax.lax.fori_loop(0, H // ATT_G, att_body, 0)

        R = OUT_R
        gw = gw_ref[...].astype(F32).reshape(1, M)
        dv = dvec_ref[...].astype(F32).reshape(1, M)

        NC = M // OCOL

        def out_copy(it, n):
            rows = pl.ds(pl.multiple_of(it * R, R), R)
            cols = pl.ds(n * OCOL, OCOL)
            return pltpu.make_async_copy(out_v.at[rows, cols], out_hbm.at[rows, cols], osem)

        def out_body(it, carry):
            rows = pl.ds(pl.multiple_of(it * R, R), R)
            prow = pl.ds(pl.multiple_of(it * (R // 2), R // 2), R // 2)
            inv = inv_ref[...]
            ys = []
            for mm in range(R // T):
                m = it * (R // T) + mm
                qm = jnp.concatenate([_tobf(q_s[lt, m]) for lt in range(NL)], axis=1)
                ys.append(jnp.dot(inv, qm, preferred_element_type=F32))
            y = jnp.concatenate(ys, axis=0)
            ctx = jnp.concatenate([_tobf(ctx_s[h, :, rows]).T for h in range(H)], axis=1)
            kv = jnp.concatenate([_tobf(kv_s[lt, prow, :]) for lt in range(NL)], axis=1).astype(F32)
            xr = x_v[rows, :].astype(F32)
            g = jax.nn.sigmoid(jnp.sum(xr * gw, axis=-1, keepdims=True))
            b = (1.0 - g) * (xr * (y + kv * dv))
            for n in range(NC):
                c0, c1 = n * OCOL, (n + 1) * OCOL
                a = jnp.dot(ctx, wo_v[:, c0:c1], preferred_element_type=F32)
                out_v[rows, c0:c1] = (g * a + b[:, c0:c1]).astype(BF)
                out_copy(it, n).start()
            return carry

        with jax.named_scope("oproj"):
            jax.lax.fori_loop(0, S // R, out_body, 0)
        with jax.named_scope("wait4"):
            pltpu.make_async_copy(out_v, out_hbm, osem).wait()

    pl.run_scoped(
        phase23,
        pltpu.VMEM((H, D // 2, S), U32),
        pltpu.VMEM((S, M), BF),
        pltpu.VMEM((SKEW, T, T), F32),
    )


@jax.jit
def pallas_gated_mix__compressed_kv_cla__ssm_conv_h3__prompt_kernel(
    A_x, A_c_kv, A_w_q, A_w_uk, A_w_uv, A_w_o, B_q, B_k, B_v, B_shift_k, B_ssm_k, B_ssm_D, gate_w,
):
    fwd_np, inv_np = _dft_consts()
    fwd = jnp.asarray(fwd_np.astype(BF))
    inv = jnp.asarray(inv_np.astype(BF))
    any_spec = pl.BlockSpec(memory_space=pl.ANY)
    out = pl.pallas_call(
        _kernel,
        out_shape=jax.ShapeDtypeStruct((S, M), BF),
        in_specs=[any_spec] * 14,
        out_specs=any_spec,
        scratch_shapes=[
            pltpu.VMEM((S, M), BF),
            pltpu.VMEM((H * D, M), BF),
            pltpu.VMEM((H, D // 2, S), U32),
            pltpu.VMEM((H, S // 2, D), U32),
            pltpu.VMEM((H, D // 2, S), U32),
            pltpu.VMEM((NL, S // 2, T), U32),
            pltpu.VMEM((NL, NB, T, T), U32),
            pltpu.VMEM((4, M), BF),
            pltpu.VMEM((M,), BF),
            pltpu.VMEM((M,), BF),
            pltpu.VMEM((2 * T, T), BF),
            pltpu.VMEM((T, 2 * T), BF),
            pltpu.SemaphoreType.DMA((14 + len(C_CHUNKS),)),
            pltpu.SemaphoreType.DMA(()),
        ],
        compiler_params=pltpu.CompilerParams(vmem_limit_bytes=120 * 1024 * 1024),
    )(
        A_x.reshape(S, M), A_c_kv.reshape(S, C),
        A_w_q.reshape(M * H, D), A_w_uk, A_w_uv.reshape(C * H, D),
        A_w_o.reshape(H * D, M),
        B_k.reshape(S, M), B_v.reshape(S, M), B_ssm_k,
        B_shift_k.T, B_ssm_D, gate_w, fwd, inv,
    )
    return out.reshape(1, S, M)
```

```python
import functools
import math

import jax
import jax.numpy as jnp
import numpy as np
import jax.experimental.pallas as pl
import jax.experimental.pallas.tpu as pltpu

BF = jnp.bfloat16
F32 = jnp.float32
U32 = jnp.uint32

S = 2048
M = 1024
C = 512
H = 32
D = 128
T = 128
NB = S // T
NL = M // T
NEG = -1e30
NT_DIMS = (((1,), (1,)), ((), ()))

ATT_G = 4
C_CHUNKS = [(0, 128), (128, 512), (512, 2048)]
SKEW = 6
OCOL = 128
WQ_SEM = 17
WUV_SEM = 21
OUT_R = 256


def _tobf(x):
    return pltpu.bitcast(x, BF)


def _tou(x):
    return pltpu.bitcast(x, U32)


def _lo_hi(w):
    lo = pltpu.bitcast(w << 16, F32)
    hi = pltpu.bitcast(w & jnp.uint32(0xFFFF0000), F32)
    return lo, hi


def _dft_consts():
    n_fft = 2 * T
    f = np.concatenate([np.arange(0, T, 2), np.arange(1, T, 2)]).astype(np.float64)
    theta = 2.0 * np.pi * (f + 0.5) / n_fft
    n = np.arange(T, dtype=np.float64)
    ang = theta[:, None] * n[None, :]
    re = np.cos(ang)
    im = -np.sin(ang)
    fwd = np.concatenate([re.reshape(T // 8, 8, T), im.reshape(T // 8, 8, T)], axis=1)
    fwd = fwd.reshape(2 * T, T)
    inv = np.stack([re, im], axis=1).reshape(2 * T, T).T * (2.0 / n_fft)
    return fwd.astype(np.float32), inv.astype(np.float32)


def _qk_tile(h, j, i, k_s, qT_s):
    qT = _tobf(qT_s[h, :, j * T:(j + 1) * T])
    kk = _tobf(k_s[h, i * T // 2:(i + 1) * T // 2, :])
    return jnp.dot(kk, qT, preferred_element_type=F32)


def _softmax_pv(h, j, i, s, st, vT_s, ctx_s):
    if i == j:
        ki = jax.lax.broadcasted_iota(jnp.int32, (T, T), 0)
        qi = jax.lax.broadcasted_iota(jnp.int32, (T, T), 1)
        s = jnp.where(ki <= qi, s, NEG)
    mc = jnp.max(s, axis=0, keepdims=True)
    m_new = mc if i == 0 else jnp.maximum(st["m"], mc)
    p = jnp.exp2(s - m_new)
    lc = jnp.sum(p.reshape(T // 8, 8, T), axis=0)
    pv = jnp.dot(_tobf(vT_s[h, :, i * T:(i + 1) * T]), p.astype(BF), preferred_element_type=F32)
    if i == 0:
        acc, l = pv, lc
    else:
        alpha = jnp.exp2(st["m"] - m_new)
        l = alpha * st["l"] + lc
        acc = alpha * st["acc"] + pv
    st.update(m=m_new, l=l, acc=acc)
    if i == j:
        lsum = jnp.sum(l, axis=0, keepdims=True)
        o = acc * (1.0 / lsum)
        ctx_s[h, :, j * T:(j + 1) * T] = _tou(o.astype(BF))


MG = 8
IG = 4
SPLIT0 = 1
KV0 = 1
KVCH = 2
FIRST = 4
LAST = 15
NG = T // 8
U_OFF = 0
W_OFF = U_OFF + NB * NG * 24
A_OFF = W_OFF + NB * NG * 24
R_OFF = A_OFF + NB * 8
DUMMY = R_OFF + NB * 8
UK_ROWS = DUMMY + 8


def _conv_pieces(lt, bk_v, bv_v, sk_v, skT_s, fwd_ref, kv_s, q_s, uk_s, dyn, dyn2):
    st = {}

    def p_kv(i, val):
        if val is not None:
            bk_v[dyn2, 0:8, :] = val.astype(BF)
        r0 = i * T
        kf = bk_v[lt, r0:r0 + T, :].astype(F32)
        prev = st["klast"] if i > 0 else jnp.zeros((8, T), F32)
        ext = jnp.concatenate([prev, kf], axis=0)
        st["klast"] = kf[T - 8:]
        sk = skT_s[lt]
        ksh = kf * sk[0:1, :]
        for j in range(1, 4):
            ksh = ksh + pltpu.roll(ext, j, 0)[8:] * sk[j:j + 1, :]
        kv = (ksh * bv_v[lt, r0:r0 + T, :].astype(F32)).astype(BF)
        kv_s[lt, r0 // 2:(r0 + T) // 2, :] = _tou(kv)
        st["kv", i] = kv

    def p_dft_k(_):
        fwd = fwd_ref[...]
        ssm = sk_v[pl.ds(pl.multiple_of(lt * T, T), T), :]
        prev = None
        for d in range(NB):
            k = jax.lax.dot_general(fwd, ssm[:, d * T:(d + 1) * T], NT_DIMS,
                                    preferred_element_type=F32)
            for g in range(NG):
                kr, ki = k[16 * g:16 * g + 8], k[16 * g + 8:16 * g + 16]
                if prev is None:
                    wr, wi = kr, ki
                else:
                    pr, pi = prev[16 * g:16 * g + 8], prev[16 * g + 8:16 * g + 16]
                    if g < NG // 2:
                        wr, wi = kr - pi, ki + pr
                    else:
                        wr, wi = kr + pi, ki - pr
                r = W_OFF + (g * NB + d) * 24
                uk_s[r:r + 8, :] = wr
                uk_s[r + 8:r + 16, :] = wi - wr
                uk_s[r + 16:r + 24, :] = -(wr + wi)
            prev = k

    def p_dft_u(i):
        fwd = fwd_ref[...]
        u = jnp.dot(fwd, st["kv", i], preferred_element_type=F32)
        for g in range(NG):
            ur, ui = u[16 * g:16 * g + 8], u[16 * g + 8:16 * g + 16]
            r = U_OFF + (g * NB + i) * 24
            uk_s[r:r + 8, :] = ur
            uk_s[r + 8:r + 16, :] = ui
            uk_s[r + 16:r + 24, :] = ur + ui

    def gate(val):
        if val is not None:
            uk_s[pl.ds(dyn, 8), :] = val

    def ld1(off, g, k, i):
        r = off + (g * NB + i) * 24 + 8 * k
        return uk_s[r:r + 8, :]

    def sub(kind, g, m0, i0, val):
        gate(val)
        ka, kb = {"a": (2, 0), "c": (1, 2), "b": (0, 1)}[kind]
        ms = range(m0, m0 + MG)
        if i0 == 0:
            if kind == "a":
                st["acc"] = {m: None for m in ms}
            else:
                st["acc"] = {m: uk_s[A_OFF + 8 * m:A_OFF + 8 * m + 8, :] for m in ms}
        acc = st["acc"]
        av = {i: ld1(U_OFF, g, ka, i) for i in range(i0, min(i0 + IG, m0 + MG))}
        bv = {}
        for i in av:
            for m in ms:
                j = m - i
                if j < 0:
                    continue
                if j not in bv:
                    bv[j] = ld1(W_OFF, g, kb, j)
                t = av[i] * bv[j]
                acc[m] = t if acc[m] is None else acc[m] + t
        if i0 + IG >= m0 + MG:
            for m in ms:
                if kind == "a":
                    uk_s[A_OFF + 8 * m:A_OFF + 8 * m + 8, :] = acc[m]
                elif kind == "c":
                    uk_s[R_OFF + 8 * m:R_OFF + 8 * m + 8, :] = acc[m]
                else:
                    re = uk_s[R_OFF + 8 * m:R_OFF + 8 * m + 8, :]
                    q_s[lt, m, g * 8:(g + 1) * 8, :] = pltpu.pack_elementwise(
                        [re, acc[m]], packed_dtype=BF)

    subs = []
    for g in range(NG):
        for kind in ("a", "c", "b"):
            for m0 in range(0, NB, MG):
                for i0 in range(0, m0 + MG, IG):
                    subs.append(functools.partial(sub, kind, g, m0, i0))
    return p_dft_k, p_kv, p_dft_u, subs


def _spread(subs, n, first, last, slabs=128):
    sched = [[] for _ in range(n)]
    npts = (last - first) * slabs
    for i, pc in enumerate(subs):
        pt = (i * npts) // len(subs)
        sched[first + pt // slabs].append((pt % slabs, pc))
    return sched


def _kernel(x_hbm, c_hbm, wq_hbm, wuk_hbm, wuv_hbm, wo_hbm, bk_hbm, bv_hbm, sk_hbm,
            shT_hbm, dvec_hbm, gw_hbm, fwd_hbm, inv_hbm,
            out_hbm,
            x_v, wo_v, qT_s, k_s, vT_s, kv_s, q_s,
            shT_ref, dvec_ref, gw_ref, fwd_ref, inv_ref, sems, osem):
    qscale = (D ** -0.5) * math.log2(math.e)

    def phase1(c_v, wq_v, wuk_v, wuv_v, bk_v, bv_v, sk_v, skT_s, uk_s, dyn_s):
        dyn_s[0] = DUMMY
        dyn_s[1] = NL
        wuk_hbm32 = wuk_hbm.bitcast(U32)
        cp_wuk = [pltpu.make_async_copy(
            wuk_hbm32.at[:, pl.ds(4 * a, 4), :], wuk_v.at[a, :, pl.ds(0, 4), :], sems.at[9 + a])
            for a in range(4)]
        cp_c = [pltpu.make_async_copy(c_hbm.at[pl.ds(r0, r1 - r0)], c_v.at[pl.ds(r0, r1 - r0)],
                                      sems.at[14 + i]) for i, (r0, r1) in enumerate(C_CHUNKS)]
        wq_hbm32 = wq_hbm.bitcast(U32)
        wuv_hbm32 = wuv_hbm.bitcast(U32)

        def cp_quarter(w_hbm32, w_v, sem0, q):
            start = 4 * q if isinstance(q, int) else pl.multiple_of(4 * q, 4)
            return pltpu.make_async_copy(w_hbm32.at[:, pl.ds(start, 4), :],
                                         w_v.at[q % 2, :, pl.ds(0, 4), :], sems.at[sem0 + q])

        cp_x = pltpu.make_async_copy(x_hbm, x_v, sems.at[3])
        cp_sk = pltpu.make_async_copy(sk_hbm, sk_v, sems.at[5])
        cp_bk = [pltpu.make_async_copy(bk_hbm.at[:, pl.ds(lt * T, T)], bk_v.at[lt], sems.at[6])
                 for lt in range(NL)]
        cp_bv = [pltpu.make_async_copy(bv_hbm.at[:, pl.ds(lt * T, T)], bv_v.at[lt], sems.at[7])
                 for lt in range(NL)]
        cp_wo = pltpu.make_async_copy(wo_hbm, wo_v, sems.at[8])
        cp_small = [pltpu.make_async_copy(a, b, sems.at[13]) for a, b in
                    [(shT_hbm, shT_ref), (dvec_hbm, dvec_ref), (gw_hbm, gw_ref),
                     (fwd_hbm, fwd_ref), (inv_hbm, inv_ref)]]
        cp_wq = [cp_quarter(wq_hbm32, wq_v, WQ_SEM, q) for q in range(2)]
        cp_wuv = [cp_quarter(wuv_hbm32, wuv_v, WUV_SEM, q) for q in range(2)]
        for cp in ([cp_wuk[0]] + cp_c + cp_wuk[1:] + cp_small + [cp_x] + cp_wq + [cp_sk]
                   + cp_bk + cp_bv + cp_wuv + [cp_wo]):
            cp.start()

        def load_weights_t(w_v, rows, it):
            w2 = w_v.reshape(2 * rows * 8, D)
            view = w2.at[pl.ds(pl.multiple_of((it % 2) * rows * 8, 8), rows * 8)]
            outs = []
            for g in range(4):
                outs += list(_lo_hi(view[pl.ds(g, rows, stride=8), :].T))
            return jnp.concatenate(outs, axis=0).astype(BF)

        wuk2 = wuk_v.reshape(4 * C * 8, D)

        def k_group(it, first):
            pltpu.make_async_copy(wuk_hbm32.at[:, pl.ds(pl.multiple_of(4 * it, 4), 4), :],
                                  wuk_v.at[it, :, pl.ds(0, 4), :], sems.at[9 + it]).wait()
            view = wuk2.at[pl.ds(pl.multiple_of(it * C * 8, 8), C * 8)]
            ws = []
            for g in range(4):
                lo, hi = _lo_hi(view[pl.ds(g, C, stride=8), :])
                ws.append(jnp.concatenate([lo, hi], axis=1).astype(BF))
            for i, (r0, r1) in enumerate(C_CHUNKS if first else [(0, S)]):
                if first:
                    cp_c[i].wait()
                for g in range(4):
                    k = jnp.dot(c_v[r0:r1, :], ws[g], preferred_element_type=F32)
                    for u in range(2):
                        k_s[it * 8 + 2 * g + u, r0 // 2:r1 // 2, :] = _tou(
                            k[:, u * D:(u + 1) * D].astype(BF))

        def k_body(it, carry):
            with jax.named_scope("k_it"):
                k_group(it, False)
            return carry

        with jax.named_scope("kproj0"):
            k_group(0, True)
        with jax.named_scope("kproj"):
            jax.lax.fori_loop(1, 4, k_body, 0)

        def proj_conv_body(it, lt, w_hbm32, w_v, sem0, rows, src_v, dst_s, scale):
            cp_quarter(w_hbm32, w_v, sem0, it).wait()
            p_dft_k, p_kv, p_dft_u, subs = _conv_pieces(
                lt, bk_v, bv_v, sk_v, skT_s, fwd_ref, kv_s, q_s, uk_s,
                pl.multiple_of(dyn_s[0], 8), dyn_s[1])
            p_dft_k(None)
            w = load_weights_t(w_v, rows, it)
            sched = _spread(subs, NB, FIRST, LAST)
            nkv = NB // KVCH
            for n in range(NB):
                src = src_v[n * T:(n + 1) * T, :]
                if n < SPLIT0:
                    o = jnp.concatenate(
                        [jax.lax.dot_general(w[p * 2 * D:(p + 1) * 2 * D], src, NT_DIMS,
                                             preferred_element_type=F32) for p in range(4)], axis=0)
                else:
                    o = jax.lax.dot_general(w, src, NT_DIMS, preferred_element_type=F32)
                if scale is not None:
                    o = o * scale
                for g in range(8):
                    dst_s[it * 8 + g, :, n * T:(n + 1) * T] = _tou(o[g * D:(g + 1) * D].astype(BF))
                if KV0 + 1 <= n <= KV0 + KVCH:
                    for i in range((n - KV0 - 1) * nkv, (n - KV0) * nkv):
                        p_dft_u(i)
                if KV0 <= n < KV0 + KVCH:
                    for k_ in range(nkv):
                        sl = (128 * k_) // nkv
                        p_kv((n - KV0) * nkv + k_, o[8 * sl:8 * sl + 8])
                for sl, pc in sched[n]:
                    pc(o[8 * sl:8 * sl + 8])

            @pl.when(it < 2)
            def _():
                cp_quarter(w_hbm32, w_v, sem0, it + 2).start()

        def q_body(it, carry):
            with jax.named_scope("q_it"):
                proj_conv_body(it, it, wq_hbm32, wq_v, WQ_SEM, M, x_v, qT_s, qscale)
            return carry

        def v_body(it, carry):
            with jax.named_scope("v_it"):
                proj_conv_body(it, 4 + it, wuv_hbm32, wuv_v, WUV_SEM, C, c_v, vT_s, None)
            return carry

        with jax.named_scope("wait1"):
            for cp in cp_small + [cp_x, cp_sk]:
                cp.wait()
            pltpu.make_async_copy(bk_v.at[0:NL], bk_v.at[0:NL], sems.at[6]).wait()
            pltpu.make_async_copy(bv_v, bv_v, sems.at[7]).wait()
        shT = shT_ref[...].astype(F32)
        for lt in range(NL):
            skT_s[lt] = jnp.concatenate(
                [shT[:, lt * T:(lt + 1) * T], jnp.zeros((4, T), F32)], axis=0)

        with jax.named_scope("qproj"):
            jax.lax.fori_loop(0, 4, q_body, 0)
        with jax.named_scope("vproj"):
            jax.lax.fori_loop(0, 4, v_body, 0)
        with jax.named_scope("wait3"):
            cp_wo.wait()

    pl.run_scoped(
        phase1,
        pltpu.VMEM((S, C), BF),
        pltpu.VMEM((2, M, 8, D), U32),
        pltpu.VMEM((4, C, 8, D), U32),
        pltpu.VMEM((2, C, 8, D), U32),
        pltpu.VMEM((NL + 1, S, T), BF),
        pltpu.VMEM((NL, S, T), BF),
        pltpu.VMEM((M, S), BF),
        pltpu.VMEM((NL, 8, T), F32),
        pltpu.VMEM((UK_ROWS, T), F32),
        pltpu.SMEM((2,), jnp.int32),
    )

    def phase23(ctx_s, out_v, spre_s):
        ORDER = 0
        if ORDER == 0:
            tiles = [(g, j, i) for j in range(NB) for g in range(ATT_G) for i in range(j + 1)]
        elif ORDER == 1:
            tiles = [(g, j, i) for j in range(NB) for i in range(j + 1) for g in range(ATT_G)]
        elif ORDER == 2:
            tiles = [(g, j, i) for g in range(ATT_G) for j in range(NB) for i in range(j + 1)]
        elif ORDER == 3:
            tiles = [(g, j, i) for j in reversed(range(NB)) for g in range(ATT_G) for i in range(j + 1)]
        elif ORDER == 4:
            tiles = [(g, j, i) for j in range(NB) for gp in range(0, ATT_G, 2) for i in range(j + 1)
                     for g in (gp, gp + 1)]

        def qk_next(base, k):
            g, j, i = tiles[k]
            spre_s[k] = _qk_tile(base + g, j, i, k_s, qT_s)

        def att_body(it, carry):
            with jax.named_scope("att_it"):
                return att_body2(it, carry)

        def att_body2(it, carry):
            base = it * ATT_G
            nxt = jnp.minimum(base + ATT_G, H - ATT_G)
            sv = {k: spre_s[k] for k in range(SKEW)}
            states = {}
            for k, (g, j, i) in enumerate(tiles):
                if k + SKEW < len(tiles):
                    g2, j2, i2 = tiles[k + SKEW]
                    sv[k + SKEW] = _qk_tile(base + g2, j2, i2, k_s, qT_s)
                else:
                    qk_next(nxt, k + SKEW - len(tiles))
                _softmax_pv(base + g, j, i, sv.pop(k), states.setdefault((g, j), {}), vT_s, ctx_s)
            return carry

        with jax.named_scope("attn"):
            for k in range(SKEW):
                qk_next(0, k)
            jax.lax.fori_loop(0, H // ATT_G, att_body, 0)

        R = OUT_R
        gw = gw_ref[...].astype(F32).reshape(1, M)
        dv = dvec_ref[...].astype(F32).reshape(1, M)

        NC = M // OCOL

        def out_copy(it, n):
            rows = pl.ds(pl.multiple_of(it * R, R), R)
            cols = pl.ds(n * OCOL, OCOL)
            return pltpu.make_async_copy(out_v.at[rows, cols], out_hbm.at[rows, cols], osem)

        def out_body(it, carry):
            rows = pl.ds(pl.multiple_of(it * R, R), R)
            prow = pl.ds(pl.multiple_of(it * (R // 2), R // 2), R // 2)
            inv = inv_ref[...]
            ys = []
            for mm in range(R // T):
                m = it * (R // T) + mm
                qm = jnp.concatenate([_tobf(q_s[lt, m]) for lt in range(NL)], axis=1)
                ys.append(jnp.dot(inv, qm, preferred_element_type=F32))
            y = jnp.concatenate(ys, axis=0)
            ctx = jnp.concatenate([_tobf(ctx_s[h, :, rows]).T for h in range(H)], axis=1)
            kv = jnp.concatenate([_tobf(kv_s[lt, prow, :]) for lt in range(NL)], axis=1).astype(F32)
            xr = x_v[rows, :].astype(F32)
            g = jax.nn.sigmoid(jnp.sum(xr * gw, axis=-1, keepdims=True))
            b = (1.0 - g) * (xr * (y + kv * dv))
            for n in range(NC):
                c0, c1 = n * OCOL, (n + 1) * OCOL
                a = jnp.dot(ctx, wo_v[:, c0:c1], preferred_element_type=F32)
                out_v[rows, c0:c1] = (g * a + b[:, c0:c1]).astype(BF)
                out_copy(it, n).start()
            return carry

        with jax.named_scope("oproj"):
            jax.lax.fori_loop(0, S // R, out_body, 0)
        with jax.named_scope("wait4"):
            pltpu.make_async_copy(out_v, out_hbm, osem).wait()

    pl.run_scoped(
        phase23,
        pltpu.VMEM((H, D // 2, S), U32),
        pltpu.VMEM((S, M), BF),
        pltpu.VMEM((SKEW, T, T), F32),
    )


@jax.jit
def pallas_gated_mix__compressed_kv_cla__ssm_conv_h3__prompt_kernel(
    A_x, A_c_kv, A_w_q, A_w_uk, A_w_uv, A_w_o, B_q, B_k, B_v, B_shift_k, B_ssm_k, B_ssm_D, gate_w,
):
    fwd_np, inv_np = _dft_consts()
    fwd = jnp.asarray(fwd_np.astype(BF))
    inv = jnp.asarray(inv_np.astype(BF))
    any_spec = pl.BlockSpec(memory_space=pl.ANY)
    out = pl.pallas_call(
        _kernel,
        out_shape=jax.ShapeDtypeStruct((S, M), BF),
        in_specs=[any_spec] * 14,
        out_specs=any_spec,
        scratch_shapes=[
            pltpu.VMEM((S, M), BF),
            pltpu.VMEM((H * D, M), BF),
            pltpu.VMEM((H, D // 2, S), U32),
            pltpu.VMEM((H, S // 2, D), U32),
            pltpu.VMEM((H, D // 2, S), U32),
            pltpu.VMEM((NL, S // 2, T), U32),
            pltpu.VMEM((NL, NB, T, T), U32),
            pltpu.VMEM((4, M), BF),
            pltpu.VMEM((M,), BF),
            pltpu.VMEM((M,), BF),
            pltpu.VMEM((2 * T, T), BF),
            pltpu.VMEM((T, 2 * T), BF),
            pltpu.SemaphoreType.DMA((WUV_SEM + 4,)),
            pltpu.SemaphoreType.DMA(()),
        ],
        compiler_params=pltpu.CompilerParams(vmem_limit_bytes=120 * 1024 * 1024),
    )(
        A_x.reshape(S, M), A_c_kv.reshape(S, C),
        A_w_q, A_w_uk, A_w_uv,
        A_w_o.reshape(H * D, M),
        B_k.reshape(S, M), B_v.reshape(S, M), B_ssm_k,
        B_shift_k.T, B_ssm_D, gate_w, fwd, inv,
    )
    return out.reshape(1, S, M)
```

```python
import functools
import math

import jax
import jax.numpy as jnp
import numpy as np
import jax.experimental.pallas as pl
import jax.experimental.pallas.tpu as pltpu

BF = jnp.bfloat16
F32 = jnp.float32
U32 = jnp.uint32

S = 2048
M = 1024
C = 512
H = 32
D = 128
T = 128
NB = S // T
NL = M // T
NEG = -1e30
NT_DIMS = (((1,), (1,)), ((), ()))

ATT_G = 4
C_CHUNKS = [(0, 128), (128, 512), (512, 2048)]
SKEW = 6
OUNROLL = 2
OCOL = 128
WQ_SEM = 17
WUV_SEM = 21
OUT_R = 256


def _tobf(x):
    return pltpu.bitcast(x, BF)


def _tou(x):
    return pltpu.bitcast(x, U32)


def _lo_hi(w):
    lo = pltpu.bitcast(w << 16, F32)
    hi = pltpu.bitcast(w & jnp.uint32(0xFFFF0000), F32)
    return lo, hi


def _dft_consts():
    n_fft = 2 * T
    f = np.concatenate([np.arange(0, T, 2), np.arange(1, T, 2)]).astype(np.float64)
    theta = 2.0 * np.pi * (f + 0.5) / n_fft
    n = np.arange(T, dtype=np.float64)
    ang = theta[:, None] * n[None, :]
    re = np.cos(ang)
    im = -np.sin(ang)
    fwd = np.concatenate([re.reshape(T // 8, 8, T), im.reshape(T // 8, 8, T)], axis=1)
    fwd = fwd.reshape(2 * T, T)
    inv = np.stack([re, im], axis=1).reshape(2 * T, T).T * (2.0 / n_fft)
    return fwd.astype(np.float32), inv.astype(np.float32)


def _qk_tile(h, j, i, k_s, qT_s):
    qT = _tobf(qT_s[h, :, j * T:(j + 1) * T])
    kk = _tobf(k_s[h, i * T // 2:(i + 1) * T // 2, :])
    return jnp.dot(kk, qT, preferred_element_type=F32)


def _softmax_pv(h, j, i, s, st, vT_s, ctx_s):
    if i == j:
        ki = jax.lax.broadcasted_iota(jnp.int32, (T, T), 0)
        qi = jax.lax.broadcasted_iota(jnp.int32, (T, T), 1)
        s = jnp.where(ki <= qi, s, NEG)
    mc = jnp.max(s, axis=0, keepdims=True)
    m_new = mc if i == 0 else jnp.maximum(st["m"], mc)
    p = jnp.exp2(s - m_new)
    lc = jnp.sum(p.reshape(T // 8, 8, T), axis=0)
    pv = jnp.dot(_tobf(vT_s[h, :, i * T:(i + 1) * T]), p.astype(BF), preferred_element_type=F32)
    if i == 0:
        acc, l = pv, lc
    else:
        alpha = jnp.exp2(st["m"] - m_new)
        l = alpha * st["l"] + lc
        acc = alpha * st["acc"] + pv
    st.update(m=m_new, l=l, acc=acc)
    if i == j:
        lsum = jnp.sum(l, axis=0, keepdims=True)
        o = acc * (1.0 / lsum)
        ctx_s[h, :, j * T:(j + 1) * T] = _tou(o.astype(BF))


MG = 8
IG = 4
SPLIT0 = 1
KV0 = 1
KVCH = 2
FIRST = 4
LAST = 15
NG = T // 8
U_OFF = 0
W_OFF = U_OFF + NB * NG * 24
A_OFF = W_OFF + NB * NG * 24
R_OFF = A_OFF + NB * 8
DUMMY = R_OFF + NB * 8
UK_ROWS = DUMMY + 8


def _conv_pieces(lt, bk_v, bv_v, sk_v, skT_s, fwd_ref, kv_s, q_s, uk_s, dyn, dyn2):
    st = {}

    def p_kv(i, val):
        if val is not None:
            bk_v[dyn2, 0:8, :] = val.astype(BF)
        r0 = i * T
        kf = bk_v[lt, r0:r0 + T, :].astype(F32)
        prev = st["klast"] if i > 0 else jnp.zeros((8, T), F32)
        ext = jnp.concatenate([prev, kf], axis=0)
        st["klast"] = kf[T - 8:]
        sk = skT_s[lt]
        ksh = kf * sk[0:1, :]
        for j in range(1, 4):
            ksh = ksh + pltpu.roll(ext, j, 0)[8:] * sk[j:j + 1, :]
        kv = (ksh * bv_v[lt, r0:r0 + T, :].astype(F32)).astype(BF)
        kv_s[lt, r0 // 2:(r0 + T) // 2, :] = _tou(kv)
        st["kv", i] = kv

    def p_dft_k(_):
        fwd = fwd_ref[...]
        ssm = sk_v[pl.ds(pl.multiple_of(lt * T, T), T), :]
        prev = None
        for d in range(NB):
            k = jax.lax.dot_general(fwd, ssm[:, d * T:(d + 1) * T], NT_DIMS,
                                    preferred_element_type=F32)
            for g in range(NG):
                kr, ki = k[16 * g:16 * g + 8], k[16 * g + 8:16 * g + 16]
                if prev is None:
                    wr, wi = kr, ki
                else:
                    pr, pi = prev[16 * g:16 * g + 8], prev[16 * g + 8:16 * g + 16]
                    if g < NG // 2:
                        wr, wi = kr - pi, ki + pr
                    else:
                        wr, wi = kr + pi, ki - pr
                r = W_OFF + (g * NB + d) * 24
                uk_s[r:r + 8, :] = wr
                uk_s[r + 8:r + 16, :] = wi - wr
                uk_s[r + 16:r + 24, :] = -(wr + wi)
            prev = k

    def p_dft_u(i):
        fwd = fwd_ref[...]
        u = jnp.dot(fwd, st["kv", i], preferred_element_type=F32)
        for g in range(NG):
            ur, ui = u[16 * g:16 * g + 8], u[16 * g + 8:16 * g + 16]
            r = U_OFF + (g * NB + i) * 24
            uk_s[r:r + 8, :] = ur
            uk_s[r + 8:r + 16, :] = ui
            uk_s[r + 16:r + 24, :] = ur + ui

    def gate(val):
        if val is not None:
            uk_s[pl.ds(dyn, 8), :] = val

    def ld1(off, g, k, i):
        r = off + (g * NB + i) * 24 + 8 * k
        return uk_s[r:r + 8, :]

    def sub(kind, g, m0, i0, val):
        gate(val)
        ka, kb = {"a": (2, 0), "c": (1, 2), "b": (0, 1)}[kind]
        ms = range(m0, m0 + MG)
        if i0 == 0:
            if kind == "a":
                st["acc"] = {m: None for m in ms}
            else:
                st["acc"] = {m: uk_s[A_OFF + 8 * m:A_OFF + 8 * m + 8, :] for m in ms}
        acc = st["acc"]
        av = {i: ld1(U_OFF, g, ka, i) for i in range(i0, min(i0 + IG, m0 + MG))}
        bv = {}
        for i in av:
            for m in ms:
                j = m - i
                if j < 0:
                    continue
                if j not in bv:
                    bv[j] = ld1(W_OFF, g, kb, j)
                t = av[i] * bv[j]
                acc[m] = t if acc[m] is None else acc[m] + t
        if i0 + IG >= m0 + MG:
            for m in ms:
                if kind == "a":
                    uk_s[A_OFF + 8 * m:A_OFF + 8 * m + 8, :] = acc[m]
                elif kind == "c":
                    uk_s[R_OFF + 8 * m:R_OFF + 8 * m + 8, :] = acc[m]
                else:
                    re = uk_s[R_OFF + 8 * m:R_OFF + 8 * m + 8, :]
                    q_s[lt, m, g * 8:(g + 1) * 8, :] = pltpu.pack_elementwise(
                        [re, acc[m]], packed_dtype=BF)

    subs = []
    for g in range(NG):
        for kind in ("a", "c", "b"):
            for m0 in range(0, NB, MG):
                for i0 in range(0, m0 + MG, IG):
                    subs.append(functools.partial(sub, kind, g, m0, i0))
    return p_dft_k, p_kv, p_dft_u, subs


def _spread(subs, n, first, last, slabs=128):
    sched = [[] for _ in range(n)]
    npts = (last - first) * slabs
    for i, pc in enumerate(subs):
        pt = (i * npts) // len(subs)
        sched[first + pt // slabs].append((pt % slabs, pc))
    return sched


def _kernel(x_hbm, c_hbm, wq_hbm, wuk_hbm, wuv_hbm, wo_hbm, bk_hbm, bv_hbm, sk_hbm,
            shT_hbm, dvec_hbm, gw_hbm, fwd_hbm, inv_hbm,
            out_hbm,
            x_v, wo_v, qT_s, k_s, vT_s, kv_s, q_s,
            shT_ref, dvec_ref, gw_ref, fwd_ref, inv_ref, sems, osem):
    qscale = (D ** -0.5) * math.log2(math.e)

    def phase1(c_v, wq_v, wuk_v, wuv_v, bk_v, bv_v, sk_v, skT_s, uk_s, dyn_s):
        dyn_s[0] = DUMMY
        dyn_s[1] = NL
        wuk_hbm32 = wuk_hbm.bitcast(U32)
        cp_wuk = [pltpu.make_async_copy(
            wuk_hbm32.at[:, pl.ds(4 * a, 4), :], wuk_v.at[a, :, pl.ds(0, 4), :], sems.at[9 + a])
            for a in range(4)]
        cp_c = [pltpu.make_async_copy(c_hbm.at[pl.ds(r0, r1 - r0)], c_v.at[pl.ds(r0, r1 - r0)],
                                      sems.at[14 + i]) for i, (r0, r1) in enumerate(C_CHUNKS)]
        wq_hbm32 = wq_hbm.bitcast(U32)
        wuv_hbm32 = wuv_hbm.bitcast(U32)

        def cp_quarter(w_hbm32, w_v, sem0, q):
            start = 4 * q if isinstance(q, int) else pl.multiple_of(4 * q, 4)
            return pltpu.make_async_copy(w_hbm32.at[:, pl.ds(start, 4), :],
                                         w_v.at[q % 2, :, pl.ds(0, 4), :], sems.at[sem0 + q])

        cp_x = pltpu.make_async_copy(x_hbm, x_v, sems.at[3])
        cp_sk = pltpu.make_async_copy(sk_hbm, sk_v, sems.at[5])
        cp_bk = [pltpu.make_async_copy(bk_hbm.at[:, pl.ds(lt * T, T)], bk_v.at[lt], sems.at[6])
                 for lt in range(NL)]
        cp_bv = [pltpu.make_async_copy(bv_hbm.at[:, pl.ds(lt * T, T)], bv_v.at[lt], sems.at[7])
                 for lt in range(NL)]
        cp_wo = pltpu.make_async_copy(wo_hbm, wo_v, sems.at[8])
        cp_tiny = [pltpu.make_async_copy(a, b, sems.at[0]) for a, b in
                   [(shT_hbm, shT_ref), (dvec_hbm, dvec_ref), (gw_hbm, gw_ref)]]
        cp_small = [pltpu.make_async_copy(a, b, sems.at[13]) for a, b in
                    [(fwd_hbm, fwd_ref), (inv_hbm, inv_ref)]]
        cp_wq = [cp_quarter(wq_hbm32, wq_v, WQ_SEM, q) for q in range(2)]
        cp_wuv = [cp_quarter(wuv_hbm32, wuv_v, WUV_SEM, q) for q in range(2)]
        for cp in (cp_tiny + [cp_wuk[0]] + cp_c + cp_wuk[1:] + cp_small + [cp_x] + cp_wq + [cp_sk]
                   + cp_bk + cp_bv + cp_wuv + [cp_wo]):
            cp.start()

        for cp in cp_tiny:
            cp.wait()
        shT = shT_ref[...].astype(F32)
        for lt in range(NL):
            skT_s[lt] = jnp.concatenate(
                [shT[:, lt * T:(lt + 1) * T], jnp.zeros((4, T), F32)], axis=0)

        def load_weights_t(w_v, rows, it):
            w2 = w_v.reshape(2 * rows * 8, D)
            view = w2.at[pl.ds(pl.multiple_of((it % 2) * rows * 8, 8), rows * 8)]
            outs = []
            for g in range(4):
                outs += list(_lo_hi(view[pl.ds(g, rows, stride=8), :].T))
            return jnp.concatenate(outs, axis=0).astype(BF)

        wuk2 = wuk_v.reshape(4 * C * 8, D)

        def k_group(it, first):
            pltpu.make_async_copy(wuk_hbm32.at[:, pl.ds(pl.multiple_of(4 * it, 4), 4), :],
                                  wuk_v.at[it, :, pl.ds(0, 4), :], sems.at[9 + it]).wait()
            view = wuk2.at[pl.ds(pl.multiple_of(it * C * 8, 8), C * 8)]
            ws = []
            for g in range(4):
                lo, hi = _lo_hi(view[pl.ds(g, C, stride=8), :])
                ws.append(jnp.concatenate([lo, hi], axis=1).astype(BF))
            for i, (r0, r1) in enumerate(C_CHUNKS if first else [(0, S)]):
                if first:
                    cp_c[i].wait()
                for g in range(4):
                    k = jnp.dot(c_v[r0:r1, :], ws[g], preferred_element_type=F32)
                    for u in range(2):
                        k_s[it * 8 + 2 * g + u, r0 // 2:r1 // 2, :] = _tou(
                            k[:, u * D:(u + 1) * D].astype(BF))

        def k_body(it, carry):
            with jax.named_scope("k_it"):
                k_group(it, False)
            return carry

        with jax.named_scope("kproj0"):
            k_group(0, True)
        with jax.named_scope("kproj"):
            jax.lax.fori_loop(1, 4, k_body, 0)

        def proj_conv_body(it, lt, w_hbm32, w_v, sem0, rows, src_v, dst_s, scale):
            cp_quarter(w_hbm32, w_v, sem0, it).wait()
            p_dft_k, p_kv, p_dft_u, subs = _conv_pieces(
                lt, bk_v, bv_v, sk_v, skT_s, fwd_ref, kv_s, q_s, uk_s,
                pl.multiple_of(dyn_s[0], 8), dyn_s[1])
            p_dft_k(None)
            w = load_weights_t(w_v, rows, it)
            sched = _spread(subs, NB, FIRST, LAST)
            nkv = NB // KVCH
            for n in range(NB):
                src = src_v[n * T:(n + 1) * T, :]
                if n < SPLIT0:
                    o = jnp.concatenate(
                        [jax.lax.dot_general(w[p * 2 * D:(p + 1) * 2 * D], src, NT_DIMS,
                                             preferred_element_type=F32) for p in range(4)], axis=0)
                else:
                    o = jax.lax.dot_general(w, src, NT_DIMS, preferred_element_type=F32)
                if scale is not None:
                    o = o * scale
                for g in range(8):
                    dst_s[it * 8 + g, :, n * T:(n + 1) * T] = _tou(o[g * D:(g + 1) * D].astype(BF))
                if KV0 + 1 <= n <= KV0 + KVCH:
                    for i in range((n - KV0 - 1) * nkv, (n - KV0) * nkv):
                        p_dft_u(i)
                if KV0 <= n < KV0 + KVCH:
                    for k_ in range(nkv):
                        sl = (128 * k_) // nkv
                        p_kv((n - KV0) * nkv + k_, o[8 * sl:8 * sl + 8])
                for sl, pc in sched[n]:
                    pc(o[8 * sl:8 * sl + 8])

            @pl.when(it < 2)
            def _():
                cp_quarter(w_hbm32, w_v, sem0, it + 2).start()

        def q_body(it, carry):
            with jax.named_scope("q_it"):
                proj_conv_body(it, it, wq_hbm32, wq_v, WQ_SEM, M, x_v, qT_s, qscale)
            return carry

        def v_body(it, carry):
            with jax.named_scope("v_it"):
                proj_conv_body(it, 4 + it, wuv_hbm32, wuv_v, WUV_SEM, C, c_v, vT_s, None)
            return carry

        with jax.named_scope("wait1"):
            for cp in cp_small + [cp_x, cp_sk]:
                cp.wait()
            pltpu.make_async_copy(bk_v.at[0:NL], bk_v.at[0:NL], sems.at[6]).wait()
            pltpu.make_async_copy(bv_v, bv_v, sems.at[7]).wait()
        with jax.named_scope("qproj"):
            jax.lax.fori_loop(0, 4, q_body, 0)
        with jax.named_scope("vproj"):
            jax.lax.fori_loop(0, 4, v_body, 0)
        with jax.named_scope("wait3"):
            cp_wo.wait()

    pl.run_scoped(
        phase1,
        pltpu.VMEM((S, C), BF),
        pltpu.VMEM((2, M, 8, D), U32),
        pltpu.VMEM((4, C, 8, D), U32),
        pltpu.VMEM((2, C, 8, D), U32),
        pltpu.VMEM((NL + 1, S, T), BF),
        pltpu.VMEM((NL, S, T), BF),
        pltpu.VMEM((M, S), BF),
        pltpu.VMEM((NL, 8, T), F32),
        pltpu.VMEM((UK_ROWS, T), F32),
        pltpu.SMEM((2,), jnp.int32),
    )

    def phase23(ctx_s, out_v, spre_s):
        ORDER = 0
        if ORDER == 0:
            tiles = [(g, j, i) for j in range(NB) for g in range(ATT_G) for i in range(j + 1)]
        elif ORDER == 1:
            tiles = [(g, j, i) for j in range(NB) for i in range(j + 1) for g in range(ATT_G)]
        elif ORDER == 2:
            tiles = [(g, j, i) for g in range(ATT_G) for j in range(NB) for i in range(j + 1)]
        elif ORDER == 3:
            tiles = [(g, j, i) for j in reversed(range(NB)) for g in range(ATT_G) for i in range(j + 1)]
        elif ORDER == 4:
            tiles = [(g, j, i) for j in range(NB) for gp in range(0, ATT_G, 2) for i in range(j + 1)
                     for g in (gp, gp + 1)]

        def qk_next(base, k):
            g, j, i = tiles[k]
            spre_s[k] = _qk_tile(base + g, j, i, k_s, qT_s)

        def att_body(it, carry):
            with jax.named_scope("att_it"):
                return att_body2(it, carry)

        def att_body2(it, carry):
            base = it * ATT_G
            nxt = jnp.minimum(base + ATT_G, H - ATT_G)
            sv = {k: spre_s[k] for k in range(SKEW)}
            states = {}
            for k, (g, j, i) in enumerate(tiles):
                if k + SKEW < len(tiles):
                    g2, j2, i2 = tiles[k + SKEW]
                    sv[k + SKEW] = _qk_tile(base + g2, j2, i2, k_s, qT_s)
                else:
                    qk_next(nxt, k + SKEW - len(tiles))
                _softmax_pv(base + g, j, i, sv.pop(k), states.setdefault((g, j), {}), vT_s, ctx_s)
            return carry

        with jax.named_scope("attn"):
            for k in range(SKEW):
                qk_next(0, k)
            jax.lax.fori_loop(0, H // ATT_G, att_body, 0)

        R = OUT_R
        gw = gw_ref[...].astype(F32).reshape(1, M)
        dv = dvec_ref[...].astype(F32).reshape(1, M)

        NC = M // OCOL

        def out_copy(it, n):
            rows = pl.ds(pl.multiple_of(it * R, R), R)
            cols = pl.ds(n * OCOL, OCOL)
            return pltpu.make_async_copy(out_v.at[rows, cols], out_hbm.at[rows, cols], osem)

        def out_body(it, carry):
            rows = pl.ds(pl.multiple_of(it * R, R), R)
            prow = pl.ds(pl.multiple_of(it * (R // 2), R // 2), R // 2)
            inv = inv_ref[...]
            ys = []
            for mm in range(R // T):
                m = it * (R // T) + mm
                qm = jnp.concatenate([_tobf(q_s[lt, m]) for lt in range(NL)], axis=1)
                ys.append(jnp.dot(inv, qm, preferred_element_type=F32))
            y = jnp.concatenate(ys, axis=0)
            ctx = jnp.concatenate([_tobf(ctx_s[h, :, rows]).T for h in range(H)], axis=1)
            kv = jnp.concatenate([_tobf(kv_s[lt, prow, :]) for lt in range(NL)], axis=1).astype(F32)
            xr = x_v[rows, :].astype(F32)
            g = jax.nn.sigmoid(jnp.sum(xr * gw, axis=-1, keepdims=True))
            b = (1.0 - g) * (xr * (y + kv * dv))
            for n in range(NC):
                c0, c1 = n * OCOL, (n + 1) * OCOL
                a = jnp.dot(ctx, wo_v[:, c0:c1], preferred_element_type=F32)
                out_v[rows, c0:c1] = (g * a + b[:, c0:c1]).astype(BF)
                out_copy(it, n).start()
            return carry

        with jax.named_scope("oproj"):
            jax.lax.fori_loop(0, S // R, out_body, 0, unroll=OUNROLL)
        with jax.named_scope("wait4"):
            pltpu.make_async_copy(out_v, out_hbm, osem).wait()

    pl.run_scoped(
        phase23,
        pltpu.VMEM((H, D // 2, S), U32),
        pltpu.VMEM((S, M), BF),
        pltpu.VMEM((SKEW, T, T), F32),
    )


@jax.jit
def pallas_gated_mix__compressed_kv_cla__ssm_conv_h3__prompt_kernel(
    A_x, A_c_kv, A_w_q, A_w_uk, A_w_uv, A_w_o, B_q, B_k, B_v, B_shift_k, B_ssm_k, B_ssm_D, gate_w,
):
    fwd_np, inv_np = _dft_consts()
    fwd = jnp.asarray(fwd_np.astype(BF))
    inv = jnp.asarray(inv_np.astype(BF))
    any_spec = pl.BlockSpec(memory_space=pl.ANY)
    out = pl.pallas_call(
        _kernel,
        out_shape=jax.ShapeDtypeStruct((S, M), BF),
        in_specs=[any_spec] * 14,
        out_specs=any_spec,
        scratch_shapes=[
            pltpu.VMEM((S, M), BF),
            pltpu.VMEM((H * D, M), BF),
            pltpu.VMEM((H, D // 2, S), U32),
            pltpu.VMEM((H, S // 2, D), U32),
            pltpu.VMEM((H, D // 2, S), U32),
            pltpu.VMEM((NL, S // 2, T), U32),
            pltpu.VMEM((NL, NB, T, T), U32),
            pltpu.VMEM((4, M), BF),
            pltpu.VMEM((M,), BF),
            pltpu.VMEM((M,), BF),
            pltpu.VMEM((2 * T, T), BF),
            pltpu.VMEM((T, 2 * T), BF),
            pltpu.SemaphoreType.DMA((WUV_SEM + 4,)),
            pltpu.SemaphoreType.DMA(()),
        ],
        compiler_params=pltpu.CompilerParams(vmem_limit_bytes=120 * 1024 * 1024),
    )(
        A_x.reshape(S, M), A_c_kv.reshape(S, C),
        A_w_q, A_w_uk, A_w_uv,
        A_w_o.reshape(H * D, M),
        B_k.reshape(S, M), B_v.reshape(S, M), B_ssm_k,
        B_shift_k.T, B_ssm_D, gate_w, fwd, inv,
    )
    return out.reshape(1, S, M)
```
